```python
import jax
import jax.numpy as jnp

def _softmax(x, axis=-1):
    return jax.nn.softmax(x, axis=axis)

def _gelu(x):
    return jax.nn.gelu(x, approximate=True)

def _silu(x):
    return jax.nn.silu(x)

def _sigmoid(x):
    return jax.nn.sigmoid(x)

def _layernorm(x, axis=-1, eps=1e-05):
    m = jnp.mean(x, axis=axis, keepdims=True)
    v = jnp.var(x, axis=axis, keepdims=True)
    return (x - m) / jnp.sqrt(v + eps)

def _scatter_add(tgt, idx, src, axis=0):
    return tgt.at[idx].add(src)

def _segment_sum(src, seg, n):
    return jax.ops.segment_sum(src, seg, n)

class _Rng:

    def __init__(self, key):
        self._k = key

    def _next(self):
        self._k, sub = jax.random.split(self._k)
        return sub

    def normal(self, shape):
        return jax.random.normal(self._next(), shape, dtype=jnp.bfloat16)

    def randint(self, lo, hi, shape):
        return jax.random.randint(self._next(), shape, lo, hi, dtype=jnp.int32)

    def uniform(self, shape, lo=0.0, hi=1.0):
        return jax.random.uniform(self._next(), shape, jnp.bfloat16, lo, hi)

    def permutation(self, n):
        return jax.random.permutation(self._next(), n)
kernel_name = 'adaLN_cond__mha_block_cached__moe_arch_mod__prompt'

def setup_inputs():
    _rng = _Rng(jax.random.key(int.from_bytes(__import__("os").urandom(4), "little")))
    _w = lambda a: (lambda t: t.astype(jnp.bfloat16) if jnp.issubdtype(t.dtype, jnp.floating) else t)(jnp.asarray(a))

    def _A_setup():
        B, Sq, D = (1, 2048, 1024)
        H, Sk, Dh = (32, 2048, 128)
        return {'x': _w((lambda *s: _rng.normal(s) * 0.05)(B, Sq, D)), 'k_cache': _w((lambda *s: _rng.normal(s) * 0.05)(B, H, Sk, Dh)), 'v_cache': _w((lambda *s: _rng.normal(s) * 0.05)(B, H, Sk, Dh)), 'wq': _w((lambda *s: _rng.normal(s) * 0.05)(D, H * Dh) * D ** (-0.5)), 'wo': _w((lambda *s: _rng.normal(s) * 0.05)(H * Dh, D) * (H * Dh) ** (-0.5))}
    _A_in = _A_setup()

    def _B_setup():
        B, S, D, F, C = (1, 2048, 1024, 3584, 2)
        return {'x': _w((lambda *s: _rng.normal(s) * 0.05)(B, S, D)), 'w_r': _w((lambda *s: _rng.normal(s) * 0.05)(D)), 'w_gate': _w((lambda *s: _rng.normal(s) * 0.05)(D, F)), 'w_up': _w((lambda *s: _rng.normal(s) * 0.05)(D, F)), 'w_down': _w((lambda *s: _rng.normal(s) * 0.05)(F, D))}
    _B_in = _B_setup()
    return {'A_x': _A_in['x'], 'A_k_cache': _A_in['k_cache'], 'A_v_cache': _A_in['v_cache'], 'A_wq': _A_in['wq'], 'A_wo': _A_in['wo'], 'B_x': _B_in['x'], 'B_w_r': _B_in['w_r'], 'B_w_gate': _B_in['w_gate'], 'B_w_up': _B_in['w_up'], 'B_w_down': _B_in['w_down'], 'c': _w((lambda *s: _rng.normal(s) * 0.05)(1, 1024)), 'w_mod': _w((lambda *s: _rng.normal(s) * 0.05)(1024, 6 * 1024) * 1024 ** (-0.5))}

def reference(A_x, A_k_cache, A_v_cache, A_wq, A_wo, B_x, B_w_r, B_w_gate, B_w_up, B_w_down, c, w_mod):

    def _A_ref(x, k_cache, v_cache, wq, wo):
        B, Sq, D = x.shape
        H, Dh = (32, 128)
        q = (lambda x, *d: x.transpose(*d))((x @ wq).reshape(B, Sq, H, Dh), 0, 2, 1, 3)
        scores = jnp.einsum('bhqd,bhkd->bhqk', q, k_cache) * Dh ** (-0.5)
        p = _softmax(scores, axis=-1)
        o = jnp.einsum('bhqk,bhkd->bhqd', p, v_cache)
        return (lambda x, *d: x.transpose(*d))(o, 0, 2, 1, 3).reshape(B, Sq, H * Dh) @ wo

    def _B_ref(x, w_r, w_gate, w_up, w_down):
        B, S, D = x.shape
        C = 2
        r = x @ w_r
        idx = jnp.argsort(-r, axis=-1)[:, :C]
        idx_e = jnp.repeat(idx.reshape(B, C, 1), D, axis=2)
        x_sel = jnp.take_along_axis(x, idx_e, axis=1)
        g = _silu(x_sel @ w_gate)
        u = x_sel @ w_up
        y = g * u @ w_down
        r_sel = _sigmoid(jnp.take_along_axis(r, idx, axis=1))
        y = y * r_sel.reshape(B, C, 1)
        b_off = (jnp.arange(B) * S).reshape(B, 1)
        flat_idx = (idx + b_off).reshape(B * C)
        zero = (x * 0.0).reshape(B * S, D)
        upd = _scatter_add(zero, flat_idx, y.reshape(B * C, D), axis=0)
        return x + upd.reshape(B, S, D)
    x = A_x
    mod = (_silu(c) @ w_mod).reshape(c.shape[0], 6, 1, -1)
    sa, ca, ga, sb, cb, gb = (mod[:, 0].copy(), mod[:, 1].copy(), mod[:, 2].copy(), mod[:, 3].copy(), mod[:, 4].copy(), mod[:, 5].copy())
    h = _layernorm(x, axis=-1) * (1 + ca) + sa
    x = x + ga * _A_ref(h, A_k_cache, A_v_cache, A_wq, A_wo)
    h = _layernorm(x, axis=-1) * (1 + cb) + sb
    x = x + gb * _B_ref(h, B_w_r, B_w_gate, B_w_up, B_w_down)
    return x
```

```python
import functools

import jax
import jax.numpy as jnp
import jax.experimental.pallas as pl
import jax.experimental.pallas.tpu as pltpu

F32, BF16, U32, I32 = jnp.float32, jnp.bfloat16, jnp.uint32, jnp.int32

S, D, H, DH, FF = 2048, 1024, 32, 128, 3584
TU = 256
TQ = 512
NQ = S // TQ
HG = 4
NG = H // HG
NT = NQ * NG
SL = TQ // NG
RC = 16
EPS = 1e-5
QSCALE = DH ** -0.5 * 1.4426950408889634

SEM_SMALL = 0
SEM_X = 1
SEM_WM = 5
SEM_WMR = 9
SEM_A0 = 10
SEM_MINI = 11
SEM_GRP = 15
SEM_FFN = 23
SEM_OUT = 24
SEM_FIX = 25
NSEM = 27
WMC = 4


def _rb(x):
    return x.astype(BF16).astype(F32)


def _ub(x):
    return pltpu.bitcast(x, BF16)


def _pk(x):
    return pltpu.bitcast(x, U32)


def _recip(l):
    r = pl.reciprocal(l, approx=True)
    return r * (2.0 - l * r)


def _ln(x):
    mu = jnp.sum(x, axis=-1, keepdims=True) * (1.0 / D)
    mb = _rb(mu)
    d = x - mb
    dm = mu - mb
    var = jnp.sum(d * d, axis=-1, keepdims=True) * (1.0 / D) - dm * dm
    var = jnp.maximum(var, 0.0)
    sd = _rb(jnp.sqrt(_rb(_rb(var) + EPS)))
    return d * (1.0 / sd)


def _kernel(x_hbm, k_hbm, v_hbm, wq_hbm, wo_hbm, wr_hbm, wg_hbm, wu_hbm, wd_hbm, c_hbm, wm_hbm,
            out_hbm,
            x_buf, h_buf, k_buf, v_buf, wq_buf, wo_buf, wg_buf, wu_buf, wd_buf, wm_buf,
            c_buf, wr_buf, mod_buf, acc, out_buf, s_sc, of_sc, l_sc, r_buf, sem):
    cp = pltpu.make_async_copy

    def d_small():
        return [cp(c_hbm, c_buf, sem.at[SEM_SMALL]), cp(wr_hbm, wr_buf, sem.at[SEM_SMALL])]

    def d_x(j):
        return [cp(x_hbm.at[0, pl.ds(j * TQ, TQ), :], x_buf.at[pl.ds(j * TQ, TQ), :], sem.at[SEM_X + j])]

    def d_wm(i):
        w = 2 * D // WMC
        return [cp(wm_hbm.at[:, pl.ds(i * w, w)], wm_buf.at[:, pl.ds(i * w, w)], sem.at[SEM_WM + i])]

    def d_wmr():
        return [cp(wm_hbm.at[:, pl.ds(2 * D, 4 * D)], wm_buf.at[:, pl.ds(2 * D, 4 * D)], sem.at[SEM_WMR])]

    def d_qk(h0, n, s_):
        r = []
        for i in range(n):
            r.append(cp(wq_hbm.at[:, pl.ds(pl.multiple_of((h0 + i) * DH, DH), DH)], wq_buf.at[h0 + i], s_))
        r.append(cp(k_hbm.at[0, pl.ds(h0, n)], k_buf.at[pl.ds(h0, n)], s_))
        return r

    def d_vo(h0, n, s_):
        rows = pl.ds(pl.multiple_of(h0 * DH, DH), n * DH)
        return [cp(v_hbm.at[0, pl.ds(h0, n)], v_buf.at[pl.ds(h0, n)], s_),
                cp(wo_hbm.at[rows, :], wo_buf.at[rows, :], s_)]

    def d_mini(i):
        s_ = sem.at[SEM_MINI + i]
        return d_vo(i, 1, s_) + d_qk(i + 1, 1, s_)

    def d_grp(t):
        s_ = sem.at[SEM_GRP + t]
        n = HG if t < NG - 1 else HG - 1
        return d_vo(HG * t, HG, s_) + d_qk(HG * t + 1, n, s_)

    def d_ffn(i):
        src, dst = ((wg_hbm, wg_buf), (wu_hbm, wu_buf), (wd_hbm, wd_buf))[i]
        return [cp(src, dst, sem.at[SEM_FFN])]

    def d_out(r0, n, s_):
        return [cp(out_buf.at[pl.ds(r0, n), :], out_hbm.at[0, pl.ds(r0, n), :], s_)]

    def start(ds):
        for d in ds:
            d.start()

    def wait(ds):
        for d in ds:
            d.wait()

    def qp(unit):
        hh, sub, par = unit
        hb = _ub(h_buf[par, sub * (TU // 2):(sub + 1) * (TU // 2), :])
        q = jnp.dot(hb, wq_buf[hh], preferred_element_type=F32)
        return (q * QSCALE).astype(BF16)

    def qk(unit, q):
        hh, sub, par = unit
        return jax.lax.dot_general(q, k_buf[hh], (((1,), (1,)), ((), ())), preferred_element_type=F32)

    def pv(unit, s):
        hh, sub, par = unit
        ls, ps = [], []
        for c in range(TU // RC):
            sc = s[c * RC:(c + 1) * RC, :]
            m = jnp.max(sc, axis=-1, keepdims=True)
            p = jnp.exp2(sc - m)
            a = p[:, 0:128]
            for i in range(1, S // 128):
                a = a + p[:, i * 128:(i + 1) * 128]
            ls.append(a)
            ps.append(p.astype(BF16))
        o = jnp.dot(jnp.concatenate(ps, axis=0), v_buf[hh], preferred_element_type=F32)
        return o, jnp.concatenate(ls, axis=0)

    def outp(unit, ol):
        hh, sub, par = unit
        of, lp = ol
        l = jnp.sum(lp, axis=-1, keepdims=True)
        o = (of * _recip(l)).astype(BF16)
        w = wo_buf[pl.ds(pl.multiple_of(hh * DH, DH), DH), :]
        acc[par, sub * TU:(sub + 1) * TU, :] += jnp.dot(o, w, preferred_element_type=F32)

    def modrow(i):
        return mod_buf[0:1, i * D:(i + 1) * D]

    def ln1(xrow0, par, hrow0, n):
        x = x_buf[pl.ds(xrow0, n), :].astype(F32)
        h = _ln(x) * modrow(1) + modrow(0)
        h_buf[par, pl.ds(hrow0, n // 2), :] = _pk(h.astype(BF16))

    def ln2(x1):
        h2 = _rb(_ln(x1) * modrow(4) + modrow(3))
        r = _rb(jnp.sum(h2 * wr_buf[...].astype(F32), axis=-1, keepdims=True))
        return h2, r

    def epi(row0, par, arow0, n, zero):
        a = acc[par, pl.ds(arow0, n), :]
        if zero:
            acc[par, pl.ds(arow0, n), :] = jnp.zeros((n, D), F32)
        x1b = (x_buf[pl.ds(row0, n), :].astype(F32) + modrow(2) * a).astype(BF16)
        x_buf[pl.ds(row0, n), :] = x1b
        x1 = x1b.astype(F32)
        h2, r = ln2(x1)
        out_buf[pl.ds(row0, n), :] = (x1 + modrow(5) * h2).astype(BF16)
        hi = row0 // 1024
        c0 = (row0 % 1024) // 8
        lane = jax.lax.broadcasted_iota(I32, (8, 128), 1)
        rc = r_buf[hi]
        for i in range(n // 8):
            rc = jnp.where(lane == c0 + i, r[i * 8:(i + 1) * 8, :], rc)
        r_buf[hi] = rc

    def run_units(units, prev, nxt, side):
        s = s_sc[...]
        ol_prev = (of_sc[...], l_sc[...])
        seq = [prev] + units + [nxt]
        for u in range(len(units)):
            if u in side:
                side[u]()
            q = qp(seq[u + 2])
            ol = pv(seq[u + 1], s)
            outp(seq[u], ol_prev)
            ol_prev = ol
            s = qk(seq[u + 2], q)
        s_sc[...] = s
        of_sc[...] = ol_prev[0]
        l_sc[...] = ol_prev[1]

    def mod_cols(c0, n):
        cf = c_buf[...].astype(F32)
        sc = (cf * jax.nn.sigmoid(cf)).astype(BF16)
        sc = jnp.broadcast_to(sc, (16, D))
        m = jnp.dot(sc, wm_buf[:, c0:c0 + n], preferred_element_type=F32)
        return _rb(m[0:8, :])

    start(d_small())
    start(d_x(0))
    for i in range(WMC):
        start(d_wm(i))
    start(d_qk(0, 1, sem.at[SEM_A0]))
    start(d_mini(0))
    start(d_x(1))
    for i in range(1, HG):
        start(d_mini(i))
    start(d_grp(1))

    acc[...] = jnp.zeros(acc.shape, F32)
    mod_buf[...] = jnp.zeros(mod_buf.shape, F32)
    r_buf[...] = jnp.zeros(r_buf.shape, F32)
    of_sc[...] = jnp.zeros(of_sc.shape, F32)
    l_sc[...] = jnp.ones(l_sc.shape, F32)

    wait(d_small())
    wcol = 2 * D // WMC
    for i in range(WMC):
        wait(d_wm(i))
        m = mod_cols(i * wcol, wcol)
        if i * wcol >= D:
            m = _rb(1.0 + m)
        mod_buf[:, i * wcol:(i + 1) * wcol] = m
    wait(d_x(0))

    def ln1_first(i, _):
        r0 = pl.multiple_of(i * 64, 64)
        ln1(r0, 0, pl.multiple_of(i * 32, 32), 64)
        return 0
    jax.lax.fori_loop(0, TQ // 64, ln1_first, 0)
    wait(d_qk(0, 1, sem.at[SEM_A0]))
    s_sc[...] = qk((0, 0, 0), qp((0, 0, 0)))
    wait(d_x(1))

    def mini(i, _):
        wait(d_mini(i))
        sl = SL // HG
        side = {0: lambda: ln1(pl.multiple_of(TQ + i * sl, sl), 1, pl.multiple_of(i * (sl // 2), sl // 2), sl)}
        run_units([(i, 0, 0), (i, 1, 0)], (jnp.maximum(i - 1, 0), 1, 0), (i + 1, 0, 0), side)
        return 0
    jax.lax.fori_loop(0, HG, mini, 0)

    def main(t, _):
        j = t >> 3
        g = t & (NG - 1)

        @pl.when(t <= 17)
        def _():
            for c_ in range(1, NG):
                @pl.when(t == c_)
                def _():
                    wait(d_grp(c_))
                    if c_ + 1 < NG:
                        start(d_grp(c_ + 1))
                    if c_ == 2:
                        start(d_wmr())
                    if c_ == 4:
                        start(d_x(2))
                    if c_ == 5:
                        start(d_x(3))
                    if c_ == NG - 1:
                        start(d_ffn(0))

            @pl.when(t == NG)
            def _():
                wait(d_wmr())
                wait(d_x(2))
                start(d_ffn(1))
                for i in range(2, 6):
                    m = mod_cols(i * D, D)
                    if i == 4:
                        m = _rb(1.0 + m)
                    mod_buf[:, i * D:(i + 1) * D] = m

            @pl.when(t == NG + 1)
            def _():
                start(d_ffn(2))

            @pl.when(t == 2 * NG)
            def _():
                wait(d_x(3))

        @pl.when(t > NG)
        def _():
            start(d_out(pl.multiple_of((t - 1 - NG) * SL, SL), SL, sem.at[SEM_OUT]))

        par = j & 1
        units = [(g * HG + (u >> 1), u & 1, par) for u in range(2 * HG)]
        tp = t - 1
        prev = ((tp & (NG - 1)) * HG + HG - 1, 1, (tp >> 3) & 1)
        tn = jnp.minimum(t + 1, NT - 1)
        nxt = ((tn & (NG - 1)) * HG, 0, (tn >> 3) & 1)
        jn = jnp.minimum(j + 1, NQ - 1)
        jp = jnp.maximum(j - 1, 0)
        side = {
            2: lambda: epi(pl.multiple_of(jp * TQ + g * SL, SL), 1 - par, pl.multiple_of(g * SL, SL), SL, True),
            4: lambda: ln1(pl.multiple_of(jn * TQ + g * SL, SL), 1 - par,
                           pl.multiple_of(g * (SL // 2), SL // 2), SL),
        }
        run_units(units, prev, nxt, side)
        return 0
    jax.lax.fori_loop(1, NT, main, 0)

    start(d_out((NT - 1 - NG) * SL, SL, sem.at[SEM_OUT]))
    lastp = (NQ - 1) & 1
    outp((H - 1, 1, lastp), (of_sc[...], l_sc[...]))

    def epi_last(i, _):
        r0 = pl.multiple_of(i * SL, SL)
        epi((NQ - 1) * TQ + r0, lastp, r0, SL, False)
        return 0
    jax.lax.fori_loop(0, TQ // SL, epi_last, 0)
    start(d_out((NQ - 1) * TQ, TQ, sem.at[SEM_OUT]))

    rv = r_buf[...].reshape(16, 128)
    sub_i = jax.lax.broadcasted_iota(I32, (16, 128), 0)
    lane_i = jax.lax.broadcasted_iota(I32, (16, 128), 1)
    rowid = ((sub_i >> 3) * 1024 + lane_i * 8 + (sub_i & 7)).astype(F32)
    big = float(S)
    m1 = jnp.max(rv, keepdims=True)
    i1f = jnp.min(jnp.where(rv == m1, rowid, big), keepdims=True)
    rv2 = jnp.where(rowid == i1f, -jnp.inf, rv)
    m2 = jnp.max(rv2, keepdims=True)
    i2f = jnp.min(jnp.where((rv2 == m2) & (rowid != i1f), rowid, big), keepdims=True)
    i1 = jnp.clip(i1f[0, 0].astype(I32), 0, S - 1)
    i2 = jnp.clip(i2f[0, 0].astype(I32), 0, S - 1)
    g1 = pl.multiple_of((i1 >> 3) << 3, 8)
    g2 = pl.multiple_of((i2 >> 3) << 3, 8)

    x1 = jnp.concatenate([x_buf[pl.ds(g1, 8), :].astype(F32), x_buf[pl.ds(g2, 8), :].astype(F32)], axis=0)
    h2, r = ln2(x1)
    for i in range(3):
        wait(d_ffn(i))
    xs = h2.astype(BF16)
    gt = _rb(jnp.dot(xs, wg_buf[...], preferred_element_type=F32))
    up = _rb(jnp.dot(xs, wu_buf[...], preferred_element_type=F32))
    a = (_rb(gt * jax.nn.sigmoid(gt)) * up).astype(BF16)
    y = _rb(jnp.dot(a, wd_buf[...], preferred_element_type=F32))
    y = _rb(y * _rb(jax.nn.sigmoid(r)))
    ri = jax.lax.broadcasted_iota(I32, (16, 1), 0)
    rows = jnp.where(ri < 8, g1 + ri, g2 + ri - 8)
    sel = (rows == i1) | (rows == i2)
    o = (x1 + modrow(5) * jnp.where(sel, _rb(h2 + y), h2))

    cp(out_buf, out_hbm.at[0], sem.at[SEM_OUT]).wait()
    out_buf[pl.ds(g1, 8), :] = o[0:8].astype(BF16)
    out_buf[pl.ds(g2, 8), :] = o[8:16].astype(BF16)
    start(d_out(g1, 8, sem.at[SEM_FIX]))

    @pl.when(g1 != g2)
    def _():
        start(d_out(g2, 8, sem.at[SEM_FIX + 1]))
        wait(d_out(g2, 8, sem.at[SEM_FIX + 1]))

    wait(d_out(g1, 8, sem.at[SEM_FIX]))


@jax.jit
def pallas_adaLN_cond__mha_block_cached__moe_arch_mod__prompt_kernel(
    A_x: jax.Array,
    A_k_cache: jax.Array,
    A_v_cache: jax.Array,
    A_wq: jax.Array,
    A_wo: jax.Array,
    B_x: jax.Array,
    B_w_r: jax.Array,
    B_w_gate: jax.Array,
    B_w_up: jax.Array,
    B_w_down: jax.Array,
    c: jax.Array,
    w_mod: jax.Array,
):
    del B_x
    vm = pltpu.VMEM
    scratch = [
        vm((S, D), BF16),
        vm((2, TQ // 2, D), U32),
        vm((H, S, DH), BF16),
        vm((H, S, DH), BF16),
        vm((H, D, DH), BF16),
        vm((H * DH, D), BF16),
        vm((D, FF), BF16),
        vm((D, FF), BF16),
        vm((FF, D), BF16),
        vm((D, 6 * D), BF16),
        vm((1, D), BF16),
        vm((1, D), BF16),
        vm((8, 6 * D), F32),
        vm((2, TQ, D), F32),
        vm((S, D), BF16),
        vm((TU, S), F32),
        vm((TU, DH), F32),
        vm((TU, DH), F32),
        vm((2, 8, 128), F32),
        pltpu.SemaphoreType.DMA((NSEM,)),
    ]
    anyspec = pl.BlockSpec(memory_space=pl.ANY)
    return pl.pallas_call(
        _kernel,
        in_specs=[anyspec] * 11,
        out_specs=anyspec,
        out_shape=jax.ShapeDtypeStruct((1, S, D), BF16),
        scratch_shapes=scratch,
        compiler_params=pltpu.CompilerParams(vmem_limit_bytes=120 * 1024 * 1024),
    )(A_x, A_k_cache, A_v_cache, A_wq, A_wo, B_w_r.reshape(1, D), B_w_gate, B_w_up, B_w_down, c, w_mod)
```

```python
import functools
import os

import jax
import jax.numpy as jnp
import jax.experimental.pallas as pl
import jax.experimental.pallas.tpu as pltpu

F32, BF16, U32, I32 = jnp.float32, jnp.bfloat16, jnp.uint32, jnp.int32

S, D, H, DH, FF = 2048, 1024, 32, 128, 3584
TU = 256
TQ = 512
NQ = S // TQ
HG = 4
NG = H // HG
NT = NQ * NG
SL = TQ // NG
PC = 16
RC = 16
WMC = 4
EPS = 1e-5
QSCALE = DH ** -0.5 * 1.4426950408889634
KMIN = -2 ** 31
SCOPES = int(os.environ.get('SCOPES', 0))
TPC = int(os.environ.get('TPC', 16))

SEM_SMALL = 0
SEM_X = 1
SEM_X1A = 5
SEM_WM = 6
SEM_WMR = 10
SEM_WQ0 = 11
SEM_KV0 = 12
SEM_MINI = 13
SEM_GRP = 17
SEM_FFN = 25
SEM_OUT = 26
SEM_FIX = 27
NSEM = 29


def _rb(x):
    return x.astype(BF16).astype(F32)


def _ub(x):
    return pltpu.bitcast(x, BF16)


def _pk(x):
    return pltpu.bitcast(x, U32)


def _recip(l):
    r = pl.reciprocal(l, approx=True)
    return r * (2.0 - l * r)


def _ln(x):
    mu = jnp.sum(x, axis=-1, keepdims=True) * (1.0 / D)
    d = x - mu
    var = jnp.sum(d * d, axis=-1, keepdims=True) * (1.0 / D)
    return d * jax.lax.rsqrt(var + EPS)


class _Scope:
    def __init__(self):
        self.cur = None

    def __call__(self, name):
        if not SCOPES:
            return
        if self.cur is not None:
            self.cur.__exit__(None, None, None)
            self.cur = None
        if name:
            self.cur = jax.named_scope(name)
            self.cur.__enter__()


def _kernel(x_hbm, k_hbm, v_hbm, wq_hbm, wo_hbm, wr_hbm, wg_hbm, wu_hbm, wd_hbm, c_hbm, wm_hbm,
            out_hbm,
            x_buf, h_buf, k_buf, v_buf, wq_buf, wo_buf, wg_buf, wu_buf, wd_buf, wm_buf,
            c_buf, wr_buf, mod_buf, acc, out_buf, s_sc, of_sc, l_sc, r_buf, sem):
    cp = pltpu.make_async_copy
    scope = _Scope()

    def d_small():
        return [cp(c_hbm, c_buf, sem.at[SEM_SMALL]), cp(wr_hbm, wr_buf, sem.at[SEM_SMALL])]

    def d_xrows(r0, n, s_):
        return [cp(x_hbm.at[0, pl.ds(r0, n), :], x_buf.at[pl.ds(r0, n), :], s_)]

    X1A = 128

    def d_x(j):
        if j == 1:
            return d_xrows(TQ + X1A, TQ - X1A, sem.at[SEM_X + 1])
        return d_xrows(j * TQ, TQ, sem.at[SEM_X + j])

    def d_x1a():
        return d_xrows(TQ, X1A, sem.at[SEM_X1A])

    WC = D // WMC

    def d_wm(i):
        return [cp(wm_hbm.at[:, pl.ds(b + i * WC, WC)], wm_buf.at[:, pl.ds(b + i * WC, WC)], sem.at[SEM_WM + i])
                for b in (0, D)]

    def d_wmr():
        return [cp(wm_hbm.at[:, pl.ds(2 * D, 4 * D)], wm_buf.at[:, pl.ds(2 * D, 4 * D)], sem.at[SEM_WMR])]

    def d_wq(h0, n, s_):
        return [cp(wq_hbm.at[:, pl.ds(pl.multiple_of((h0 + i) * DH, DH), DH)], wq_buf.at[h0 + i], s_)
                for i in range(n)]

    def d_k(h0, n, s_):
        return [cp(k_hbm.at[0, pl.ds(h0, n)], k_buf.at[pl.ds(h0, n)], s_)]

    def d_v(h0, n, s_):
        return [cp(v_hbm.at[0, pl.ds(h0, n)], v_buf.at[pl.ds(h0, n)], s_)]

    def d_wo(h0, n, s_):
        rows = pl.ds(pl.multiple_of(h0 * DH, DH), n * DH)
        return [cp(wo_hbm.at[rows, :], wo_buf.at[rows, :], s_)]

    def d_mini(i):
        s_ = sem.at[SEM_MINI + i]
        return d_wq(i, 1, s_) + d_wo(i - 1, 1, s_) + d_k(i, 1, s_) + d_v(i, 1, s_)

    def d_grp(t):
        s_ = sem.at[SEM_GRP + t]
        h0 = HG * t
        return d_wq(h0, HG, s_) + d_wo(h0 - 1, HG, s_) + d_k(h0, HG, s_) + d_v(h0, HG, s_)

    def d_late():
        return d_wmr() + d_wo(H - 1, 1, sem.at[SEM_WMR])

    def d_ffn(i):
        src, dst = ((wg_hbm, wg_buf), (wu_hbm, wu_buf), (wd_hbm, wd_buf.at[:, pl.ds(0, D)]))[i]
        return [cp(src, dst, sem.at[SEM_FFN])]

    def d_out(r0, n, s_):
        return [cp(out_buf.at[pl.ds(r0, n), :], out_hbm.at[0, pl.ds(r0, n), :], s_)]

    def start(ds):
        for d in ds:
            d.start()

    def wait(ds):
        for d in ds:
            d.wait()

    def qp(unit, anchor=False, zero=None):
        hh, sub, par = unit
        hb = h_buf[par, sub * (TU // 2):(sub + 1) * (TU // 2), :]
        if anchor:
            z16 = pl.multiple_of(zero * 16, 16)
            d0 = _pk(out_buf[pl.ds(z16, 16), 0:128])
            d1 = pltpu.bitcast(r_buf[zero], U32)
            d2 = _pk(x_buf[pl.ds(z16, 16), 0:128])
            top = jnp.concatenate([jnp.where(zero > 0, d0, hb[0:8, 0:128]),
                                   jnp.where(zero > 0, d1, hb[0:8, 128:256]),
                                   jnp.where(zero > 0, d2, hb[0:8, 256:384]), hb[0:8, 384:]], axis=1)
            hb = jnp.concatenate([top, hb[8:]], axis=0)
        q = jnp.dot(_ub(hb), wq_buf[hh], preferred_element_type=F32)
        return (q * QSCALE).astype(BF16)

    def qk(unit, q):
        hh, sub, par = unit
        return jax.lax.dot_general(q, k_buf[hh], (((1,), (1,)), ((), ())), preferred_element_type=F32)

    def pv(unit, s, zero):
        hh, sub, par = unit
        ls, ps = [], []
        nc = S // 128
        for c in range(TU // RC):
            sc = s[c * RC:(c + 1) * RC, :]
            m = jnp.max(sc, axis=-1, keepdims=True)
            p = jnp.exp2(sc - m)
            cols = [p[:, i * 128:(i + 1) * 128] for i in range(nc)]
            a = cols[0]
            for i in range(1, nc):
                if i == nc - 4:
                    part = a
                a = a + cols[i]
            cols[nc - 4] = jnp.where(zero > 0, part, cols[nc - 4])
            ls.append(a)
            ps.append(jnp.concatenate(cols, axis=1))
        o = jnp.dot(jnp.concatenate(ps, axis=0).astype(BF16), v_buf[hh], preferred_element_type=F32)
        return o, jnp.concatenate(ls, axis=0)

    def outp(unit, ol):
        hh, sub, par = unit
        of, lp = ol
        l = jnp.sum(lp, axis=-1, keepdims=True)
        o = (of * _recip(l)).astype(BF16)
        w = wo_buf[pl.ds(pl.multiple_of(hh * DH, DH), DH), :]
        acc[par, sub * TU:(sub + 1) * TU, :] += jnp.dot(o, w, preferred_element_type=F32)

    def modrow(i):
        return mod_buf[:, i * D:(i + 1) * D][None]

    def ln1(xrow0, par, hrow0, n, zero):
        x = x_buf[pl.ds(xrow0, n), :].astype(F32)
        d = acc[zero, pl.ds(pl.multiple_of(zero * 8, 8), n), 0:128]
        x = jnp.concatenate([jnp.where(zero > 0, d, x[:, 0:128]), x[:, 128:]], axis=1)
        h = (_ln(x.reshape(n // 8, 8, D)) * modrow(1) + modrow(0)).reshape(n, D)
        h_buf[par, pl.ds(hrow0, n // 2), :] = _pk(h.astype(BF16))

    def epi(row0, par, arow0, n, valid):
        a = acc[par, pl.ds(arow0, n), :].reshape(n // 8, 8, D)
        if valid is not None:
            acc[par, pl.ds(arow0, n), :] = jnp.zeros((n, D), F32)
        x1 = x_buf[pl.ds(row0, n), :].astype(F32).reshape(n // 8, 8, D) + modrow(2) * a
        h2 = _ln(x1) * modrow(4) + modrow(3)
        wrow = row0 if valid is None else pl.multiple_of(jnp.where(valid, row0, S), n)
        x_buf[pl.ds(wrow, n), :] = h2.reshape(n, D).astype(BF16)
        out_buf[pl.ds(row0, n), :] = (x1 + modrow(5) * h2).reshape(n, D).astype(BF16)
        r = jnp.sum(h2 * modrow(6), axis=-1, keepdims=True)
        b = pltpu.bitcast(jnp.broadcast_to(r, (n // 8, 8, 128)), I32)
        key = (b ^ ((b >> 31) & 0x7FFFFFFF)) | (S - 1)
        rid = jax.lax.broadcasted_iota(I32, (8, 128), 0) + row0
        best, second = r_buf[0], r_buf[1]
        for i in range(n // 8):
            k = key[i] - (rid + 8 * i)
            if valid is not None:
                k = jnp.where(valid, k, KMIN)
            second = jnp.maximum(second, jnp.minimum(best, k))
            best = jnp.maximum(best, k)
        r_buf[0] = best
        r_buf[1] = second

    def run_units(seq, side, zero):
        s = s_sc[...]
        ol_prev = (of_sc[...], l_sc[...])
        for u in range(len(seq) - 2):
            q = qp(seq[u + 2], u - 1 in side and side[u - 1][1], zero)
            ol = pv(seq[u + 1], s, zero)
            outp(seq[u], ol_prev)
            ol_prev = ol
            if u in side:
                side[u][0]()
            s = qk(seq[u + 2], q)
        s_sc[...] = s
        of_sc[...] = ol_prev[0]
        l_sc[...] = ol_prev[1]

    def mod_cols(c0, n):
        cf = c_buf[...].astype(F32)
        sc = (cf * jax.nn.sigmoid(cf)).astype(BF16)
        sc = jnp.broadcast_to(sc, (16, D))
        m = jnp.dot(sc, wm_buf[:, c0:c0 + n], preferred_element_type=F32)
        return _rb(m[0:8, :])

    start(d_small())
    start(d_x(0))
    for i in range(WMC):
        start(d_wm(i))
    start(d_wq(0, 1, sem.at[SEM_WQ0]))
    start(d_k(0, 1, sem.at[SEM_KV0]) + d_v(0, 1, sem.at[SEM_KV0]))
    start(d_mini(1))
    start(d_x1a())
    start(d_mini(2))
    start(d_mini(3))
    start(d_grp(1))
    start(d_x(1))
    start(d_grp(2))

    scope('p_init')
    acc[...] = jnp.zeros(acc.shape, F32)
    mod_buf[...] = jnp.zeros(mod_buf.shape, F32)
    r_buf[...] = jnp.full(r_buf.shape, KMIN, I32)
    out_buf[0:16, :] = jnp.zeros((16, D), BF16)

    wait(d_small())
    wr = wr_buf[...].astype(F32)
    for i in range(8):
        mod_buf[:, 6 * D + i * 128:6 * D + (i + 1) * 128] = jnp.broadcast_to(wr[i:i + 1, :], (8, 128))
    scope('p_ln')
    wait(d_x(0))

    def norm_first(i, _):
        for half in range(2):
            r0 = pl.multiple_of(i * 32, 32)
            x = x_buf[pl.ds(half * TU + r0, 32), :].astype(F32)
            s_sc[pl.ds(r0, 32), half * D:(half + 1) * D] = _ln(x)
        return 0
    jax.lax.fori_loop(0, TU // 32, norm_first, 0)

    scope('p_mod')
    for i in range(WMC):
        wait(d_wm(i))
        sa = mod_cols(i * WC, WC)
        ca = _rb(1.0 + mod_cols(D + i * WC, WC))
        mod_buf[:, i * WC:(i + 1) * WC] = sa
        mod_buf[:, D + i * WC:D + (i + 1) * WC] = ca
        for half in range(2):
            n = s_sc[:, half * D + i * WC:half * D + (i + 1) * WC].reshape(TU // 8, 8, WC)
            h = (n * ca[None] + sa[None]).reshape(TU, WC)
            h_buf[0, half * (TU // 2):(half + 1) * (TU // 2), i * WC:(i + 1) * WC] = _pk(h.astype(BF16))

    scope('p_b1')
    wait(d_wq(0, 1, sem.at[SEM_WQ0]))
    q0 = qp((0, 0, 0))
    q1 = qp((0, 1, 0))
    scope('p_b2')
    wait(d_k(0, 1, sem.at[SEM_KV0]) + d_v(0, 1, sem.at[SEM_KV0]))
    zero0 = r_buf[0, 0, 0] & 1
    s0 = qk((0, 0, 0), q0)
    s_sc[...] = qk((0, 1, 0), q1)
    o0, l0 = pv((0, 0, 0), s0, zero0)
    of_sc[...] = o0
    l_sc[...] = l0
    scope('p_x1a')
    wait(d_x1a())
    scope(None)

    def mini(i, _):
        scope('mini_wait')
        wait(d_mini(i))
        scope(None)
        zero = i >> 10
        side = {}
        for u in range(2):
            r0 = ((i - 1) * 2 + u) * PC
            side[u] = (functools.partial(ln1, pl.multiple_of(TQ + r0, PC), 1,
                                         pl.multiple_of(r0 // 2, PC // 2), PC, zero), False)
        run_units([(i - 1, 0, 0), (i - 1, 1, 0), (i, 0, 0), (i, 1, 0)], side, zero)
        return 0
    jax.lax.fori_loop(1, HG, mini, 0)
    for t in range(3, NG):
        start(d_grp(t))
    start(d_late())
    start(d_x(2))
    start(d_x(3))
    for i in range(3):
        start(d_ffn(i))

    def main(t, _):
        j = t >> 3
        g = t & (NG - 1)

        @pl.when(t < NG)
        def _():
            scope('grp_wait')
            wait(d_grp(t))
            scope(None)

        @pl.when(t == 2)
        def _():
            wait(d_x(1))

        @pl.when(t == NG)
        def _():
            scope('modrest')
            wait(d_late())
            wait(d_x(2))
            wait(d_x(3))
            for i in range(3):
                wait(d_ffn(i))
            for i in range(2, 6):
                m = mod_cols(i * D, D)
                if i == 4:
                    m = _rb(1.0 + m)
                mod_buf[:, i * D:(i + 1) * D] = m
            scope(None)

        @pl.when(t > NG)
        def _():
            start(d_out(pl.multiple_of((t - 1 - NG) * SL, SL), SL, sem.at[SEM_OUT]))

        par = j & 1
        tp = t - 1
        hp = (tp & (NG - 1)) * HG + HG - 1
        pp = (tp >> 3) & 1
        seq = [(hp, 0, pp), (hp, 1, pp)] + [(g * HG + (u >> 1), u & 1, par) for u in range(2 * HG)]
        jn = jnp.minimum(j + 1, NQ - 1)
        jp = jnp.maximum(j - 1, 0)
        zero = t >> 10
        side = {}
        for i in range(SL // PC):
            r0 = g * SL + i * PC
            side[2 * i] = (functools.partial(
                epi, pl.multiple_of(jp * TQ + r0, PC), 1 - par, pl.multiple_of(r0, PC), PC, j > 0), True)
            side[2 * i + 1] = (functools.partial(
                ln1, pl.multiple_of(jn * TQ + r0, PC), 1 - par, pl.multiple_of(r0 // 2, PC // 2), PC, zero), False)
        run_units(seq, side, zero)
        return 0
    jax.lax.fori_loop(1, NT, main, 0)

    scope('t_epi')
    start(d_out((NT - 1 - NG) * SL, SL, sem.at[SEM_OUT]))
    lastp = (NQ - 1) & 1
    base = (NQ - 1) * TQ
    outp((H - 1, 0, lastp), (of_sc[...], l_sc[...]))
    ol = pv((H - 1, 1, lastp), s_sc[...], zero0)
    for i in range(TU // TPC):
        epi(base + i * TPC, lastp, i * TPC, TPC, None)
    start(d_out(base, TU, sem.at[SEM_OUT]))
    outp((H - 1, 1, lastp), ol)
    for i in range(TU // TPC, TQ // TPC):
        epi(base + i * TPC, lastp, i * TPC, TPC, None)
    start(d_out(base + TU, TU, sem.at[SEM_OUT]))

    scope('t_ffn')
    best, second = r_buf[0], r_buf[1]
    for sh in (4, 2, 1):
        b2 = pltpu.roll(best, sh, 0)
        s2 = pltpu.roll(second, sh, 0)
        second = jnp.maximum(jnp.minimum(best, b2), jnp.maximum(second, s2))
        best = jnp.maximum(best, b2)
    i1 = (S - 1) - (best[0, 0] & (S - 1))
    i2 = (S - 1) - (second[0, 0] & (S - 1))
    g1 = pl.multiple_of((i1 >> 3) << 3, 8)
    g2 = pl.multiple_of((i2 >> 3) << 3, 8)

    xs = jnp.concatenate([x_buf[pl.ds(g1, 8), :], x_buf[pl.ds(g2, 8), :]], axis=0)
    gt = _rb(jnp.dot(xs, wg_buf[...], preferred_element_type=F32))
    up = _rb(jnp.dot(xs, wu_buf[...], preferred_element_type=F32))
    a = (_rb(gt * jax.nn.sigmoid(gt)) * up).astype(BF16)
    y = _rb(jnp.dot(a, wd_buf[:, 0:D], preferred_element_type=F32))

    def score(k):
        return pltpu.bitcast(k ^ ((k >> 31) & 0x7FFFFFFF), F32)
    ri = jax.lax.broadcasted_iota(I32, (16, 128), 0)
    rows = jnp.where(ri < 8, g1 + ri, g2 + ri - 8)
    r1 = jnp.concatenate([score(best)] * 2, axis=0)
    r2 = jnp.concatenate([score(second)] * 2, axis=0)
    gate = _rb(jax.nn.sigmoid(_rb(jnp.where(rows == i1, r1, r2))))
    sel = (rows == i1) | (rows == i2)
    upd = jnp.where(sel[:, 0:1], _rb(y * gate[:, 0:1]), 0.0) * mod_buf[0:1, 5 * D:6 * D]
    o1 = (out_buf[pl.ds(g1, 8), :].astype(F32) + upd[0:8]).astype(BF16)
    o2 = (out_buf[pl.ds(g2, 8), :].astype(F32) + upd[8:16]).astype(BF16)

    scope('t_fix')
    cp(out_buf, out_hbm.at[0], sem.at[SEM_OUT]).wait()
    out_buf[pl.ds(g1, 8), :] = o1
    out_buf[pl.ds(g2, 8), :] = o2
    start(d_out(g1, 8, sem.at[SEM_FIX]))

    @pl.when(g1 != g2)
    def _():
        start(d_out(g2, 8, sem.at[SEM_FIX + 1]))
        wait(d_out(g2, 8, sem.at[SEM_FIX + 1]))

    wait(d_out(g1, 8, sem.at[SEM_FIX]))
    scope(None)


@jax.jit
def pallas_adaLN_cond__mha_block_cached__moe_arch_mod__prompt_kernel(
    A_x: jax.Array,
    A_k_cache: jax.Array,
    A_v_cache: jax.Array,
    A_wq: jax.Array,
    A_wo: jax.Array,
    B_x: jax.Array,
    B_w_r: jax.Array,
    B_w_gate: jax.Array,
    B_w_up: jax.Array,
    B_w_down: jax.Array,
    c: jax.Array,
    w_mod: jax.Array,
):
    del B_x
    vm = pltpu.VMEM
    scratch = [
        vm((S + PC, D), BF16),
        vm((2, TQ // 2, D), U32),
        vm((H, S, DH), BF16),
        vm((H, S, DH), BF16),
        vm((H, D, DH), BF16),
        vm((H * DH, D), BF16),
        vm((D, FF), BF16),
        vm((D, FF), BF16),
        vm((FF, D + 128), BF16),
        vm((D, 6 * D + 128), BF16),
        vm((1, D), BF16),
        vm((8, 128), BF16),
        vm((8, 7 * D), F32),
        vm((2, TQ, D), F32),
        vm((S, D), BF16),
        vm((TU, S), F32),
        vm((TU, DH), F32),
        vm((TU, DH), F32),
        vm((2, 8, 128), I32),
        pltpu.SemaphoreType.DMA((NSEM,)),
    ]
    anyspec = pl.BlockSpec(memory_space=pl.ANY)
    return pl.pallas_call(
        _kernel,
        in_specs=[anyspec] * 11,
        out_specs=anyspec,
        out_shape=jax.ShapeDtypeStruct((1, S, D), BF16),
        scratch_shapes=scratch,
        compiler_params=pltpu.CompilerParams(vmem_limit_bytes=120 * 1024 * 1024, disable_bounds_checks=True),
    )(A_x, A_k_cache, A_v_cache, A_wq, A_wo, B_w_r.reshape(8, 128), B_w_gate, B_w_up, B_w_down, c, w_mod)
```

```python
import functools
import os

import jax
import jax.numpy as jnp
import jax.experimental.pallas as pl
import jax.experimental.pallas.tpu as pltpu

F32, BF16, U32, I32 = jnp.float32, jnp.bfloat16, jnp.uint32, jnp.int32

S, D, H, DH, FF = 2048, 1024, 32, 128, 3584
TU = 256
TQ = 512
NQ = S // TQ
HG = int(os.environ.get('HG', 4))
NG = H // HG
LG = NG.bit_length() - 1
NT = NQ * NG
SL = TQ // NG
PC = 16
RC = int(os.environ.get('RC', 16))
AC = int(os.environ.get('AC', 4))
SORD = int(os.environ.get('SORD', 0))
EPC = int(os.environ.get('EPC', 16))
QANCH = int(os.environ.get('QANCH', 1))
WMC = 4
EPS = 1e-5
QSCALE = DH ** -0.5 * 1.4426950408889634
KMIN = -2 ** 31
SCOPES = int(os.environ.get('SCOPES', 0))
TV = int(os.environ.get('TV', 2))
CPC = int(os.environ.get('CPC', 16))
CSPAN = int(os.environ.get('CSPAN', 40))
RFORM = int(os.environ.get('RFORM', 0))
CBAR = int(os.environ.get('CBAR', 0))
TPC = int(os.environ.get('TPC', 64))

SEM_SMALL = 0
SEM_X = 1
SEM_X1A = 5
SEM_WM = 6
SEM_WMR = 10
SEM_WQ0 = 11
SEM_KV0 = 12
SEM_FFN = 13
SEM_OUT = 14
SEM_FIX = 15
SEM_OUT2 = 17
SEM_MINI = 18
SEM_GRP = SEM_MINI + HG
NSEM = SEM_GRP + NG


def _rb(x):
    return x.astype(BF16).astype(F32)


def _ub(x):
    return pltpu.bitcast(x, BF16)


def _pk(x):
    return pltpu.bitcast(x, U32)


def _recip(l):
    r = pl.reciprocal(l, approx=True)
    return r * (2.0 - l * r)


def _ln(x):
    mu = jnp.sum(x, axis=-1, keepdims=True) * (1.0 / D)
    d = x - mu
    var = jnp.sum(d * d, axis=-1, keepdims=True) * (1.0 / D)
    return d * jax.lax.rsqrt(var + EPS)


class _Scope:
    def __init__(self):
        self.cur = None

    def __call__(self, name):
        if not SCOPES:
            return
        if self.cur is not None:
            self.cur.__exit__(None, None, None)
            self.cur = None
        if name:
            self.cur = jax.named_scope(name)
            self.cur.__enter__()


def _kernel(x_hbm, k_hbm, v_hbm, wq_hbm, wo_hbm, wr_hbm, wg_hbm, wu_hbm, wd_hbm, c_hbm, wm_hbm,
            out_hbm,
            x_buf, h_buf, k_buf, v_buf, wq_buf, wo_buf, wg_buf, wu_buf, wd_buf, wm_buf,
            c_buf, wr_buf, mod_buf, acc, out_buf, s_sc, of_sc, l_sc, r_buf, st_buf, sem):
    cp = pltpu.make_async_copy
    scope = _Scope()

    def d_small():
        return [cp(c_hbm, c_buf, sem.at[SEM_SMALL]), cp(wr_hbm, wr_buf, sem.at[SEM_SMALL])]

    def d_xrows(r0, n, s_):
        return [cp(x_hbm.at[0, pl.ds(r0, n), :], x_buf.at[pl.ds(r0, n), :], s_)]

    X1A = 2 * SL

    def d_x(j):
        if j == 1:
            return d_xrows(TQ + X1A, TQ - X1A, sem.at[SEM_X + 1])
        return d_xrows(j * TQ, TQ, sem.at[SEM_X + j])

    def d_x1a():
        return d_xrows(TQ, X1A, sem.at[SEM_X1A])

    WC = D // WMC

    def d_wm(i):
        return [cp(wm_hbm.at[:, pl.ds(b + i * WC, WC)], wm_buf.at[:, pl.ds(b + i * WC, WC)], sem.at[SEM_WM + i])
                for b in (0, D)]

    def d_wmr():
        return [cp(wm_hbm.at[:, pl.ds(2 * D, 4 * D)], wm_buf.at[:, pl.ds(2 * D, 4 * D)], sem.at[SEM_WMR])]

    def d_wq(h0, n, s_):
        return [cp(wq_hbm.at[:, pl.ds(pl.multiple_of((h0 + i) * DH, DH), DH)], wq_buf.at[h0 + i], s_)
                for i in range(n)]

    def d_k(h0, n, s_):
        return [cp(k_hbm.at[0, pl.ds(h0, n)], k_buf.at[pl.ds(h0, n)], s_)]

    def d_v(h0, n, s_):
        return [cp(v_hbm.at[0, pl.ds(h0, n)], v_buf.at[pl.ds(h0, n)], s_)]

    def d_wo(h0, n, s_):
        rows = pl.ds(pl.multiple_of(h0 * DH, DH), n * DH)
        return [cp(wo_hbm.at[rows, :], wo_buf.at[rows, :], s_)]

    def d_mini(i):
        s_ = sem.at[SEM_MINI + i]
        return d_wq(i, 1, s_) + d_wo(i - 1, 1, s_) + d_k(i, 1, s_) + d_v(i, 1, s_)

    def d_grp(t):
        s_ = sem.at[SEM_GRP + t]
        h0 = HG * t
        return d_wq(h0, HG, s_) + d_wo(h0 - 1, HG, s_) + d_k(h0, HG, s_) + d_v(h0, HG, s_)

    def d_late():
        return d_wmr() + d_wo(H - 1, 1, sem.at[SEM_WMR])

    def d_ffn(i):
        src, dst = ((wg_hbm, wg_buf), (wu_hbm, wu_buf), (wd_hbm, wd_buf.at[:, pl.ds(0, D)]))[i]
        return [cp(src, dst, sem.at[SEM_FFN])]

    def d_out(r0, n, s_):
        return [cp(out_buf.at[pl.ds(r0, n), :], out_hbm.at[0, pl.ds(r0, n), :], s_)]

    def start(ds):
        for d in ds:
            d.start()

    def wait(ds):
        for d in ds:
            d.wait()

    def qp(unit, anchor=False, zero=None):
        hh, sub, par = unit
        hb = h_buf[par, sub * (TU // 2):(sub + 1) * (TU // 2), :]
        if anchor:
            z16 = pl.multiple_of(zero * 16, 16)
            d0 = _pk(out_buf[pl.ds(z16, 16), 0:128])
            d1 = pltpu.bitcast(r_buf[zero], U32)
            d2 = _pk(x_buf[pl.ds(z16, 16), 0:128])
            top = jnp.concatenate([jnp.where(zero > 0, d0, hb[0:8, 0:128]),
                                   jnp.where(zero > 0, d1, hb[0:8, 128:256]),
                                   jnp.where(zero > 0, d2, hb[0:8, 256:384]), hb[0:8, 384:]], axis=1)
            hb = jnp.concatenate([top, hb[8:]], axis=0)
        q = jnp.dot(_ub(hb), wq_buf[hh], preferred_element_type=F32)
        return (q * QSCALE).astype(BF16)

    def qk(unit, q):
        hh, sub, par = unit
        return jax.lax.dot_general(q, k_buf[hh], (((1,), (1,)), ((), ())), preferred_element_type=F32)

    def pv(unit, s, zero):
        hh, sub, par = unit
        ls, ps = [], []
        nc = S // 128
        for c in range(TU // RC):
            sc = s[c * RC:(c + 1) * RC, :]
            m = jnp.max(sc, axis=-1, keepdims=True)
            p = jnp.exp2(sc - m)
            cols = [p[:, i * 128:(i + 1) * 128] for i in range(nc)]
            a = cols[0]
            for i in range(1, nc):
                if i == nc - AC:
                    part = a
                a = a + cols[i]
            cols[nc - AC] = jnp.where(zero > 0, part, cols[nc - AC])
            ls.append(a)
            ps.append(jnp.concatenate(cols, axis=1))
        o = jnp.dot(jnp.concatenate(ps, axis=0).astype(BF16), v_buf[hh], preferred_element_type=F32)
        return o, jnp.concatenate(ls, axis=0)

    def outp(unit, ol):
        hh, sub, par = unit
        of, lp = ol
        l = jnp.sum(lp, axis=-1, keepdims=True)
        o = (of * _recip(l)).astype(BF16)
        w = wo_buf[pl.ds(pl.multiple_of(hh * DH, DH), DH), :]
        acc[par, sub * TU:(sub + 1) * TU, :] += jnp.dot(o, w, preferred_element_type=F32)

    def modrow(i):
        return mod_buf[:, i * D:(i + 1) * D][None]

    def ln1(xrow0, par, hrow0, n, zero):
        x = x_buf[pl.ds(xrow0, n), :].astype(F32)
        d = acc[zero, pl.ds(pl.multiple_of(zero * 8, 8), n), 0:128]
        x = jnp.concatenate([jnp.where(zero > 0, d, x[:, 0:128]), x[:, 128:]], axis=1)
        h = (_ln(x.reshape(n // 8, 8, D)) * modrow(1) + modrow(0)).reshape(n, D)
        h_buf[par, pl.ds(hrow0, n // 2), :] = _pk(h.astype(BF16))

    def top2_update(r, row0, valid):
        b = pltpu.bitcast(r, I32)
        key = (b ^ ((b >> 31) & 0x7FFFFFFF)) | (S - 1)
        rid = jax.lax.broadcasted_iota(I32, (8, 128), 0) + row0
        best, second = r_buf[0], r_buf[1]
        for i in range(r.shape[0]):
            k = key[i] - (rid + 8 * i)
            if valid is not None:
                k = jnp.where(valid, k, KMIN)
            second = jnp.maximum(second, jnp.minimum(best, k))
            best = jnp.maximum(best, k)
        r_buf[0] = best
        r_buf[1] = second

    def rconst(i):
        return mod_buf[:, 7 * D + i * 128:7 * D + (i + 1) * 128][None]

    def epi(row0, par, arow0, n, valid):
        a = acc[par, pl.ds(arow0, n), :].reshape(n // 8, 8, D)
        acc[par, pl.ds(arow0, n), :] = jnp.zeros((n, D), F32)
        x1 = x_buf[pl.ds(row0, n), :].astype(F32).reshape(n // 8, 8, D) + modrow(2) * a
        d = x1 - jnp.sum(x1, axis=-1, keepdims=True) * (1.0 / D)
        rstd = jax.lax.rsqrt(jnp.sum(d * d, axis=-1, keepdims=True) * (1.0 / D) + EPS)
        h2 = d * rstd * modrow(4) + modrow(3)
        x_buf[pl.ds(pl.multiple_of(jnp.where(valid, row0, S), n), n), :] = h2.reshape(n, D).astype(BF16)
        out_buf[pl.ds(row0, n), :] = (x1 + modrow(5) * h2).reshape(n, D).astype(BF16)
        if RFORM:
            top2_update(jnp.sum(d * modrow(6), axis=-1, keepdims=True) * rstd + rconst(0), row0, valid)
        else:
            r = jnp.sum(h2 * mod_buf[:, 7 * D + 256:8 * D + 256][None], axis=-1, keepdims=True)
            top2_update(jnp.broadcast_to(r, (n // 8, 8, 128)), row0, valid)

    def epi_a(row0, par, arow0, n):
        a = acc[par, arow0:arow0 + n, :].reshape(n // 8, 8, D)
        x1 = x_buf[row0:row0 + n, :].astype(F32).reshape(n // 8, 8, D) + modrow(2) * a
        acc[par, arow0:arow0 + n, :] = x1.reshape(n, D)
        mu = jnp.sum(x1, axis=-1, keepdims=True) * (1.0 / D)
        var = jnp.maximum(jnp.sum(x1 * x1, axis=-1, keepdims=True) * (1.0 / D) - mu * mu, 0.0)
        rstd = jnp.broadcast_to(jax.lax.rsqrt(var + EPS), (n // 8, 8, 128))
        mu = jnp.broadcast_to(mu, (n // 8, 8, 128))
        st_buf[0, arow0:arow0 + n, :] = mu.reshape(n, 128)
        st_buf[1, arow0:arow0 + n, :] = rstd.reshape(n, 128)
        xu = jnp.sum(x1 * modrow(6), axis=-1, keepdims=True)
        top2_update((xu - mu * rconst(1)) * rstd + rconst(0), row0, None)

    def last_norm(par, arow0, n):
        x1 = acc[par, pl.ds(arow0, n), :].reshape(n // 8, 8, D)
        mu = jnp.concatenate([st_buf[0, pl.ds(arow0, n), :]] * 8, axis=1).reshape(n // 8, 8, D)
        rstd = jnp.concatenate([st_buf[1, pl.ds(arow0, n), :]] * 8, axis=1).reshape(n // 8, 8, D)
        return x1, (x1 - mu) * rstd

    def run_units(seq, side, zero):
        s = s_sc[...]
        ol_prev = (of_sc[...], l_sc[...])
        for u in range(len(seq) - 2):
            q = qp(seq[u + 2], u - 1 in side and side[u - 1][1], zero)
            ol = pv(seq[u + 1], s, zero)
            outp(seq[u], ol_prev)
            ol_prev = ol
            if u in side:
                side[u][0]()
            s = qk(seq[u + 2], q)
        s_sc[...] = s
        of_sc[...] = ol_prev[0]
        l_sc[...] = ol_prev[1]

    def mod_cols(c0, n):
        cf = c_buf[...].astype(F32)
        sc = (cf * jax.nn.sigmoid(cf)).astype(BF16)
        sc = jnp.broadcast_to(sc, (16, D))
        m = jnp.dot(sc, wm_buf[:, c0:c0 + n], preferred_element_type=F32)
        return _rb(m[0:8, :])

    start(d_small())
    start(d_x(0))
    for i in range(WMC):
        start(d_wm(i))
    start(d_wq(0, 1, sem.at[SEM_WQ0]))
    start(d_k(0, 1, sem.at[SEM_KV0]) + d_v(0, 1, sem.at[SEM_KV0]))
    start(d_mini(1))
    start(d_x1a())
    for i in range(2, HG):
        start(d_mini(i))
    start(d_grp(1))
    start(d_x(1))
    if HG == 4:
        start(d_grp(2))

    scope('p_init')
    acc[...] = jnp.zeros(acc.shape, F32)
    mod_buf[...] = jnp.zeros(mod_buf.shape, F32)
    r_buf[...] = jnp.full(r_buf.shape, KMIN, I32)
    out_buf[0:16, :] = jnp.zeros((16, D), BF16)

    wait(d_small())
    wr = wr_buf[...].astype(F32)
    for i in range(8):
        mod_buf[:, 6 * D + i * 128:6 * D + (i + 1) * 128] = jnp.broadcast_to(wr[i:i + 1, :], (8, 128))
    scope('p_ln')
    wait(d_x(0))

    def norm_first(i, _):
        for half in range(2):
            r0 = pl.multiple_of(i * 32, 32)
            x = x_buf[pl.ds(half * TU + r0, 32), :].astype(F32)
            s_sc[pl.ds(r0, 32), half * D:(half + 1) * D] = _ln(x)
        return 0
    jax.lax.fori_loop(0, TU // 32, norm_first, 0)

    scope('p_mod')
    for i in range(WMC):
        wait(d_wm(i))
        sa = mod_cols(i * WC, WC)
        ca = _rb(1.0 + mod_cols(D + i * WC, WC))
        mod_buf[:, i * WC:(i + 1) * WC] = sa
        mod_buf[:, D + i * WC:D + (i + 1) * WC] = ca
        for half in range(2):
            n = s_sc[:, half * D + i * WC:half * D + (i + 1) * WC].reshape(TU // 8, 8, WC)
            h = (n * ca[None] + sa[None]).reshape(TU, WC)
            h_buf[0, half * (TU // 2):(half + 1) * (TU // 2), i * WC:(i + 1) * WC] = _pk(h.astype(BF16))

    scope('p_b1')
    wait(d_wq(0, 1, sem.at[SEM_WQ0]))
    q0 = qp((0, 0, 0))
    q1 = qp((0, 1, 0))
    scope('p_b2')
    wait(d_k(0, 1, sem.at[SEM_KV0]) + d_v(0, 1, sem.at[SEM_KV0]))
    zero0 = r_buf[0, 0, 0] & 1
    s0 = qk((0, 0, 0), q0)
    s_sc[...] = qk((0, 1, 0), q1)
    o0, l0 = pv((0, 0, 0), s0, zero0)
    of_sc[...] = o0
    l_sc[...] = l0
    scope('p_x1a')
    wait(d_x1a())
    scope(None)

    def mini(i, _):
        scope('mini_wait')
        wait(d_mini(i))
        scope(None)
        zero = i >> 10
        side = {}
        for u in range(2):
            r0 = ((i - 1) * 2 + u) * PC
            side[u] = (functools.partial(ln1, pl.multiple_of(TQ + r0, PC), 1,
                                         pl.multiple_of(r0 // 2, PC // 2), PC, zero), False)
        run_units([(i - 1, 0, 0), (i - 1, 1, 0), (i, 0, 0), (i, 1, 0)], side, zero)
        return 0
    jax.lax.fori_loop(1, HG, mini, 0)
    for t in range(3 if HG == 4 else 2, NG):
        start(d_grp(t))
    start(d_late())
    start(d_x(2))
    start(d_x(3))
    for i in range(3):
        start(d_ffn(i))

    def main(t, _):
        j = t >> LG
        g = t & (NG - 1)

        @pl.when(t < NG)
        def _():
            scope('grp_wait')
            wait(d_grp(t))
            scope(None)

        @pl.when(t == 2)
        def _():
            wait(d_x(1))

        @pl.when(t == NG)
        def _():
            scope('modrest')
            wait(d_late())
            wait(d_x(2))
            wait(d_x(3))
            for i in range(3):
                wait(d_ffn(i))
            for i in range(2, 6):
                m = mod_cols(i * D, D)
                if i == 4:
                    m = _rb(1.0 + m)
                mod_buf[:, i * D:(i + 1) * D] = m
            wr = mod_buf[:, 6 * D:7 * D]
            u = mod_buf[:, 4 * D:5 * D] * wr
            mod_buf[:, 6 * D:7 * D] = u
            mod_buf[:, 7 * D + 256:8 * D + 256] = wr
            mod_buf[:, 7 * D:7 * D + 128] = jnp.broadcast_to(
                jnp.sum(mod_buf[:, 3 * D:4 * D] * wr, axis=-1, keepdims=True), (8, 128))
            mod_buf[:, 7 * D + 128:7 * D + 256] = jnp.broadcast_to(jnp.sum(u, axis=-1, keepdims=True), (8, 128))
            scope(None)

        @pl.when(t > NG)
        def _():
            start(d_out(pl.multiple_of((t - 1 - NG) * SL, SL), SL, sem.at[SEM_OUT]))

        par = j & 1
        tp = t - 1
        hp = (tp & (NG - 1)) * HG + HG - 1
        pp = (tp >> LG) & 1
        seq = [(hp, 0, pp), (hp, 1, pp)] + [(g * HG + (u >> 1), u & 1, par) for u in range(2 * HG)]
        jn = jnp.minimum(j + 1, NQ - 1)
        jp = jnp.maximum(j - 1, 0)
        zero = t >> 10
        side = {}
        def e_(r0, n):
            return functools.partial(epi, pl.multiple_of(jp * TQ + r0, n), 1 - par, pl.multiple_of(r0, n), n, j > 0)
        def l_(r0):
            return functools.partial(
                ln1, pl.multiple_of(jn * TQ + r0, PC), 1 - par, pl.multiple_of(r0 // 2, PC // 2), PC, zero)
        def both(a, b):
            def f():
                a()
                b()
            return f
        for i in range(SL // PC):
            r0 = g * SL + i * PC
            if EPC == PC:
                side[2 * i + SORD] = (e_(r0, PC), bool(QANCH))
                side[2 * i + 1 - SORD] = (l_(r0), False)
            else:
                side[2 * i + SORD] = (e_(r0 + SORD * 8, 8), bool(QANCH))
                side[2 * i + 1 - SORD] = (both(e_(r0 + (1 - SORD) * 8, 8), l_(r0)), bool(QANCH))
        run_units(seq, side, zero)
        return 0
    jax.lax.fori_loop(1, NT, main, 0)

    scope('t_epi')
    start(d_out((NT - 1 - NG) * SL, SL, sem.at[SEM_OUT]))
    lastp = (NQ - 1) & 1
    base = (NQ - 1) * TQ
    def epis(half):
        for i in range(half * TU // TPC, (half + 1) * TU // TPC):
            epi_a(base + i * TPC, lastp, i * TPC, TPC)
    if TV == 0:
        outp((H - 1, 0, lastp), (of_sc[...], l_sc[...]))
        ol = pv((H - 1, 1, lastp), s_sc[...], zero0)
        epis(0)
        outp((H - 1, 1, lastp), ol)
        epis(1)
    elif TV == 2:
        ol = pv((H - 1, 1, lastp), s_sc[...], zero0)
        outp((H - 1, 0, lastp), (of_sc[...], l_sc[...]))
        outp((H - 1, 1, lastp), ol)
        epis(0)
        epis(1)

    scope('t_ffn')
    best, second = r_buf[0], r_buf[1]
    for sh in (4, 2, 1):
        b2 = pltpu.roll(best, sh, 0)
        s2 = pltpu.roll(second, sh, 0)
        second = jnp.maximum(jnp.minimum(best, b2), jnp.maximum(second, s2))
        best = jnp.maximum(best, b2)
    i1 = (S - 1) - (best[0, 0] & (S - 1))
    i2 = (S - 1) - (second[0, 0] & (S - 1))
    g1 = pl.multiple_of((i1 >> 3) << 3, 8)
    g2 = pl.multiple_of((i2 >> 3) << 3, 8)

    def h2_rows(g):
        nrm = last_norm(lastp, pl.multiple_of(jnp.maximum(g - base, 0), 8), 8)[1]
        last = (nrm * modrow(4) + modrow(3)).reshape(8, D)
        return jnp.where(g >= base, last, x_buf[pl.ds(g, 8), :].astype(F32))
    xs = jnp.concatenate([h2_rows(g1), h2_rows(g2)], axis=0).astype(BF16)
    gt = jnp.dot(xs, wg_buf[...], preferred_element_type=F32)
    if CSPAN > 28:
        up = jnp.dot(xs, wu_buf[...], preferred_element_type=F32)
        gbits = pltpu.bitcast(jnp.concatenate([gt, up], axis=1), I32)
    else:
        gbits = pltpu.bitcast(gt, I32)
    ga_, gb_ = modrow(5) * modrow(4), modrow(5) * modrow(3)
    npc = TQ // CPC
    for i in range(npc):
        z = jnp.where(i1 < 0, gbits[0, 128 * (i * CSPAN // npc)], 0)
        x1, nrm = last_norm(lastp, pl.multiple_of(z * CPC + i * CPC, CPC), CPC)
        out_buf[base + i * CPC:base + (i + 1) * CPC, :] = (x1 + nrm * ga_ + gb_).reshape(CPC, D).astype(BF16)
        if i == npc // 2 - 1:
            start(d_out(base, TU, sem.at[SEM_OUT2]))
    start(d_out(base + TU, TU, sem.at[SEM_OUT2]))
    if CBAR:
        cp(out_buf.at[pl.ds(0, base), :], out_hbm.at[0, pl.ds(0, base), :], sem.at[SEM_OUT]).wait()
    if CSPAN <= 28:
        up = jnp.dot(xs, wu_buf[...], preferred_element_type=F32)
    gt = _rb(gt)
    a = (_rb(gt * jax.nn.sigmoid(gt)) * _rb(up)).astype(BF16)
    y = _rb(jnp.dot(a, wd_buf[:, 0:D], preferred_element_type=F32))

    def score(k):
        return pltpu.bitcast(k ^ ((k >> 31) & 0x7FFFFFFF), F32)
    ri = jax.lax.broadcasted_iota(I32, (16, 128), 0)
    rows = jnp.where(ri < 8, g1 + ri, g2 + ri - 8)
    r1 = jnp.concatenate([score(best)] * 2, axis=0)
    r2 = jnp.concatenate([score(second)] * 2, axis=0)
    gate = _rb(jax.nn.sigmoid(_rb(jnp.where(rows == i1, r1, r2))))
    sel = (rows == i1) | (rows == i2)
    upd = jnp.where(sel[:, 0:1], _rb(y * gate[:, 0:1]), 0.0) * mod_buf[0:1, 5 * D:6 * D]
    o1 = (out_buf[pl.ds(g1, 8), :].astype(F32) + upd[0:8]).astype(BF16)
    o2 = (out_buf[pl.ds(g2, 8), :].astype(F32) + upd[8:16]).astype(BF16)

    scope('t_fix')
    if not CBAR:
        cp(out_buf.at[pl.ds(0, base), :], out_hbm.at[0, pl.ds(0, base), :], sem.at[SEM_OUT]).wait()
    wait(d_out(base, TQ, sem.at[SEM_OUT2]))
    out_buf[pl.ds(g1, 8), :] = o1
    out_buf[pl.ds(g2, 8), :] = o2
    start(d_out(g1, 8, sem.at[SEM_FIX]))

    @pl.when(g1 != g2)
    def _():
        start(d_out(g2, 8, sem.at[SEM_FIX + 1]))
        wait(d_out(g2, 8, sem.at[SEM_FIX + 1]))

    wait(d_out(g1, 8, sem.at[SEM_FIX]))
    scope(None)


@jax.jit
def pallas_adaLN_cond__mha_block_cached__moe_arch_mod__prompt_kernel(
    A_x: jax.Array,
    A_k_cache: jax.Array,
    A_v_cache: jax.Array,
    A_wq: jax.Array,
    A_wo: jax.Array,
    B_x: jax.Array,
    B_w_r: jax.Array,
    B_w_gate: jax.Array,
    B_w_up: jax.Array,
    B_w_down: jax.Array,
    c: jax.Array,
    w_mod: jax.Array,
):
    del B_x
    vm = pltpu.VMEM
    scratch = [
        vm((S + PC, D), BF16),
        vm((2, TQ // 2, D), U32),
        vm((H, S, DH), BF16),
        vm((H, S, DH), BF16),
        vm((H, D, DH), BF16),
        vm((H * DH, D), BF16),
        vm((D, FF), BF16),
        vm((D, FF), BF16),
        vm((FF, D + 128), BF16),
        vm((D, 6 * D + 128), BF16),
        vm((1, D), BF16),
        vm((8, 128), BF16),
        vm((8, 8 * D + 256), F32),
        vm((2, TQ, D), F32),
        vm((S, D), BF16),
        vm((TU, S), F32),
        vm((TU, DH), F32),
        vm((TU, DH), F32),
        vm((2, 8, 128), I32),
        vm((2, TQ, 128), F32),
        pltpu.SemaphoreType.DMA((NSEM,)),
    ]
    anyspec = pl.BlockSpec(memory_space=pl.ANY)
    return pl.pallas_call(
        _kernel,
        in_specs=[anyspec] * 11,
        out_specs=anyspec,
        out_shape=jax.ShapeDtypeStruct((1, S, D), BF16),
        scratch_shapes=scratch,
        compiler_params=pltpu.CompilerParams(vmem_limit_bytes=120 * 1024 * 1024, disable_bounds_checks=True,
                                             disable_semaphore_checks=True),
    )(A_x, A_k_cache, A_v_cache, A_wq, A_wo, B_w_r.reshape(8, 128), B_w_gate, B_w_up, B_w_down, c, w_mod)
```

```python
import functools
import os

import jax
import jax.numpy as jnp
import jax.experimental.pallas as pl
import jax.experimental.pallas.tpu as pltpu

F32, BF16, U32, I32 = jnp.float32, jnp.bfloat16, jnp.uint32, jnp.int32

S, D, H, DH, FF = 2048, 1024, 32, 128, 3584
TU = 256
TQ = 512
NQ = S // TQ
HP = int(os.environ.get('HP', 6))
NM = {4: 3, 6: 7}[HP]
NT = (NQ * H - 1 - NM) // HP
NG = (H - 1 - NM) // HP
PC = 16
RC = int(os.environ.get('RC', 16))
AC = int(os.environ.get('AC', 2))
SORD = int(os.environ.get('SORD', 1))
EPC = int(os.environ.get('EPC', 16))
QANCH = int(os.environ.get('QANCH', 1))
WMC = 4
EPS = 1e-5
QSCALE = DH ** -0.5 * 1.4426950408889634
KMIN = -2 ** 31
SCOPES = int(os.environ.get('SCOPES', 0))
TV = int(os.environ.get('TV', 2))
CPC = int(os.environ.get('CPC', 16))
CSPAN = int(os.environ.get('CSPAN', 40))
RFORM = int(os.environ.get('RFORM', 0))
CBAR = int(os.environ.get('CBAR', 0))
TPC = int(os.environ.get('TPC', 64))

SEM_SMALL = 0
SEM_X = 1
SEM_X1A = 5
SEM_WM = 6
SEM_WMR = 10
SEM_WQ0 = 11
SEM_KV0 = 12
SEM_FFN = 13
SEM_OUT = 14
SEM_FIX = 15
SEM_OUT2 = 17
SEM_MINI = 18
SEM_GRP = SEM_MINI + NM + 1
NSEM = SEM_GRP + NG


def _rb(x):
    return x.astype(BF16).astype(F32)


def _ub(x):
    return pltpu.bitcast(x, BF16)


def _pk(x):
    return pltpu.bitcast(x, U32)


def _recip(l):
    r = pl.reciprocal(l, approx=True)
    return r * (2.0 - l * r)


def _ln(x):
    mu = jnp.sum(x, axis=-1, keepdims=True) * (1.0 / D)
    d = x - mu
    var = jnp.sum(d * d, axis=-1, keepdims=True) * (1.0 / D)
    return d * jax.lax.rsqrt(var + EPS)


class _Scope:
    def __init__(self):
        self.cur = None

    def __call__(self, name):
        if not SCOPES:
            return
        if self.cur is not None:
            self.cur.__exit__(None, None, None)
            self.cur = None
        if name:
            self.cur = jax.named_scope(name)
            self.cur.__enter__()


def _kernel(x_hbm, k_hbm, v_hbm, wq_hbm, wo_hbm, wr_hbm, wg_hbm, wu_hbm, wd_hbm, c_hbm, wm_hbm,
            out_hbm,
            x_buf, h_buf, k_buf, v_buf, wq_buf, wo_buf, wg_buf, wu_buf, wd_buf, wm_buf,
            c_buf, wr_buf, mod_buf, acc, out_buf, s_sc, of_sc, l_sc, r_buf, st_buf, sem):
    cp = pltpu.make_async_copy
    scope = _Scope()

    def d_small():
        return [cp(c_hbm, c_buf, sem.at[SEM_SMALL]), cp(wr_hbm, wr_buf, sem.at[SEM_SMALL])]

    def d_xrows(r0, n, s_):
        return [cp(x_hbm.at[0, pl.ds(r0, n), :], x_buf.at[pl.ds(r0, n), :], s_)]

    X1A = 128

    def d_x(j):
        if j == 1:
            return d_xrows(TQ + X1A, TQ - X1A, sem.at[SEM_X + 1])
        return d_xrows(j * TQ, TQ, sem.at[SEM_X + j])

    def d_x1a():
        return d_xrows(TQ, X1A, sem.at[SEM_X1A])

    WC = D // WMC

    def d_wm(i):
        return [cp(wm_hbm.at[:, pl.ds(b + i * WC, WC)], wm_buf.at[:, pl.ds(b + i * WC, WC)], sem.at[SEM_WM + i])
                for b in (0, D)]

    def d_wmr():
        return [cp(wm_hbm.at[:, pl.ds(2 * D, 4 * D)], wm_buf.at[:, pl.ds(2 * D, 4 * D)], sem.at[SEM_WMR])]

    def d_wq(h0, n, s_):
        return [cp(wq_hbm.at[:, pl.ds(pl.multiple_of((h0 + i) * DH, DH), DH)], wq_buf.at[h0 + i], s_)
                for i in range(n)]

    def d_k(h0, n, s_):
        return [cp(k_hbm.at[0, pl.ds(h0, n)], k_buf.at[pl.ds(h0, n)], s_)]

    def d_v(h0, n, s_):
        return [cp(v_hbm.at[0, pl.ds(h0, n)], v_buf.at[pl.ds(h0, n)], s_)]

    def d_wo(h0, n, s_):
        rows = pl.ds(pl.multiple_of(h0 * DH, DH), n * DH)
        return [cp(wo_hbm.at[rows, :], wo_buf.at[rows, :], s_)]

    def d_mini(i):
        s_ = sem.at[SEM_MINI + i]
        return d_wq(i, 1, s_) + d_wo(i - 1, 1, s_) + d_k(i, 1, s_) + d_v(i, 1, s_)

    def d_grp(t):
        s_ = sem.at[SEM_GRP + t]
        h0 = HP * t + NM + 1
        return d_wq(h0, HP, s_) + d_wo(h0 - 1, HP, s_) + d_k(h0, HP, s_) + d_v(h0, HP, s_)

    def d_late():
        return d_wmr() + d_wo(H - 1, 1, sem.at[SEM_WMR])

    def d_ffn(i):
        src, dst = ((wg_hbm, wg_buf), (wu_hbm, wu_buf), (wd_hbm, wd_buf.at[:, pl.ds(0, D)]))[i]
        return [cp(src, dst, sem.at[SEM_FFN])]

    def d_out(r0, n, s_):
        return [cp(out_buf.at[pl.ds(r0, n), :], out_hbm.at[0, pl.ds(r0, n), :], s_)]

    def start(ds):
        for d in ds:
            d.start()

    def wait(ds):
        for d in ds:
            d.wait()

    def qp(unit, anchor=False, zero=None):
        hh, sub, par = unit
        hb = h_buf[par, sub * (TU // 2):(sub + 1) * (TU // 2), :]
        if anchor:
            z16 = pl.multiple_of(zero * 16, 16)
            d0 = _pk(out_buf[pl.ds(z16, 16), 0:128])
            d1 = pltpu.bitcast(r_buf[zero], U32)
            d2 = _pk(x_buf[pl.ds(z16, 16), 0:128])
            top = jnp.concatenate([jnp.where(zero > 0, d0, hb[0:8, 0:128]),
                                   jnp.where(zero > 0, d1, hb[0:8, 128:256]),
                                   jnp.where(zero > 0, d2, hb[0:8, 256:384]), hb[0:8, 384:]], axis=1)
            hb = jnp.concatenate([top, hb[8:]], axis=0)
        q = jnp.dot(_ub(hb), wq_buf[hh], preferred_element_type=F32)
        return (q * QSCALE).astype(BF16)

    def qk(unit, q):
        hh, sub, par = unit
        return jax.lax.dot_general(q, k_buf[hh], (((1,), (1,)), ((), ())), preferred_element_type=F32)

    def pv(unit, s, zero):
        hh, sub, par = unit
        ls, ps = [], []
        nc = S // 128
        for c in range(TU // RC):
            sc = s[c * RC:(c + 1) * RC, :]
            m = jnp.max(sc, axis=-1, keepdims=True)
            p = jnp.exp2(sc - m)
            cols = [p[:, i * 128:(i + 1) * 128] for i in range(nc)]
            a = cols[0]
            for i in range(1, nc):
                if i == nc - AC:
                    part = a
                a = a + cols[i]
            cols[nc - AC] = jnp.where(zero > 0, part, cols[nc - AC])
            ls.append(a)
            ps.append(jnp.concatenate(cols, axis=1))
        o = jnp.dot(jnp.concatenate(ps, axis=0).astype(BF16), v_buf[hh], preferred_element_type=F32)
        return o, jnp.concatenate(ls, axis=0)

    def outp(unit, ol):
        hh, sub, par = unit
        of, lp = ol
        l = jnp.sum(lp, axis=-1, keepdims=True)
        o = (of * _recip(l)).astype(BF16)
        w = wo_buf[pl.ds(pl.multiple_of(hh * DH, DH), DH), :]
        acc[par, sub * TU:(sub + 1) * TU, :] += jnp.dot(o, w, preferred_element_type=F32)

    def modrow(i):
        return mod_buf[:, i * D:(i + 1) * D][None]

    def ln1(xrow0, par, hrow0, n, zero):
        x = x_buf[pl.ds(xrow0, n), :].astype(F32)
        d = acc[zero, pl.ds(pl.multiple_of(zero * 8, 8), n), 0:128]
        x = jnp.concatenate([jnp.where(zero > 0, d, x[:, 0:128]), x[:, 128:]], axis=1)
        h = (_ln(x.reshape(n // 8, 8, D)) * modrow(1) + modrow(0)).reshape(n, D)
        h_buf[par, pl.ds(hrow0, n // 2), :] = _pk(h.astype(BF16))

    def top2_update(r, row0, valid):
        b = pltpu.bitcast(r, I32)
        key = (b ^ ((b >> 31) & 0x7FFFFFFF)) | (S - 1)
        rid = jax.lax.broadcasted_iota(I32, (8, 128), 0) + row0
        best, second = r_buf[0], r_buf[1]
        for i in range(r.shape[0]):
            k = key[i] - (rid + 8 * i)
            if valid is not None:
                k = jnp.where(valid, k, KMIN)
            second = jnp.maximum(second, jnp.minimum(best, k))
            best = jnp.maximum(best, k)
        r_buf[0] = best
        r_buf[1] = second

    def epi(row0, par, arow0, n, valid):
        a = acc[par, pl.ds(arow0, n), :].reshape(n // 8, 8, D)
        acc[par, pl.ds(arow0, n), :] = jnp.zeros((n, D), F32)
        x1 = x_buf[pl.ds(row0, n), :].astype(F32).reshape(n // 8, 8, D) + modrow(2) * a
        d = x1 - jnp.sum(x1, axis=-1, keepdims=True) * (1.0 / D)
        rstd = jax.lax.rsqrt(jnp.sum(d * d, axis=-1, keepdims=True) * (1.0 / D) + EPS)
        h2 = d * rstd * modrow(4) + modrow(3)
        x_buf[pl.ds(pl.multiple_of(jnp.where(valid, row0, S), n), n), :] = h2.reshape(n, D).astype(BF16)
        out_buf[pl.ds(row0, n), :] = (x1 + modrow(5) * h2).reshape(n, D).astype(BF16)
        r = jnp.sum(h2 * modrow(6), axis=-1, keepdims=True)
        top2_update(jnp.broadcast_to(r, (n // 8, 8, 128)), row0, valid)

    def epi_a(row0, par, arow0, n, u, su, c0):
        a = acc[par, arow0:arow0 + n, :].reshape(n // 8, 8, D)
        x1 = x_buf[row0:row0 + n, :].astype(F32).reshape(n // 8, 8, D) + modrow(2) * a
        acc[par, arow0:arow0 + n, :] = x1.reshape(n, D)
        mu = jnp.sum(x1, axis=-1, keepdims=True) * (1.0 / D)
        var = jnp.maximum(jnp.sum(x1 * x1, axis=-1, keepdims=True) * (1.0 / D) - mu * mu, 0.0)
        rstd = jnp.broadcast_to(jax.lax.rsqrt(var + EPS), (n // 8, 8, 128))
        mu = jnp.broadcast_to(mu, (n // 8, 8, 128))
        st_buf[0, arow0:arow0 + n, :] = mu.reshape(n, 128)
        st_buf[1, arow0:arow0 + n, :] = rstd.reshape(n, 128)
        xu = jnp.sum(x1 * u, axis=-1, keepdims=True)
        top2_update((xu - mu * su) * rstd + c0, row0, None)

    def last_norm(par, arow0, n):
        x1 = acc[par, pl.ds(arow0, n), :].reshape(n // 8, 8, D)
        mu = jnp.concatenate([st_buf[0, pl.ds(arow0, n), :]] * 8, axis=1).reshape(n // 8, 8, D)
        rstd = jnp.concatenate([st_buf[1, pl.ds(arow0, n), :]] * 8, axis=1).reshape(n // 8, 8, D)
        return x1, (x1 - mu) * rstd

    def run_units(seq, side, zero):
        s = s_sc[...]
        ol_prev = (of_sc[...], l_sc[...])
        for u in range(len(seq) - 2):
            q = qp(seq[u + 2], u - 1 in side and side[u - 1][1], zero)
            ol = pv(seq[u + 1], s, zero)
            outp(seq[u], ol_prev)
            ol_prev = ol
            if u in side:
                side[u][0]()
            s = qk(seq[u + 2], q)
        s_sc[...] = s
        of_sc[...] = ol_prev[0]
        l_sc[...] = ol_prev[1]

    def mod_cols(c0, n):
        cf = c_buf[...].astype(F32)
        sc = (cf * jax.nn.sigmoid(cf)).astype(BF16)
        sc = jnp.broadcast_to(sc, (16, D))
        m = jnp.dot(sc, wm_buf[:, c0:c0 + n], preferred_element_type=F32)
        return _rb(m[0:8, :])

    start(d_small())
    start(d_x(0))
    for i in range(WMC):
        start(d_wm(i))
    start(d_wq(0, 1, sem.at[SEM_WQ0]))
    start(d_k(0, 1, sem.at[SEM_KV0]) + d_v(0, 1, sem.at[SEM_KV0]))
    start(d_mini(1))
    start(d_x1a())
    for i in range(2, NM + 1):
        start(d_mini(i))
    if HP == 4:
        start(d_grp(0))
        start(d_x(1))
        start(d_grp(1))
    else:
        start(d_x(1))
        start(d_grp(0))

    scope('p_init')
    acc[...] = jnp.zeros(acc.shape, F32)
    mod_buf[...] = jnp.zeros(mod_buf.shape, F32)
    r_buf[...] = jnp.full(r_buf.shape, KMIN, I32)
    out_buf[0:16, :] = jnp.zeros((16, D), BF16)

    wait(d_small())
    wr = wr_buf[...].astype(F32)
    for i in range(8):
        mod_buf[:, 6 * D + i * 128:6 * D + (i + 1) * 128] = jnp.broadcast_to(wr[i:i + 1, :], (8, 128))
    scope('p_ln')
    wait(d_x(0))

    def norm_first(i, _):
        for half in range(2):
            r0 = pl.multiple_of(i * 32, 32)
            x = x_buf[pl.ds(half * TU + r0, 32), :].astype(F32)
            s_sc[pl.ds(r0, 32), half * D:(half + 1) * D] = _ln(x)
        return 0
    jax.lax.fori_loop(0, TU // 32, norm_first, 0)

    scope('p_mod')
    for i in range(WMC):
        wait(d_wm(i))
        sa = mod_cols(i * WC, WC)
        ca = _rb(1.0 + mod_cols(D + i * WC, WC))
        mod_buf[:, i * WC:(i + 1) * WC] = sa
        mod_buf[:, D + i * WC:D + (i + 1) * WC] = ca
        for half in range(2):
            n = s_sc[:, half * D + i * WC:half * D + (i + 1) * WC].reshape(TU // 8, 8, WC)
            h = (n * ca[None] + sa[None]).reshape(TU, WC)
            h_buf[0, half * (TU // 2):(half + 1) * (TU // 2), i * WC:(i + 1) * WC] = _pk(h.astype(BF16))

    scope('p_b1')
    wait(d_wq(0, 1, sem.at[SEM_WQ0]))
    q0 = qp((0, 0, 0))
    q1 = qp((0, 1, 0))
    scope('p_b2')
    wait(d_k(0, 1, sem.at[SEM_KV0]) + d_v(0, 1, sem.at[SEM_KV0]))
    zero0 = r_buf[0, 0, 0] & 1
    s0 = qk((0, 0, 0), q0)
    s_sc[...] = qk((0, 1, 0), q1)
    o0, l0 = pv((0, 0, 0), s0, zero0)
    of_sc[...] = o0
    l_sc[...] = l0
    scope('p_x1a')
    wait(d_x1a())
    scope(None)

    def mini(i, _):
        scope('mini_wait')
        wait(d_mini(i))
        scope(None)
        zero = i >> 10
        side = {}
        for u in range(2):
            r0 = (i - 1 + u) * PC
            side[u] = (functools.partial(ln1, pl.multiple_of(TQ + r0, PC), 1,
                                         pl.multiple_of(r0 // 2, PC // 2), PC, zero), False)
        run_units([(i - 1, 0, 0), (i - 1, 1, 0), (i, 0, 0), (i, 1, 0)], side, zero)
        return 0
    jax.lax.fori_loop(1, NM + 1, mini, 0)
    for t in range(2 if HP == 4 else 1, NG):
        start(d_grp(t))
    start(d_late())
    start(d_x(2))
    start(d_x(3))
    for i in range(3):
        start(d_ffn(i))

    def main(t, _):
        @pl.when(t < NG)
        def _():
            scope('grp_wait')
            wait(d_grp(t))
            scope(None)

        @pl.when(t == (1 if HP == 4 else 0))
        def _():
            wait(d_x(1))

        @pl.when(t == NG)
        def _():
            scope('modrest')
            wait(d_late())
            wait(d_x(2))
            wait(d_x(3))
            for i in range(3):
                wait(d_ffn(i))
            for i in range(2, 6):
                m = mod_cols(i * D, D)
                if i == 4:
                    m = _rb(1.0 + m)
                mod_buf[:, i * D:(i + 1) * D] = m
            scope(None)

        @pl.when(t > NG)
        def _():
            start(d_out(pl.multiple_of((t - 1 - NG) * (HP * PC), PC), HP * PC, sem.at[SEM_OUT]))

        p0 = t * HP + NM + 1
        zero = t >> 10
        seq, side = [], {}
        for k in range(-1, HP):
            if HP == 4 and k >= 0:
                hh, j = (p0 & (H - 1)) + k, p0 >> 5
            else:
                hh, j = (p0 + k) & (H - 1), (p0 + k) >> 5
            par = j & 1
            seq += [(hh, 0, par), (hh, 1, par)]
            if k < 0:
                continue
            r0 = hh * PC
            side[2 * k + SORD] = (functools.partial(
                epi, pl.multiple_of(jnp.maximum(j - 1, 0) * TQ + r0, PC), 1 - par, pl.multiple_of(r0, PC), PC,
                j > 0), True)
            side[2 * k + 1 - SORD] = (functools.partial(
                ln1, pl.multiple_of(jnp.minimum(j + 1, NQ - 1) * TQ + r0, PC), 1 - par,
                pl.multiple_of(hh * (PC // 2), PC // 2), PC, zero), False)
        run_units(seq, side, zero)
        return 0
    jax.lax.fori_loop(0, NT, main, 0)

    scope('t_epi')
    start(d_out((NT - 1 - NG) * HP * PC, HP * PC, sem.at[SEM_OUT]))
    lastp = (NQ - 1) & 1
    base = (NQ - 1) * TQ
    ru = modrow(4) * modrow(6)
    rsu = jnp.sum(ru, axis=-1, keepdims=True)
    rc0 = jnp.sum(modrow(3) * modrow(6), axis=-1, keepdims=True)

    def epis(half):
        for i in range(half * TU // TPC, (half + 1) * TU // TPC):
            epi_a(base + i * TPC, lastp, i * TPC, TPC, ru, rsu, rc0)
    if TV == 0:
        outp((H - 1, 0, lastp), (of_sc[...], l_sc[...]))
        ol = pv((H - 1, 1, lastp), s_sc[...], zero0)
        epis(0)
        outp((H - 1, 1, lastp), ol)
        epis(1)
    elif TV == 2:
        ol = pv((H - 1, 1, lastp), s_sc[...], zero0)
        outp((H - 1, 0, lastp), (of_sc[...], l_sc[...]))
        outp((H - 1, 1, lastp), ol)
        epis(0)
        epis(1)

    scope('t_ffn')
    best, second = r_buf[0], r_buf[1]
    for sh in (4, 2, 1):
        b2 = pltpu.roll(best, sh, 0)
        s2 = pltpu.roll(second, sh, 0)
        second = jnp.maximum(jnp.minimum(best, b2), jnp.maximum(second, s2))
        best = jnp.maximum(best, b2)
    i1 = (S - 1) - (best[0, 0] & (S - 1))
    i2 = (S - 1) - (second[0, 0] & (S - 1))
    g1 = pl.multiple_of((i1 >> 3) << 3, 8)
    g2 = pl.multiple_of((i2 >> 3) << 3, 8)

    def h2_rows(g):
        nrm = last_norm(lastp, pl.multiple_of(jnp.maximum(g - base, 0), 8), 8)[1]
        last = (nrm * modrow(4) + modrow(3)).reshape(8, D)
        return jnp.where(g >= base, last, x_buf[pl.ds(g, 8), :].astype(F32))
    xs = jnp.concatenate([h2_rows(g1), h2_rows(g2)], axis=0).astype(BF16)
    gt = jnp.dot(xs, wg_buf[...], preferred_element_type=F32)
    if CSPAN > 28:
        up = jnp.dot(xs, wu_buf[...], preferred_element_type=F32)
        gbits = pltpu.bitcast(jnp.concatenate([gt, up], axis=1), I32)
    else:
        gbits = pltpu.bitcast(gt, I32)
    ga_, gb_ = modrow(5) * modrow(4), modrow(5) * modrow(3)
    npc = TQ // CPC
    for i in range(npc):
        z = jnp.where(i1 < 0, gbits[0, 128 * (i * CSPAN // npc)], 0)
        x1, nrm = last_norm(lastp, pl.multiple_of(z * CPC + i * CPC, CPC), CPC)
        out_buf[base + i * CPC:base + (i + 1) * CPC, :] = (x1 + nrm * ga_ + gb_).reshape(CPC, D).astype(BF16)
        if i == npc // 2 - 1:
            start(d_out(base, TU, sem.at[SEM_OUT2]))
    start(d_out(base + TU, TU, sem.at[SEM_OUT2]))
    if CBAR:
        cp(out_buf.at[pl.ds(0, base), :], out_hbm.at[0, pl.ds(0, base), :], sem.at[SEM_OUT]).wait()
    if CSPAN <= 28:
        up = jnp.dot(xs, wu_buf[...], preferred_element_type=F32)
    gt = _rb(gt)
    a = (_rb(gt * jax.nn.sigmoid(gt)) * _rb(up)).astype(BF16)
    y = _rb(jnp.dot(a, wd_buf[:, 0:D], preferred_element_type=F32))

    def score(k):
        return pltpu.bitcast(k ^ ((k >> 31) & 0x7FFFFFFF), F32)
    ri = jax.lax.broadcasted_iota(I32, (16, 128), 0)
    rows = jnp.where(ri < 8, g1 + ri, g2 + ri - 8)
    r1 = jnp.concatenate([score(best)] * 2, axis=0)
    r2 = jnp.concatenate([score(second)] * 2, axis=0)
    gate = _rb(jax.nn.sigmoid(_rb(jnp.where(rows == i1, r1, r2))))
    sel = (rows == i1) | (rows == i2)
    upd = jnp.where(sel[:, 0:1], _rb(y * gate[:, 0:1]), 0.0) * mod_buf[0:1, 5 * D:6 * D]
    o1 = (out_buf[pl.ds(g1, 8), :].astype(F32) + upd[0:8]).astype(BF16)
    o2 = (out_buf[pl.ds(g2, 8), :].astype(F32) + upd[8:16]).astype(BF16)

    scope('t_fix')
    if not CBAR:
        cp(out_buf.at[pl.ds(0, base), :], out_hbm.at[0, pl.ds(0, base), :], sem.at[SEM_OUT]).wait()
    wait(d_out(base, TQ, sem.at[SEM_OUT2]))
    out_buf[pl.ds(g1, 8), :] = o1
    out_buf[pl.ds(g2, 8), :] = o2
    start(d_out(g1, 8, sem.at[SEM_FIX]))

    @pl.when(g1 != g2)
    def _():
        start(d_out(g2, 8, sem.at[SEM_FIX + 1]))
        wait(d_out(g2, 8, sem.at[SEM_FIX + 1]))

    wait(d_out(g1, 8, sem.at[SEM_FIX]))
    scope(None)


@jax.jit
def pallas_adaLN_cond__mha_block_cached__moe_arch_mod__prompt_kernel(
    A_x: jax.Array,
    A_k_cache: jax.Array,
    A_v_cache: jax.Array,
    A_wq: jax.Array,
    A_wo: jax.Array,
    B_x: jax.Array,
    B_w_r: jax.Array,
    B_w_gate: jax.Array,
    B_w_up: jax.Array,
    B_w_down: jax.Array,
    c: jax.Array,
    w_mod: jax.Array,
):
    del B_x
    vm = pltpu.VMEM
    scratch = [
        vm((S + PC, D), BF16),
        vm((2, TQ // 2, D), U32),
        vm((H, S, DH), BF16),
        vm((H, S, DH), BF16),
        vm((H, D, DH), BF16),
        vm((H * DH, D), BF16),
        vm((D, FF), BF16),
        vm((D, FF), BF16),
        vm((FF, D + 128), BF16),
        vm((D, 6 * D + 128), BF16),
        vm((1, D), BF16),
        vm((8, 128), BF16),
        vm((8, 7 * D), F32),
        vm((2, TQ, D), F32),
        vm((S, D), BF16),
        vm((TU, S), F32),
        vm((TU, DH), F32),
        vm((TU, DH), F32),
        vm((2, 8, 128), I32),
        vm((2, TQ, 128), F32),
        pltpu.SemaphoreType.DMA((NSEM,)),
    ]
    anyspec = pl.BlockSpec(memory_space=pl.ANY)
    return pl.pallas_call(
        _kernel,
        in_specs=[anyspec] * 11,
        out_specs=anyspec,
        out_shape=jax.ShapeDtypeStruct((1, S, D), BF16),
        scratch_shapes=scratch,
        compiler_params=pltpu.CompilerParams(vmem_limit_bytes=120 * 1024 * 1024, disable_bounds_checks=True,
                                             disable_semaphore_checks=True),
    )(A_x, A_k_cache, A_v_cache, A_wq, A_wo, B_w_r.reshape(8, 128), B_w_gate, B_w_up, B_w_down, c, w_mod)
```

```python
import functools

import jax
import jax.numpy as jnp
import jax.experimental.pallas as pl
import jax.experimental.pallas.tpu as pltpu

F32, BF16, U32, I32 = jnp.float32, jnp.bfloat16, jnp.uint32, jnp.int32

S, D, H, DH, FF = 2048, 1024, 32, 128, 3584
TU = 256
TQ = 512
NQ = S // TQ
HP = 6
NM = {4: 3, 6: 7}[HP]
NT = (NQ * H - 1 - NM) // HP
NG = (H - 1 - NM) // HP
PC = 16
RC = 16
AC = 2
SORD = 1
WMC = 4
EPS = 1e-5
QSCALE = DH ** -0.5 * 1.4426950408889634
KMIN = -2 ** 31
CPC = 16
CSPAN = 40
TPC = 64

SEM_SMALL = 0
SEM_X = 1
SEM_X1A = 5
SEM_WM = 6
SEM_WMR = 10
SEM_WQ0 = 11
SEM_KV0 = 12
SEM_FFN = 13
SEM_OUT = 14
SEM_FIX = 15
SEM_OUT2 = 17
SEM_MINI = 18
SEM_GRP = SEM_MINI + NM + 1
NSEM = SEM_GRP + NG


def _rb(x):
    return x.astype(BF16).astype(F32)


def _ub(x):
    return pltpu.bitcast(x, BF16)


def _pk(x):
    return pltpu.bitcast(x, U32)


def _recip(l):
    r = pl.reciprocal(l, approx=True)
    return r * (2.0 - l * r)


def _ln(x):
    mu = jnp.sum(x, axis=-1, keepdims=True) * (1.0 / D)
    d = x - mu
    var = jnp.sum(d * d, axis=-1, keepdims=True) * (1.0 / D)
    return d * jax.lax.rsqrt(var + EPS)


def _kernel(x_hbm, k_hbm, v_hbm, wq_hbm, wo_hbm, wr_hbm, wg_hbm, wu_hbm, wd_hbm, c_hbm, wm_hbm,
            out_hbm,
            x_buf, h_buf, k_buf, v_buf, wq_buf, wo_buf, wg_buf, wu_buf, wd_buf, wm_buf,
            c_buf, wr_buf, mod_buf, acc, out_buf, s_sc, of_sc, l_sc, r_buf, st_buf, sem):
    cp = pltpu.make_async_copy

    def d_small():
        return [cp(c_hbm, c_buf, sem.at[SEM_SMALL]), cp(wr_hbm, wr_buf, sem.at[SEM_SMALL])]

    def d_xrows(r0, n, s_):
        return [cp(x_hbm.at[0, pl.ds(r0, n), :], x_buf.at[pl.ds(r0, n), :], s_)]

    X1A = 128

    def d_x(j):
        if j == 1:
            return d_xrows(TQ + X1A, TQ - X1A, sem.at[SEM_X + 1])
        return d_xrows(j * TQ, TQ, sem.at[SEM_X + j])

    def d_x1a():
        return d_xrows(TQ, X1A, sem.at[SEM_X1A])

    WC = D // WMC

    def d_wm(i):
        return [cp(wm_hbm.at[:, pl.ds(b + i * WC, WC)], wm_buf.at[:, pl.ds(b + i * WC, WC)], sem.at[SEM_WM + i])
                for b in (0, D)]

    def d_wmr():
        return [cp(wm_hbm.at[:, pl.ds(2 * D, 4 * D)], wm_buf.at[:, pl.ds(2 * D, 4 * D)], sem.at[SEM_WMR])]

    def d_wq(h0, n, s_):
        return [cp(wq_hbm.at[:, pl.ds(pl.multiple_of((h0 + i) * DH, DH), DH)], wq_buf.at[h0 + i], s_)
                for i in range(n)]

    def d_k(h0, n, s_):
        return [cp(k_hbm.at[0, pl.ds(h0, n)], k_buf.at[pl.ds(h0, n)], s_)]

    def d_v(h0, n, s_):
        return [cp(v_hbm.at[0, pl.ds(h0, n)], v_buf.at[pl.ds(h0, n)], s_)]

    def d_wo(h0, n, s_):
        rows = pl.ds(pl.multiple_of(h0 * DH, DH), n * DH)
        return [cp(wo_hbm.at[rows, :], wo_buf.at[rows, :], s_)]

    def d_mini(i):
        s_ = sem.at[SEM_MINI + i]
        return d_wq(i, 1, s_) + d_wo(i - 1, 1, s_) + d_k(i, 1, s_) + d_v(i, 1, s_)

    def d_grp(t):
        s_ = sem.at[SEM_GRP + t]
        h0 = HP * t + NM + 1
        return d_wq(h0, HP, s_) + d_wo(h0 - 1, HP, s_) + d_k(h0, HP, s_) + d_v(h0, HP, s_)

    def d_late():
        return d_wmr() + d_wo(H - 1, 1, sem.at[SEM_WMR])

    def d_ffn(i):
        src, dst = ((wg_hbm, wg_buf), (wu_hbm, wu_buf), (wd_hbm, wd_buf.at[:, pl.ds(0, D)]))[i]
        return [cp(src, dst, sem.at[SEM_FFN])]

    def d_out(r0, n, s_):
        return [cp(out_buf.at[pl.ds(r0, n), :], out_hbm.at[0, pl.ds(r0, n), :], s_)]

    def start(ds):
        for d in ds:
            d.start()

    def wait(ds):
        for d in ds:
            d.wait()

    def qp(unit, anchor=False, zero=None):
        hh, sub, par = unit
        hb = h_buf[par, sub * (TU // 2):(sub + 1) * (TU // 2), :]
        if anchor:
            z16 = pl.multiple_of(zero * 16, 16)
            d0 = _pk(out_buf[pl.ds(z16, 16), 0:128])
            d1 = pltpu.bitcast(r_buf[zero], U32)
            d2 = _pk(x_buf[pl.ds(z16, 16), 0:128])
            top = jnp.concatenate([jnp.where(zero > 0, d0, hb[0:8, 0:128]),
                                   jnp.where(zero > 0, d1, hb[0:8, 128:256]),
                                   jnp.where(zero > 0, d2, hb[0:8, 256:384]), hb[0:8, 384:]], axis=1)
            hb = jnp.concatenate([top, hb[8:]], axis=0)
        q = jnp.dot(_ub(hb), wq_buf[hh], preferred_element_type=F32)
        return (q * QSCALE).astype(BF16)

    def qk(unit, q):
        hh, sub, par = unit
        return jax.lax.dot_general(q, k_buf[hh], (((1,), (1,)), ((), ())), preferred_element_type=F32)

    def pv(unit, s, zero):
        hh, sub, par = unit
        ls, ps = [], []
        nc = S // 128
        for c in range(TU // RC):
            sc = s[c * RC:(c + 1) * RC, :]
            m = jnp.max(sc, axis=-1, keepdims=True)
            p = jnp.exp2(sc - m)
            cols = [p[:, i * 128:(i + 1) * 128] for i in range(nc)]
            a = cols[0]
            for i in range(1, nc):
                if i == nc - AC:
                    part = a
                a = a + cols[i]
            cols[nc - AC] = jnp.where(zero > 0, part, cols[nc - AC])
            ls.append(a)
            ps.append(jnp.concatenate(cols, axis=1))
        o = jnp.dot(jnp.concatenate(ps, axis=0).astype(BF16), v_buf[hh], preferred_element_type=F32)
        return o, jnp.concatenate(ls, axis=0)

    def outp(unit, ol):
        hh, sub, par = unit
        of, lp = ol
        l = jnp.sum(lp, axis=-1, keepdims=True)
        o = (of * _recip(l)).astype(BF16)
        w = wo_buf[pl.ds(pl.multiple_of(hh * DH, DH), DH), :]
        acc[par, sub * TU:(sub + 1) * TU, :] += jnp.dot(o, w, preferred_element_type=F32)

    def modrow(i):
        return mod_buf[:, i * D:(i + 1) * D][None]

    def ln1(xrow0, par, hrow0, n, zero):
        x = x_buf[pl.ds(xrow0, n), :].astype(F32)
        d = acc[zero, pl.ds(pl.multiple_of(zero * 8, 8), n), 0:128]
        x = jnp.concatenate([jnp.where(zero > 0, d, x[:, 0:128]), x[:, 128:]], axis=1)
        h = (_ln(x.reshape(n // 8, 8, D)) * modrow(1) + modrow(0)).reshape(n, D)
        h_buf[par, pl.ds(hrow0, n // 2), :] = _pk(h.astype(BF16))

    def top2_update(r, row0, valid):
        b = pltpu.bitcast(r, I32)
        key = (b ^ ((b >> 31) & 0x7FFFFFFF)) | (S - 1)
        rid = jax.lax.broadcasted_iota(I32, (8, 128), 0) + row0
        best, second = r_buf[0], r_buf[1]
        for i in range(r.shape[0]):
            k = key[i] - (rid + 8 * i)
            if valid is not None:
                k = jnp.where(valid, k, KMIN)
            second = jnp.maximum(second, jnp.minimum(best, k))
            best = jnp.maximum(best, k)
        r_buf[0] = best
        r_buf[1] = second

    def epi(row0, par, arow0, n, valid):
        a = acc[par, pl.ds(arow0, n), :].reshape(n // 8, 8, D)
        acc[par, pl.ds(arow0, n), :] = jnp.zeros((n, D), F32)
        x1 = x_buf[pl.ds(row0, n), :].astype(F32).reshape(n // 8, 8, D) + modrow(2) * a
        d = x1 - jnp.sum(x1, axis=-1, keepdims=True) * (1.0 / D)
        rstd = jax.lax.rsqrt(jnp.sum(d * d, axis=-1, keepdims=True) * (1.0 / D) + EPS)
        h2 = d * rstd * modrow(4) + modrow(3)
        x_buf[pl.ds(pl.multiple_of(jnp.where(valid, row0, S), n), n), :] = h2.reshape(n, D).astype(BF16)
        out_buf[pl.ds(row0, n), :] = (x1 + modrow(5) * h2).reshape(n, D).astype(BF16)
        r = jnp.sum(h2 * modrow(6), axis=-1, keepdims=True)
        top2_update(jnp.broadcast_to(r, (n // 8, 8, 128)), row0, valid)

    def epi_a(row0, par, arow0, n, u, su, c0):
        a = acc[par, arow0:arow0 + n, :].reshape(n // 8, 8, D)
        x1 = x_buf[row0:row0 + n, :].astype(F32).reshape(n // 8, 8, D) + modrow(2) * a
        acc[par, arow0:arow0 + n, :] = x1.reshape(n, D)
        mu = jnp.sum(x1, axis=-1, keepdims=True) * (1.0 / D)
        var = jnp.maximum(jnp.sum(x1 * x1, axis=-1, keepdims=True) * (1.0 / D) - mu * mu, 0.0)
        rstd = jnp.broadcast_to(jax.lax.rsqrt(var + EPS), (n // 8, 8, 128))
        mu = jnp.broadcast_to(mu, (n // 8, 8, 128))
        st_buf[0, arow0:arow0 + n, :] = mu.reshape(n, 128)
        st_buf[1, arow0:arow0 + n, :] = rstd.reshape(n, 128)
        xu = jnp.sum(x1 * u, axis=-1, keepdims=True)
        top2_update((xu - mu * su) * rstd + c0, row0, None)

    def last_norm(par, arow0, n):
        x1 = acc[par, pl.ds(arow0, n), :].reshape(n // 8, 8, D)
        mu = jnp.concatenate([st_buf[0, pl.ds(arow0, n), :]] * 8, axis=1).reshape(n // 8, 8, D)
        rstd = jnp.concatenate([st_buf[1, pl.ds(arow0, n), :]] * 8, axis=1).reshape(n // 8, 8, D)
        return x1, (x1 - mu) * rstd

    def run_units(seq, side, zero):
        s = s_sc[...]
        ol_prev = (of_sc[...], l_sc[...])
        for u in range(len(seq) - 2):
            q = qp(seq[u + 2], u - 1 in side and side[u - 1][1], zero)
            ol = pv(seq[u + 1], s, zero)
            outp(seq[u], ol_prev)
            ol_prev = ol
            if u in side:
                side[u][0]()
            s = qk(seq[u + 2], q)
        s_sc[...] = s
        of_sc[...] = ol_prev[0]
        l_sc[...] = ol_prev[1]

    def mod_cols(c0, n):
        cf = c_buf[...].astype(F32)
        sc = (cf * jax.nn.sigmoid(cf)).astype(BF16)
        sc = jnp.broadcast_to(sc, (16, D))
        m = jnp.dot(sc, wm_buf[:, c0:c0 + n], preferred_element_type=F32)
        return _rb(m[0:8, :])

    start(d_small())
    start(d_x(0))
    for i in range(WMC):
        start(d_wm(i))
    start(d_wq(0, 1, sem.at[SEM_WQ0]))
    start(d_k(0, 1, sem.at[SEM_KV0]) + d_v(0, 1, sem.at[SEM_KV0]))
    start(d_mini(1))
    start(d_x1a())
    for i in range(2, NM + 1):
        start(d_mini(i))
    if HP == 4:
        start(d_grp(0))
        start(d_x(1))
        start(d_grp(1))
    else:
        start(d_x(1))
        start(d_grp(0))
    acc[...] = jnp.zeros(acc.shape, F32)
    mod_buf[...] = jnp.zeros(mod_buf.shape, F32)
    r_buf[...] = jnp.full(r_buf.shape, KMIN, I32)
    out_buf[0:16, :] = jnp.zeros((16, D), BF16)

    wait(d_small())
    wr = wr_buf[...].astype(F32)
    for i in range(8):
        mod_buf[:, 6 * D + i * 128:6 * D + (i + 1) * 128] = jnp.broadcast_to(wr[i:i + 1, :], (8, 128))
    wait(d_x(0))

    def norm_first(i, _):
        for half in range(2):
            r0 = pl.multiple_of(i * 32, 32)
            x = x_buf[pl.ds(half * TU + r0, 32), :].astype(F32)
            s_sc[pl.ds(r0, 32), half * D:(half + 1) * D] = _ln(x)
        return 0
    jax.lax.fori_loop(0, TU // 32, norm_first, 0)
    for i in range(WMC):
        wait(d_wm(i))
        sa = mod_cols(i * WC, WC)
        ca = _rb(1.0 + mod_cols(D + i * WC, WC))
        mod_buf[:, i * WC:(i + 1) * WC] = sa
        mod_buf[:, D + i * WC:D + (i + 1) * WC] = ca
        for half in range(2):
            n = s_sc[:, half * D + i * WC:half * D + (i + 1) * WC].reshape(TU // 8, 8, WC)
            h = (n * ca[None] + sa[None]).reshape(TU, WC)
            h_buf[0, half * (TU // 2):(half + 1) * (TU // 2), i * WC:(i + 1) * WC] = _pk(h.astype(BF16))
    wait(d_wq(0, 1, sem.at[SEM_WQ0]))
    q0 = qp((0, 0, 0))
    q1 = qp((0, 1, 0))
    wait(d_k(0, 1, sem.at[SEM_KV0]) + d_v(0, 1, sem.at[SEM_KV0]))
    zero0 = r_buf[0, 0, 0] & 1
    s0 = qk((0, 0, 0), q0)
    s_sc[...] = qk((0, 1, 0), q1)
    o0, l0 = pv((0, 0, 0), s0, zero0)
    of_sc[...] = o0
    l_sc[...] = l0
    wait(d_x1a())

    def mini(i, _):
        wait(d_mini(i))
        zero = i >> 10
        side = {}
        for u in range(2):
            r0 = (i - 1 + u) * PC
            side[u] = (functools.partial(ln1, pl.multiple_of(TQ + r0, PC), 1,
                                         pl.multiple_of(r0 // 2, PC // 2), PC, zero), False)
        run_units([(i - 1, 0, 0), (i - 1, 1, 0), (i, 0, 0), (i, 1, 0)], side, zero)
        return 0
    jax.lax.fori_loop(1, NM + 1, mini, 0)
    for t in range(2 if HP == 4 else 1, NG):
        start(d_grp(t))
    start(d_late())
    start(d_x(2))
    start(d_x(3))
    for i in range(3):
        start(d_ffn(i))

    def main(t, _):
        @pl.when(t < NG)
        def _():
            wait(d_grp(t))

        @pl.when(t == (1 if HP == 4 else 0))
        def _():
            wait(d_x(1))

        @pl.when(t == NG)
        def _():
            wait(d_late())
            wait(d_x(2))
            wait(d_x(3))
            for i in range(3):
                wait(d_ffn(i))
            for i in range(2, 6):
                m = mod_cols(i * D, D)
                if i == 4:
                    m = _rb(1.0 + m)
                mod_buf[:, i * D:(i + 1) * D] = m

        @pl.when(t > NG)
        def _():
            start(d_out(pl.multiple_of((t - 1 - NG) * (HP * PC), PC), HP * PC, sem.at[SEM_OUT]))

        p0 = t * HP + NM + 1
        zero = t >> 10
        seq, side = [], {}
        for k in range(-1, HP):
            if HP == 4 and k >= 0:
                hh, j = (p0 & (H - 1)) + k, p0 >> 5
            else:
                hh, j = (p0 + k) & (H - 1), (p0 + k) >> 5
            par = j & 1
            seq += [(hh, 0, par), (hh, 1, par)]
            if k < 0:
                continue
            r0 = hh * PC
            side[2 * k + SORD] = (functools.partial(
                epi, pl.multiple_of(jnp.maximum(j - 1, 0) * TQ + r0, PC), 1 - par, pl.multiple_of(r0, PC), PC,
                j > 0), True)
            side[2 * k + 1 - SORD] = (functools.partial(
                ln1, pl.multiple_of(jnp.minimum(j + 1, NQ - 1) * TQ + r0, PC), 1 - par,
                pl.multiple_of(hh * (PC // 2), PC // 2), PC, zero), False)
        run_units(seq, side, zero)
        return 0
    jax.lax.fori_loop(0, NT, main, 0)

    start(d_out((NT - 1 - NG) * HP * PC, HP * PC, sem.at[SEM_OUT]))
    lastp = (NQ - 1) & 1
    base = (NQ - 1) * TQ
    ru = modrow(4) * modrow(6)
    rsu = jnp.sum(ru, axis=-1, keepdims=True)
    rc0 = jnp.sum(modrow(3) * modrow(6), axis=-1, keepdims=True)

    def epis(half):
        for i in range(half * TU // TPC, (half + 1) * TU // TPC):
            epi_a(base + i * TPC, lastp, i * TPC, TPC, ru, rsu, rc0)
    ol = pv((H - 1, 1, lastp), s_sc[...], zero0)
    outp((H - 1, 0, lastp), (of_sc[...], l_sc[...]))
    outp((H - 1, 1, lastp), ol)
    epis(0)
    epis(1)
    best, second = r_buf[0], r_buf[1]
    for sh in (4, 2, 1):
        b2 = pltpu.roll(best, sh, 0)
        s2 = pltpu.roll(second, sh, 0)
        second = jnp.maximum(jnp.minimum(best, b2), jnp.maximum(second, s2))
        best = jnp.maximum(best, b2)
    i1 = (S - 1) - (best[0, 0] & (S - 1))
    i2 = (S - 1) - (second[0, 0] & (S - 1))
    g1 = pl.multiple_of((i1 >> 3) << 3, 8)
    g2 = pl.multiple_of((i2 >> 3) << 3, 8)

    def h2_rows(g):
        nrm = last_norm(lastp, pl.multiple_of(jnp.maximum(g - base, 0), 8), 8)[1]
        last = (nrm * modrow(4) + modrow(3)).reshape(8, D)
        return jnp.where(g >= base, last, x_buf[pl.ds(g, 8), :].astype(F32))
    xs = jnp.concatenate([h2_rows(g1), h2_rows(g2)], axis=0).astype(BF16)
    gt = jnp.dot(xs, wg_buf[...], preferred_element_type=F32)
    up = jnp.dot(xs, wu_buf[...], preferred_element_type=F32)
    gbits = pltpu.bitcast(jnp.concatenate([gt, up], axis=1), I32)
    ga_, gb_ = modrow(5) * modrow(4), modrow(5) * modrow(3)
    npc = TQ // CPC
    for i in range(npc):
        z = jnp.where(i1 < 0, gbits[0, 128 * (i * CSPAN // npc)], 0)
        x1, nrm = last_norm(lastp, pl.multiple_of(z * CPC + i * CPC, CPC), CPC)
        out_buf[base + i * CPC:base + (i + 1) * CPC, :] = (x1 + nrm * ga_ + gb_).reshape(CPC, D).astype(BF16)
        if i == npc // 2 - 1:
            start(d_out(base, TU, sem.at[SEM_OUT2]))
    start(d_out(base + TU, TU, sem.at[SEM_OUT2]))
    gt = _rb(gt)
    a = (_rb(gt * jax.nn.sigmoid(gt)) * _rb(up)).astype(BF16)
    y = _rb(jnp.dot(a, wd_buf[:, 0:D], preferred_element_type=F32))

    def score(k):
        return pltpu.bitcast(k ^ ((k >> 31) & 0x7FFFFFFF), F32)
    ri = jax.lax.broadcasted_iota(I32, (16, 128), 0)
    rows = jnp.where(ri < 8, g1 + ri, g2 + ri - 8)
    r1 = jnp.concatenate([score(best)] * 2, axis=0)
    r2 = jnp.concatenate([score(second)] * 2, axis=0)
    gate = _rb(jax.nn.sigmoid(_rb(jnp.where(rows == i1, r1, r2))))
    sel = (rows == i1) | (rows == i2)
    upd = jnp.where(sel[:, 0:1], _rb(y * gate[:, 0:1]), 0.0) * mod_buf[0:1, 5 * D:6 * D]
    o1 = (out_buf[pl.ds(g1, 8), :].astype(F32) + upd[0:8]).astype(BF16)
    o2 = (out_buf[pl.ds(g2, 8), :].astype(F32) + upd[8:16]).astype(BF16)
    cp(out_buf.at[pl.ds(0, base), :], out_hbm.at[0, pl.ds(0, base), :], sem.at[SEM_OUT]).wait()
    wait(d_out(base, TQ, sem.at[SEM_OUT2]))
    out_buf[pl.ds(g1, 8), :] = o1
    out_buf[pl.ds(g2, 8), :] = o2
    start(d_out(g1, 8, sem.at[SEM_FIX]))

    @pl.when(g1 != g2)
    def _():
        start(d_out(g2, 8, sem.at[SEM_FIX + 1]))
        wait(d_out(g2, 8, sem.at[SEM_FIX + 1]))

    wait(d_out(g1, 8, sem.at[SEM_FIX]))


@jax.jit
def pallas_adaLN_cond__mha_block_cached__moe_arch_mod__prompt_kernel(
    A_x: jax.Array,
    A_k_cache: jax.Array,
    A_v_cache: jax.Array,
    A_wq: jax.Array,
    A_wo: jax.Array,
    B_x: jax.Array,
    B_w_r: jax.Array,
    B_w_gate: jax.Array,
    B_w_up: jax.Array,
    B_w_down: jax.Array,
    c: jax.Array,
    w_mod: jax.Array,
):
    del B_x
    vm = pltpu.VMEM
    scratch = [
        vm((S + PC, D), BF16),
        vm((2, TQ // 2, D), U32),
        vm((H, S, DH), BF16),
        vm((H, S, DH), BF16),
        vm((H, D, DH), BF16),
        vm((H * DH, D), BF16),
        vm((D, FF), BF16),
        vm((D, FF), BF16),
        vm((FF, D + 128), BF16),
        vm((D, 6 * D + 128), BF16),
        vm((1, D), BF16),
        vm((8, 128), BF16),
        vm((8, 7 * D), F32),
        vm((2, TQ, D), F32),
        vm((S, D), BF16),
        vm((TU, S), F32),
        vm((TU, DH), F32),
        vm((TU, DH), F32),
        vm((2, 8, 128), I32),
        vm((2, TQ, 128), F32),
        pltpu.SemaphoreType.DMA((NSEM,)),
    ]
    anyspec = pl.BlockSpec(memory_space=pl.ANY)
    return pl.pallas_call(
        _kernel,
        in_specs=[anyspec] * 11,
        out_specs=anyspec,
        out_shape=jax.ShapeDtypeStruct((1, S, D), BF16),
        scratch_shapes=scratch,
        compiler_params=pltpu.CompilerParams(vmem_limit_bytes=120 * 1024 * 1024, disable_bounds_checks=True,
                                             disable_semaphore_checks=True),
    )(A_x, A_k_cache, A_v_cache, A_wq, A_wo, B_w_r.reshape(8, 128), B_w_gate, B_w_up, B_w_down, c, w_mod)
```

```python
import functools

import jax
import jax.numpy as jnp
import jax.experimental.pallas as pl
import jax.experimental.pallas.tpu as pltpu

F32, BF16, U32, I32 = jnp.float32, jnp.bfloat16, jnp.uint32, jnp.int32

S, D, H, DH, FF = 2048, 1024, 32, 128, 3584
TU = 256
TQ = 512
NQ = S // TQ
HP = 6
NM = {4: 3, 6: 7}[HP]
NT = (NQ * H - 1 - NM) // HP
NG = (H - 1 - NM) // HP
PC = 16
RC = 16
AC = 2
WMC = 4
EPS = 1e-5
QSCALE = DH ** -0.5 * 1.4426950408889634
KMIN = -2 ** 31
CPC = 16
CSPAN = 40
TPC = 64

SEM_SMALL = 0
SEM_X = 1
SEM_X1A = 5
SEM_WM = 6
SEM_WMR = 10
SEM_WQ0 = 11
SEM_KV0 = 12
SEM_FFN = 13
SEM_OUT = 14
SEM_FIX = 15
SEM_OUT2 = 17
SEM_MINI = 18
SEM_GRP = SEM_MINI + NM + 1
NSEM = SEM_GRP + NG


def _rb(x):
    return x.astype(BF16).astype(F32)


def _ub(x):
    return pltpu.bitcast(x, BF16)


def _pk(x):
    return pltpu.bitcast(x, U32)


def _recip(l):
    r = pl.reciprocal(l, approx=True)
    return r * (2.0 - l * r)


def _ln(x):
    mu = jnp.sum(x, axis=-1, keepdims=True) * (1.0 / D)
    d = x - mu
    var = jnp.sum(d * d, axis=-1, keepdims=True) * (1.0 / D)
    return d * jax.lax.rsqrt(var + EPS)


def _stats(x):
    mu = jnp.sum(x, axis=-1, keepdims=True) * (1.0 / D)
    var = jnp.maximum(jnp.sum(x * x, axis=-1, keepdims=True) * (1.0 / D) - mu * mu, 0.0)
    return mu, jax.lax.rsqrt(var + EPS)


def _kernel(x_hbm, k_hbm, v_hbm, wq_hbm, wo_hbm, wr_hbm, wg_hbm, wu_hbm, wd_hbm, c_hbm, wm_hbm,
            out_hbm,
            x_buf, h_buf, k_buf, v_buf, wq_buf, wo_buf, wg_buf, wu_buf, wd_buf, wm_buf,
            c_buf, wr_buf, mod_buf, acc, out_buf, s_sc, of_sc, l_sc, r_buf, st_buf, sem):
    cp = pltpu.make_async_copy

    def d_small():
        return [cp(c_hbm, c_buf, sem.at[SEM_SMALL]), cp(wr_hbm, wr_buf, sem.at[SEM_SMALL])]

    def d_xrows(r0, n, s_):
        return [cp(x_hbm.at[0, pl.ds(r0, n), :], x_buf.at[pl.ds(r0, n), :], s_)]

    X1A = 128

    def d_x(j):
        if j == 1:
            return d_xrows(TQ + X1A, TQ - X1A, sem.at[SEM_X + 1])
        return d_xrows(j * TQ, TQ, sem.at[SEM_X + j])

    def d_x1a():
        return d_xrows(TQ, X1A, sem.at[SEM_X1A])

    WC = D // WMC

    def d_wm(i):
        return [cp(wm_hbm.at[:, pl.ds(b + i * WC, WC)], wm_buf.at[:, pl.ds(b + i * WC, WC)], sem.at[SEM_WM + i])
                for b in (0, D)]

    def d_wmr():
        return [cp(wm_hbm.at[:, pl.ds(2 * D, 4 * D)], wm_buf.at[:, pl.ds(2 * D, 4 * D)], sem.at[SEM_WMR])]

    def d_wq(h0, n, s_):
        return [cp(wq_hbm.at[:, pl.ds(pl.multiple_of((h0 + i) * DH, DH), DH)], wq_buf.at[h0 + i], s_)
                for i in range(n)]

    def d_k(h0, n, s_):
        return [cp(k_hbm.at[0, pl.ds(h0, n)], k_buf.at[pl.ds(h0, n)], s_)]

    def d_v(h0, n, s_):
        return [cp(v_hbm.at[0, pl.ds(h0, n)], v_buf.at[pl.ds(h0, n)], s_)]

    def d_wo(h0, n, s_):
        rows = pl.ds(pl.multiple_of(h0 * DH, DH), n * DH)
        return [cp(wo_hbm.at[rows, :], wo_buf.at[rows, :], s_)]

    def d_mini(i):
        s_ = sem.at[SEM_MINI + i]
        return d_wq(i, 1, s_) + d_wo(i - 1, 1, s_) + d_k(i, 1, s_) + d_v(i, 1, s_)

    def d_grp(t):
        s_ = sem.at[SEM_GRP + t]
        h0 = HP * t + NM + 1
        return d_wq(h0, HP, s_) + d_wo(h0 - 1, HP, s_) + d_k(h0, HP, s_) + d_v(h0, HP, s_)

    def d_late():
        return d_wmr() + d_wo(H - 1, 1, sem.at[SEM_WMR])

    def d_ffn(i):
        src, dst = ((wg_hbm, wg_buf), (wu_hbm, wu_buf), (wd_hbm, wd_buf.at[:, pl.ds(0, D)]))[i]
        return [cp(src, dst, sem.at[SEM_FFN])]

    def d_out(r0, n, s_):
        return [cp(out_buf.at[pl.ds(r0, n), :], out_hbm.at[0, pl.ds(r0, n), :], s_)]

    def start(ds):
        for d in ds:
            d.start()

    def wait(ds):
        for d in ds:
            d.wait()

    def qp(unit, anchor=False, zero=None):
        hh, sub, par = unit
        hb = h_buf[par, sub * (TU // 2):(sub + 1) * (TU // 2), :]
        if anchor:
            z16 = pl.multiple_of(zero * 16, 16)
            d0 = _pk(out_buf[pl.ds(z16, 16), 0:128])
            d1 = pltpu.bitcast(r_buf[zero], U32)
            d2 = _pk(x_buf[pl.ds(z16, 16), 0:128])
            top = jnp.concatenate([jnp.where(zero > 0, d0, hb[0:8, 0:128]),
                                   jnp.where(zero > 0, d1, hb[0:8, 128:256]),
                                   jnp.where(zero > 0, d2, hb[0:8, 256:384]), hb[0:8, 384:]], axis=1)
            hb = jnp.concatenate([top, hb[8:]], axis=0)
        q = jnp.dot(_ub(hb), wq_buf[hh], preferred_element_type=F32)
        return (q * QSCALE).astype(BF16)

    def qk(unit, q):
        hh, sub, par = unit
        return jax.lax.dot_general(q, k_buf[hh], (((1,), (1,)), ((), ())), preferred_element_type=F32)

    def softmax(s, zero):
        ls, ps = [], []
        nc = S // 128
        for c in range(TU // RC):
            sc = s[c * RC:(c + 1) * RC, :]
            m = jnp.max(sc, axis=-1, keepdims=True)
            p = jnp.exp2(sc - m)
            cols = [p[:, i * 128:(i + 1) * 128] for i in range(nc)]
            a = cols[0]
            for i in range(1, nc):
                if i == nc - AC:
                    part = a
                a = a + cols[i]
            cols[nc - AC] = jnp.where(zero > 0, part, cols[nc - AC])
            ls.append(a)
            ps.append(jnp.concatenate(cols, axis=1))
        return jnp.concatenate(ps, axis=0).astype(BF16), jnp.concatenate(ls, axis=0)

    def pv(unit, s, zero):
        hh, sub, par = unit
        pb, lp = softmax(s, zero)
        return jnp.dot(pb, v_buf[hh], preferred_element_type=F32), lp

    def outp(unit, ol):
        hh, sub, par = unit
        of, lp = ol
        l = jnp.sum(lp, axis=-1, keepdims=True)
        o = (of * _recip(l)).astype(BF16)
        w = wo_buf[pl.ds(pl.multiple_of(hh * DH, DH), DH), :]
        acc[par, sub * TU:(sub + 1) * TU, :] += jnp.dot(o, w, preferred_element_type=F32)

    def modrow(i):
        return mod_buf[:, i * D:(i + 1) * D][None]

    def ln1_stats(xrow0, n, zero):
        x = x_buf[pl.ds(xrow0, n), :].astype(F32)
        d = acc[zero, pl.ds(pl.multiple_of(zero * 8, 8), n), 0:128]
        x = jnp.concatenate([jnp.where(zero > 0, d, x[:, 0:128]), x[:, 128:]], axis=1).reshape(n // 8, 8, D)
        return _stats(x)

    def ln1(xrow0, par, hrow0, n, onepass, stats=None):
        x = x_buf[pl.ds(xrow0, n), :].astype(F32).reshape(n // 8, 8, D)
        if stats is None and onepass:
            stats = _stats(x)
        nrm = _ln(x) if stats is None else (x - stats[0]) * stats[1]
        h = (nrm * modrow(1) + modrow(0)).reshape(n, D)
        h_buf[par, pl.ds(hrow0, n // 2), :] = _pk(h.astype(BF16))

    def top2_update(r, row0, valid):
        b = pltpu.bitcast(r, I32)
        key = (b ^ ((b >> 31) & 0x7FFFFFFF)) | (S - 1)
        rid = jax.lax.broadcasted_iota(I32, (8, 128), 0) + row0
        best, second = r_buf[0], r_buf[1]
        for i in range(r.shape[0]):
            k = key[i] - (rid + 8 * i)
            if valid is not None:
                k = jnp.where(valid, k, KMIN)
            second = jnp.maximum(second, jnp.minimum(best, k))
            best = jnp.maximum(best, k)
        r_buf[0] = best
        r_buf[1] = second

    def epi(row0, par, arow0, n, valid):
        a = acc[par, pl.ds(arow0, n), :].reshape(n // 8, 8, D)
        acc[par, pl.ds(arow0, n), :] = jnp.zeros((n, D), F32)
        x1 = x_buf[pl.ds(row0, n), :].astype(F32).reshape(n // 8, 8, D) + modrow(2) * a
        d = x1 - jnp.sum(x1, axis=-1, keepdims=True) * (1.0 / D)
        rstd = jax.lax.rsqrt(jnp.sum(d * d, axis=-1, keepdims=True) * (1.0 / D) + EPS)
        h2 = d * rstd * modrow(4) + modrow(3)
        x_buf[pl.ds(pl.multiple_of(jnp.where(valid, row0, S), n), n), :] = h2.reshape(n, D).astype(BF16)
        out_buf[pl.ds(row0, n), :] = (x1 + modrow(5) * h2).reshape(n, D).astype(BF16)
        r = jnp.sum(h2 * modrow(6), axis=-1, keepdims=True)
        top2_update(jnp.broadcast_to(r, (n // 8, 8, 128)), row0, valid)

    def epi_a(row0, par, arow0, n, u, su, c0):
        a = acc[par, arow0:arow0 + n, :].reshape(n // 8, 8, D)
        x1 = x_buf[row0:row0 + n, :].astype(F32).reshape(n // 8, 8, D) + modrow(2) * a
        acc[par, arow0:arow0 + n, :] = x1.reshape(n, D)
        mu, rstd = [jnp.broadcast_to(v, (n // 8, 8, 128)) for v in _stats(x1)]
        st_buf[0, arow0:arow0 + n, :] = mu.reshape(n, 128)
        st_buf[1, arow0:arow0 + n, :] = rstd.reshape(n, 128)
        xu = jnp.sum(x1 * u, axis=-1, keepdims=True)
        top2_update((xu - mu * su) * rstd + c0, row0, None)

    def last_norm(par, arow0, n):
        x1 = acc[par, pl.ds(arow0, n), :].reshape(n // 8, 8, D)
        mu = jnp.concatenate([st_buf[0, pl.ds(arow0, n), :]] * 8, axis=1).reshape(n // 8, 8, D)
        rstd = jnp.concatenate([st_buf[1, pl.ds(arow0, n), :]] * 8, axis=1).reshape(n // 8, 8, D)
        return x1, (x1 - mu) * rstd

    def run_units(seq, side, zero):
        s = s_sc[...]
        ol_prev = (of_sc[...], l_sc[...])
        for u in range(len(seq) - 2):
            q = qp(seq[u + 2], u > 0 and side[u - 1][1], zero)
            ol = pv(seq[u + 1], s, zero)
            outp(seq[u], ol_prev)
            ol_prev = ol
            side[u][0](q)
            s = qk(seq[u + 2], q)
        s_sc[...] = s
        of_sc[...] = ol_prev[0]
        l_sc[...] = ol_prev[1]

    def mod_cols(c0, n):
        cf = c_buf[...].astype(F32)
        sc = (cf * jax.nn.sigmoid(cf)).astype(BF16)
        sc = jnp.broadcast_to(sc, (16, D))
        m = jnp.dot(sc, wm_buf[:, c0:c0 + n], preferred_element_type=F32)
        return _rb(m[0:8, :])

    start(d_small())
    start(d_x(0))
    for i in range(WMC):
        start(d_wm(i))
    start(d_wq(0, 1, sem.at[SEM_WQ0]))
    start(d_k(0, 1, sem.at[SEM_KV0]) + d_v(0, 1, sem.at[SEM_KV0]))
    start(d_mini(1))
    start(d_x1a())
    for i in range(2, NM + 1):
        start(d_mini(i))
    if HP == 4:
        start(d_grp(0))
        start(d_x(1))
        start(d_grp(1))
    else:
        start(d_x(1))
        start(d_grp(0))
    acc[...] = jnp.zeros(acc.shape, F32)
    mod_buf[...] = jnp.zeros(mod_buf.shape, F32)
    r_buf[...] = jnp.full(r_buf.shape, KMIN, I32)
    out_buf[0:16, :] = jnp.zeros((16, D), BF16)

    wait(d_small())
    wr = wr_buf[...].astype(F32)
    for i in range(8):
        mod_buf[:, 6 * D + i * 128:6 * D + (i + 1) * 128] = jnp.broadcast_to(wr[i:i + 1, :], (8, 128))
    wait(d_x(0))

    def norm_first(i, _):
        for half in range(2):
            r0 = pl.multiple_of(i * 32, 32)
            x = x_buf[pl.ds(half * TU + r0, 32), :].astype(F32)
            s_sc[pl.ds(r0, 32), half * D:(half + 1) * D] = _ln(x)
        return 0
    jax.lax.fori_loop(0, TU // 32, norm_first, 0)
    for i in range(WMC):
        wait(d_wm(i))
        sa = mod_cols(i * WC, WC)
        ca = _rb(1.0 + mod_cols(D + i * WC, WC))
        mod_buf[:, i * WC:(i + 1) * WC] = sa
        mod_buf[:, D + i * WC:D + (i + 1) * WC] = ca
        for half in range(2):
            n = s_sc[:, half * D + i * WC:half * D + (i + 1) * WC].reshape(TU // 8, 8, WC)
            h = (n * ca[None] + sa[None]).reshape(TU, WC)
            h_buf[0, half * (TU // 2):(half + 1) * (TU // 2), i * WC:(i + 1) * WC] = _pk(h.astype(BF16))
    wait(d_wq(0, 1, sem.at[SEM_WQ0]))
    q0 = qp((0, 0, 0))
    q1 = qp((0, 1, 0))
    wait(d_k(0, 1, sem.at[SEM_KV0]) + d_v(0, 1, sem.at[SEM_KV0]))
    zero0 = r_buf[0, 0, 0] & 1
    s0 = qk((0, 0, 0), q0)
    s_sc[...] = qk((0, 1, 0), q1)
    o0, l0 = pv((0, 0, 0), s0, zero0)
    of_sc[...] = o0
    l_sc[...] = l0
    wait(d_x1a())

    def mini(i, _):
        wait(d_mini(i))
        zero = i >> 10
        def piece(u):
            r0 = (i - 1 + u) * PC
            return lambda q: ln1(pl.multiple_of(TQ + r0, PC), 1, pl.multiple_of(r0 // 2, PC // 2), PC, False)
        side = [(piece(0), False), (piece(1), False)]
        run_units([(i - 1, 0, 0), (i - 1, 1, 0), (i, 0, 0), (i, 1, 0)], side, zero)
        return 0
    jax.lax.fori_loop(1, NM + 1, mini, 0)
    for t in range(2 if HP == 4 else 1, NG):
        start(d_grp(t))
    start(d_late())
    start(d_x(2))
    start(d_x(3))
    for i in range(3):
        start(d_ffn(i))

    def main(t, _):
        @pl.when(t < NG)
        def _():
            wait(d_grp(t))

        @pl.when(t == (1 if HP == 4 else 0))
        def _():
            wait(d_x(1))

        @pl.when(t == NG)
        def _():
            wait(d_late())
            wait(d_x(2))
            wait(d_x(3))
            for i in range(3):
                wait(d_ffn(i))
            for i in range(2, 6):
                m = mod_cols(i * D, D)
                if i == 4:
                    m = _rb(1.0 + m)
                mod_buf[:, i * D:(i + 1) * D] = m

        @pl.when(t > NG)
        def _():
            start(d_out(pl.multiple_of((t - 1 - NG) * (HP * PC), PC), HP * PC, sem.at[SEM_OUT]))

        p0 = t * HP + NM + 1
        zero = t >> 10
        seq, side, stats = [], [], {}
        pairs = [((p0 + k) & (H - 1), (p0 + k) >> 5) for k in range(-1, HP)]
        for hh, j in pairs:
            seq += [(hh, 0, j & 1), (hh, 1, j & 1)]

        def xnext(k):
            hh, j = pairs[k + 1]
            return pl.multiple_of(jnp.minimum(j + 1, NQ - 1) * TQ + hh * PC, PC)

        def ln1_piece(k, q):
            hh, j = pairs[k + 1]
            st = stats.get(k)
            if st is not None:
                mu = jnp.where(zero > 0, q[0:PC].astype(F32).reshape(PC // 8, 8, 128),
                               jnp.broadcast_to(st[0], (PC // 8, 8, 128)))
                st = (jnp.concatenate([mu] * 8, axis=2), st[1])
            ln1(xnext(k), 1 - (j & 1), pl.multiple_of(hh * (PC // 2), PC // 2), PC, True, st)

        def epi_piece(k, q):
            hh, j = pairs[k + 1]
            if k + 1 < HP:
                stats[k + 1] = ln1_stats(xnext(k + 1), PC, zero)
            epi(pl.multiple_of(jnp.maximum(j - 1, 0) * TQ + hh * PC, PC), 1 - (j & 1),
                pl.multiple_of(hh * PC, PC), PC, j > 0)

        for k in range(HP):
            side += [(functools.partial(ln1_piece, k), False), (functools.partial(epi_piece, k), True)]
        run_units(seq, side, zero)
        return 0
    jax.lax.fori_loop(0, NT, main, 0)

    start(d_out((NT - 1 - NG) * HP * PC, HP * PC, sem.at[SEM_OUT]))
    lastp = (NQ - 1) & 1
    base = (NQ - 1) * TQ
    ru = modrow(4) * modrow(6)
    rsu = jnp.sum(ru, axis=-1, keepdims=True)
    rc0 = jnp.sum(modrow(3) * modrow(6), axis=-1, keepdims=True)

    def epis(half):
        for i in range(half * TU // TPC, (half + 1) * TU // TPC):
            epi_a(base + i * TPC, lastp, i * TPC, TPC, ru, rsu, rc0)
    ol = pv((H - 1, 1, lastp), s_sc[...], zero0)
    outp((H - 1, 0, lastp), (of_sc[...], l_sc[...]))
    outp((H - 1, 1, lastp), ol)
    epis(0)
    epis(1)
    best, second = r_buf[0], r_buf[1]
    for sh in (4, 2, 1):
        b2 = pltpu.roll(best, sh, 0)
        s2 = pltpu.roll(second, sh, 0)
        second = jnp.maximum(jnp.minimum(best, b2), jnp.maximum(second, s2))
        best = jnp.maximum(best, b2)
    i1 = (S - 1) - (best[0, 0] & (S - 1))
    i2 = (S - 1) - (second[0, 0] & (S - 1))
    g1 = pl.multiple_of((i1 >> 3) << 3, 8)
    g2 = pl.multiple_of((i2 >> 3) << 3, 8)

    def h2_rows(g):
        nrm = last_norm(lastp, pl.multiple_of(jnp.maximum(g - base, 0), 8), 8)[1]
        last = (nrm * modrow(4) + modrow(3)).reshape(8, D)
        return jnp.where(g >= base, last, x_buf[pl.ds(g, 8), :].astype(F32))
    xs = jnp.concatenate([h2_rows(g1), h2_rows(g2)], axis=0).astype(BF16)
    gt = jnp.dot(xs, wg_buf[...], preferred_element_type=F32)
    up = jnp.dot(xs, wu_buf[...], preferred_element_type=F32)
    gbits = pltpu.bitcast(jnp.concatenate([gt, up], axis=1), I32)
    ga_, gb_ = modrow(5) * modrow(4), modrow(5) * modrow(3)
    npc = TQ // CPC
    for i in range(npc):
        z = jnp.where(i1 < 0, gbits[0, 128 * (i * CSPAN // npc)], 0)
        x1, nrm = last_norm(lastp, pl.multiple_of(z * CPC + i * CPC, CPC), CPC)
        out_buf[base + i * CPC:base + (i + 1) * CPC, :] = (x1 + nrm * ga_ + gb_).reshape(CPC, D).astype(BF16)
        if i == npc // 2 - 1:
            start(d_out(base, TU, sem.at[SEM_OUT2]))
    start(d_out(base + TU, TU, sem.at[SEM_OUT2]))
    gt = _rb(gt)
    a = (_rb(gt * jax.nn.sigmoid(gt)) * _rb(up)).astype(BF16)
    y = _rb(jnp.dot(a, wd_buf[:, 0:D], preferred_element_type=F32))

    def score(k):
        return pltpu.bitcast(k ^ ((k >> 31) & 0x7FFFFFFF), F32)
    ri = jax.lax.broadcasted_iota(I32, (16, 128), 0)
    rows = jnp.where(ri < 8, g1 + ri, g2 + ri - 8)
    r1 = jnp.concatenate([score(best)] * 2, axis=0)
    r2 = jnp.concatenate([score(second)] * 2, axis=0)
    gate = _rb(jax.nn.sigmoid(_rb(jnp.where(rows == i1, r1, r2))))
    sel = (rows == i1) | (rows == i2)
    upd = jnp.where(sel[:, 0:1], _rb(y * gate[:, 0:1]), 0.0) * mod_buf[0:1, 5 * D:6 * D]
    o1 = (out_buf[pl.ds(g1, 8), :].astype(F32) + upd[0:8]).astype(BF16)
    o2 = (out_buf[pl.ds(g2, 8), :].astype(F32) + upd[8:16]).astype(BF16)
    cp(out_buf.at[pl.ds(0, base), :], out_hbm.at[0, pl.ds(0, base), :], sem.at[SEM_OUT]).wait()
    wait(d_out(base, TQ, sem.at[SEM_OUT2]))
    out_buf[pl.ds(g1, 8), :] = o1
    out_buf[pl.ds(g2, 8), :] = o2
    start(d_out(g1, 8, sem.at[SEM_FIX]))

    @pl.when(g1 != g2)
    def _():
        start(d_out(g2, 8, sem.at[SEM_FIX + 1]))
        wait(d_out(g2, 8, sem.at[SEM_FIX + 1]))

    wait(d_out(g1, 8, sem.at[SEM_FIX]))


@jax.jit
def pallas_adaLN_cond__mha_block_cached__moe_arch_mod__prompt_kernel(
    A_x: jax.Array,
    A_k_cache: jax.Array,
    A_v_cache: jax.Array,
    A_wq: jax.Array,
    A_wo: jax.Array,
    B_x: jax.Array,
    B_w_r: jax.Array,
    B_w_gate: jax.Array,
    B_w_up: jax.Array,
    B_w_down: jax.Array,
    c: jax.Array,
    w_mod: jax.Array,
):
    del B_x
    vm = pltpu.VMEM
    scratch = [
        vm((S + PC, D), BF16),
        vm((2, TQ // 2, D), U32),
        vm((H, S, DH), BF16),
        vm((H, S, DH), BF16),
        vm((H, D, DH), BF16),
        vm((H * DH, D), BF16),
        vm((D, FF), BF16),
        vm((D, FF), BF16),
        vm((FF, D + 128), BF16),
        vm((D, 6 * D + 128), BF16),
        vm((1, D), BF16),
        vm((8, 128), BF16),
        vm((8, 7 * D), F32),
        vm((2, TQ, D), F32),
        vm((S, D), BF16),
        vm((TU, S), F32),
        vm((TU, DH), F32),
        vm((TU, DH), F32),
        vm((2, 8, 128), I32),
        vm((2, TQ, 128), F32),
        pltpu.SemaphoreType.DMA((NSEM,)),
    ]
    anyspec = pl.BlockSpec(memory_space=pl.ANY)
    return pl.pallas_call(
        _kernel,
        in_specs=[anyspec] * 11,
        out_specs=anyspec,
        out_shape=jax.ShapeDtypeStruct((1, S, D), BF16),
        scratch_shapes=scratch,
        compiler_params=pltpu.CompilerParams(vmem_limit_bytes=120 * 1024 * 1024, disable_bounds_checks=True,
                                             disable_semaphore_checks=True),
    )(A_x, A_k_cache, A_v_cache, A_wq, A_wo, B_w_r.reshape(8, 128), B_w_gate, B_w_up, B_w_down, c, w_mod)
```

```python
import functools

import jax
import jax.numpy as jnp
import jax.experimental.pallas as pl
import jax.experimental.pallas.tpu as pltpu

F32, BF16, U32, I32 = jnp.float32, jnp.bfloat16, jnp.uint32, jnp.int32

S, D, H, DH, FF = 2048, 1024, 32, 128, 3584
TU = 256
TQ = 512
NQ = S // TQ
HP = 6
NM = {4: 3, 6: 7}[HP]
NT = (NQ * H - 1 - NM) // HP
NG = (H - 1 - NM) // HP
PC = 16
RC = 16
AC = 2
WMC = 4
EPS = 1e-5
QSCALE = DH ** -0.5 * 1.4426950408889634
KMIN = -2 ** 31
CPC = 32
CSPAN = 40
TPC = 64

SEM_SMALL = 0
SEM_X = 1
SEM_X1A = 5
SEM_WM = 6
SEM_WMR = 10
SEM_WQ0 = 11
SEM_KV0 = 12
SEM_FFN = 13
SEM_OUT = 14
SEM_FIX = 15
SEM_OUT2 = 17
SEM_V0 = 18
SEM_MINI = 19
SEM_GRP = SEM_MINI + NM + 1
NSEM = SEM_GRP + NG


def _rb(x):
    return x.astype(BF16).astype(F32)


def _ub(x):
    return pltpu.bitcast(x, BF16)


def _pk(x):
    return pltpu.bitcast(x, U32)


def _recip(l):
    r = pl.reciprocal(l, approx=True)
    return r * (2.0 - l * r)


def _ln(x):
    mu = jnp.sum(x, axis=-1, keepdims=True) * (1.0 / D)
    d = x - mu
    var = jnp.sum(d * d, axis=-1, keepdims=True) * (1.0 / D)
    return d * jax.lax.rsqrt(var + EPS)


def _stats(x):
    mu = jnp.sum(x, axis=-1, keepdims=True) * (1.0 / D)
    var = jnp.maximum(jnp.sum(x * x, axis=-1, keepdims=True) * (1.0 / D) - mu * mu, 0.0)
    return mu, jax.lax.rsqrt(var + EPS)


def _kernel(x_hbm, k_hbm, v_hbm, wq_hbm, wo_hbm, wr_hbm, wg_hbm, wu_hbm, wd_hbm, c_hbm, wm_hbm,
            out_hbm,
            x_buf, h_buf, k_buf, v_buf, wq_buf, wo_buf, wg_buf, wu_buf, wd_buf, wm_buf,
            c_buf, wr_buf, mod_buf, acc, out_buf, s_sc, of_sc, l_sc, r_buf, st_buf, sem):
    cp = pltpu.make_async_copy

    def d_small():
        return [cp(c_hbm, c_buf, sem.at[SEM_SMALL]), cp(wr_hbm, wr_buf, sem.at[SEM_SMALL])]

    def d_xrows(r0, n, s_):
        return [cp(x_hbm.at[0, pl.ds(r0, n), :], x_buf.at[pl.ds(r0, n), :], s_)]

    X1A = 128

    def d_x(j):
        if j == 1:
            return d_xrows(TQ + X1A, TQ - X1A, sem.at[SEM_X + 1])
        return d_xrows(j * TQ, TQ, sem.at[SEM_X + j])

    def d_x1a():
        return d_xrows(TQ, X1A, sem.at[SEM_X1A])

    WC = D // WMC

    def d_wm(i):
        return [cp(wm_hbm.at[:, pl.ds(b + i * WC, WC)], wm_buf.at[:, pl.ds(b + i * WC, WC)], sem.at[SEM_WM + i])
                for b in (0, D)]

    def d_wmr():
        return [cp(wm_hbm.at[:, pl.ds(2 * D, 4 * D)], wm_buf.at[:, pl.ds(2 * D, 4 * D)], sem.at[SEM_WMR])]

    def d_wq(h0, n, s_):
        return [cp(wq_hbm.at[:, pl.ds(pl.multiple_of((h0 + i) * DH, DH), DH)], wq_buf.at[h0 + i], s_)
                for i in range(n)]

    def d_k(h0, n, s_):
        return [cp(k_hbm.at[0, pl.ds(h0, n)], k_buf.at[pl.ds(h0, n)], s_)]

    def d_v(h0, n, s_):
        return [cp(v_hbm.at[0, pl.ds(h0, n)], v_buf.at[pl.ds(h0, n)], s_)]

    def d_wo(h0, n, s_):
        rows = pl.ds(pl.multiple_of(h0 * DH, DH), n * DH)
        return [cp(wo_hbm.at[rows, :], wo_buf.at[rows, :], s_)]

    def d_mini(i):
        s_ = sem.at[SEM_MINI + i]
        return d_wq(i, 1, s_) + d_wo(i - 1, 1, s_) + d_k(i, 1, s_) + d_v(i, 1, s_)

    def d_grp(t):
        s_ = sem.at[SEM_GRP + t]
        h0 = HP * t + NM + 1
        return d_wq(h0, HP, s_) + d_wo(h0 - 1, HP, s_) + d_k(h0, HP, s_) + d_v(h0, HP, s_)

    def d_late():
        return d_wmr() + d_wo(H - 1, 1, sem.at[SEM_WMR])

    def d_ffn(i):
        src, dst = ((wg_hbm, wg_buf), (wu_hbm, wu_buf), (wd_hbm, wd_buf.at[:, pl.ds(0, D)]))[i]
        return [cp(src, dst, sem.at[SEM_FFN])]

    def d_out(r0, n, s_):
        return [cp(out_buf.at[pl.ds(r0, n), :], out_hbm.at[0, pl.ds(r0, n), :], s_)]

    def start(ds):
        for d in ds:
            d.start()

    def wait(ds):
        for d in ds:
            d.wait()

    def qp(unit, anchor=False, zero=None):
        hh, sub, par = unit
        hb = h_buf[par, sub * (TU // 2):(sub + 1) * (TU // 2), :]
        if anchor:
            z16 = pl.multiple_of(zero * 16, 16)
            d0 = _pk(out_buf[pl.ds(z16, 16), 0:128])
            d1 = pltpu.bitcast(r_buf[zero], U32)
            d2 = _pk(x_buf[pl.ds(z16, 16), 0:128])
            top = jnp.concatenate([jnp.where(zero > 0, d0, hb[0:8, 0:128]),
                                   jnp.where(zero > 0, d1, hb[0:8, 128:256]),
                                   jnp.where(zero > 0, d2, hb[0:8, 256:384]), hb[0:8, 384:]], axis=1)
            hb = jnp.concatenate([top, hb[8:]], axis=0)
        q = jnp.dot(_ub(hb), wq_buf[hh], preferred_element_type=F32)
        return (q * QSCALE).astype(BF16)

    def qk(unit, q):
        hh, sub, par = unit
        return jax.lax.dot_general(q, k_buf[hh], (((1,), (1,)), ((), ())), preferred_element_type=F32)

    def softmax(s, zero):
        ls, ps = [], []
        nc = S // 128
        for c in range(TU // RC):
            sc = s[c * RC:(c + 1) * RC, :]
            m = jnp.max(sc, axis=-1, keepdims=True)
            p = jnp.exp2(sc - m)
            cols = [p[:, i * 128:(i + 1) * 128] for i in range(nc)]
            a = cols[0]
            for i in range(1, nc):
                if i == nc - AC:
                    part = a
                a = a + cols[i]
            cols[nc - AC] = jnp.where(zero > 0, part, cols[nc - AC])
            ls.append(a)
            ps.append(jnp.concatenate(cols, axis=1))
        return jnp.concatenate(ps, axis=0).astype(BF16), jnp.concatenate(ls, axis=0)

    def pv(unit, s, zero):
        hh, sub, par = unit
        pb, lp = softmax(s, zero)
        return jnp.dot(pb, v_buf[hh], preferred_element_type=F32), lp

    def outp(unit, ol):
        hh, sub, par = unit
        of, lp = ol
        l = jnp.sum(lp, axis=-1, keepdims=True)
        o = (of * _recip(l)).astype(BF16)
        w = wo_buf[pl.ds(pl.multiple_of(hh * DH, DH), DH), :]
        acc[par, sub * TU:(sub + 1) * TU, :] += jnp.dot(o, w, preferred_element_type=F32)

    def modrow(i):
        return mod_buf[:, i * D:(i + 1) * D][None]

    def ln1_stats(xrow0, n, zero):
        x = x_buf[pl.ds(xrow0, n), :].astype(F32)
        d = acc[zero, pl.ds(pl.multiple_of(zero * 8, 8), n), 0:128]
        x = jnp.concatenate([jnp.where(zero > 0, d, x[:, 0:128]), x[:, 128:]], axis=1).reshape(n // 8, 8, D)
        return _stats(x)

    def ln1(xrow0, par, hrow0, n, onepass, stats=None):
        x = x_buf[pl.ds(xrow0, n), :].astype(F32).reshape(n // 8, 8, D)
        if stats is None and onepass:
            stats = _stats(x)
        nrm = _ln(x) if stats is None else (x - stats[0]) * stats[1]
        h = (nrm * modrow(1) + modrow(0)).reshape(n, D)
        h_buf[par, pl.ds(hrow0, n // 2), :] = _pk(h.astype(BF16))

    def top2_update(r, row0, valid):
        b = pltpu.bitcast(r, I32)
        key = (b ^ ((b >> 31) & 0x7FFFFFFF)) | (S - 1)
        rid = jax.lax.broadcasted_iota(I32, (8, 128), 0) + row0
        best, second = r_buf[0], r_buf[1]
        for i in range(r.shape[0]):
            k = key[i] - (rid + 8 * i)
            if valid is not None:
                k = jnp.where(valid, k, KMIN)
            second = jnp.maximum(second, jnp.minimum(best, k))
            best = jnp.maximum(best, k)
        r_buf[0] = best
        r_buf[1] = second

    def epi(row0, par, arow0, n, valid):
        a = acc[par, pl.ds(arow0, n), :].reshape(n // 8, 8, D)
        acc[par, pl.ds(arow0, n), :] = jnp.zeros((n, D), F32)
        x1 = x_buf[pl.ds(row0, n), :].astype(F32).reshape(n // 8, 8, D) + modrow(2) * a
        d = x1 - jnp.sum(x1, axis=-1, keepdims=True) * (1.0 / D)
        rstd = jax.lax.rsqrt(jnp.sum(d * d, axis=-1, keepdims=True) * (1.0 / D) + EPS)
        h2 = d * rstd * modrow(4) + modrow(3)
        x_buf[pl.ds(pl.multiple_of(jnp.where(valid, row0, S), n), n), :] = h2.reshape(n, D).astype(BF16)
        out_buf[pl.ds(row0, n), :] = (x1 + modrow(5) * h2).reshape(n, D).astype(BF16)
        r = jnp.sum(h2 * modrow(6), axis=-1, keepdims=True)
        top2_update(jnp.broadcast_to(r, (n // 8, 8, 128)), row0, valid)

    def epi_a(row0, par, arow0, n, u, su, c0):
        a = acc[par, arow0:arow0 + n, :].reshape(n // 8, 8, D)
        x1 = x_buf[row0:row0 + n, :].astype(F32).reshape(n // 8, 8, D) + modrow(2) * a
        acc[par, arow0:arow0 + n, :] = x1.reshape(n, D)
        mu, rstd = [jnp.broadcast_to(v, (n // 8, 8, 128)) for v in _stats(x1)]
        st_buf[0, arow0:arow0 + n, :] = mu.reshape(n, 128)
        st_buf[1, arow0:arow0 + n, :] = rstd.reshape(n, 128)
        xu = jnp.sum(x1 * u, axis=-1, keepdims=True)
        top2_update((xu - mu * su) * rstd + c0, row0, None)

    def last_norm(par, arow0, n):
        x1 = acc[par, pl.ds(arow0, n), :].reshape(n // 8, 8, D)
        mu = jnp.concatenate([st_buf[0, pl.ds(arow0, n), :]] * 8, axis=1).reshape(n // 8, 8, D)
        rstd = jnp.concatenate([st_buf[1, pl.ds(arow0, n), :]] * 8, axis=1).reshape(n // 8, 8, D)
        return x1, (x1 - mu) * rstd

    def run_units(seq, side, zero):
        s = s_sc[...]
        ol_prev = (of_sc[...], l_sc[...])
        for u in range(len(seq) - 2):
            q = qp(seq[u + 2], u > 0 and side[u - 1][1], zero)
            ol = pv(seq[u + 1], s, zero)
            outp(seq[u], ol_prev)
            ol_prev = ol
            side[u][0](q)
            s = qk(seq[u + 2], q)
        s_sc[...] = s
        of_sc[...] = ol_prev[0]
        l_sc[...] = ol_prev[1]

    def mod_cols(c0, n):
        cf = c_buf[...].astype(F32)
        sc = (cf * jax.nn.sigmoid(cf)).astype(BF16)
        sc = jnp.broadcast_to(sc, (16, D))
        m = jnp.dot(sc, wm_buf[:, c0:c0 + n], preferred_element_type=F32)
        return _rb(m[0:8, :])

    start(d_small())
    start(d_x(0))
    for i in range(WMC):
        start(d_wm(i))
    start(d_wq(0, 1, sem.at[SEM_WQ0]))
    start(d_k(0, 1, sem.at[SEM_KV0]) + d_v(0, 1, sem.at[SEM_V0]))
    start(d_mini(1))
    start(d_x1a())
    for i in range(2, NM + 1):
        start(d_mini(i))
    if HP == 4:
        start(d_grp(0))
        start(d_x(1))
        start(d_grp(1))
    else:
        start(d_x(1))
        start(d_grp(0))
    acc[...] = jnp.zeros(acc.shape, F32)
    mod_buf[...] = jnp.zeros(mod_buf.shape, F32)
    r_buf[...] = jnp.full(r_buf.shape, KMIN, I32)
    out_buf[0:16, :] = jnp.zeros((16, D), BF16)

    zero0 = r_buf[0, 0, 0] & 1

    def rest(_i, _c):
        wait(d_small())
        wr = wr_buf[...].astype(F32)
        for i in range(8):
            mod_buf[:, 6 * D + i * 128:6 * D + (i + 1) * 128] = jnp.broadcast_to(wr[i:i + 1, :], (8, 128))
        wait(d_x(0))

        def norm_first(i, _):
            for half in range(2):
                r0 = pl.multiple_of(i * 32, 32)
                x = x_buf[pl.ds(half * TU + r0, 32), :].astype(F32)
                s_sc[pl.ds(r0, 32), half * D:(half + 1) * D] = _ln(x)
            return 0
        jax.lax.fori_loop(0, TU // 32, norm_first, 0)
        for i in range(WMC):
            wait(d_wm(i))
            sa = mod_cols(i * WC, WC)
            ca = _rb(1.0 + mod_cols(D + i * WC, WC))
            mod_buf[:, i * WC:(i + 1) * WC] = sa
            mod_buf[:, D + i * WC:D + (i + 1) * WC] = ca
            for half in range(2):
                n = s_sc[:, half * D + i * WC:half * D + (i + 1) * WC].reshape(TU // 8, 8, WC)
                h = (n * ca[None] + sa[None]).reshape(TU, WC)
                h_buf[0, half * (TU // 2):(half + 1) * (TU // 2), i * WC:(i + 1) * WC] = _pk(h.astype(BF16))
        wait(d_wq(0, 1, sem.at[SEM_WQ0]))
        q0 = qp((0, 0, 0))
        q1 = qp((0, 1, 0))
        wait(d_k(0, 1, sem.at[SEM_KV0]))
        s0 = qk((0, 0, 0), q0)
        wait(d_v(0, 1, sem.at[SEM_V0]))
        s_sc[...] = qk((0, 1, 0), q1)
        o0, l0 = pv((0, 0, 0), s0, zero0)
        of_sc[...] = o0
        l_sc[...] = l0

        def mini(i, _):
            wait(d_mini(i))

            @pl.when(i == 2)
            def _():
                wait(d_x1a())
            zero = i >> 10
            def piece(u):
                pc = jnp.minimum(2 * (i - 2) + u, NM)
                return lambda q: ln1(pl.multiple_of(TQ + pc * PC, PC), 1,
                                     pl.multiple_of(jnp.maximum(pc, 0) * (PC // 2), PC // 2), PC, False)
            side = [(piece(0), False), (piece(1), False)]
            run_units([(i - 1, 0, 0), (i - 1, 1, 0), (i, 0, 0), (i, 1, 0)], side, zero)
            return 0
        jax.lax.fori_loop(1, NM + 1, mini, 0)
        for t in range(2 if HP == 4 else 1, NG):
            start(d_grp(t))
        start(d_late())
        start(d_x(2))
        start(d_x(3))
        for i in range(3):
            start(d_ffn(i))

        def main(t, _):
            @pl.when(t < NG)
            def _():
                wait(d_grp(t))

            @pl.when(t == (1 if HP == 4 else 0))
            def _():
                wait(d_x(1))

            @pl.when(t == NG)
            def _():
                wait(d_late())
                wait(d_x(2))
                wait(d_x(3))
                for i in range(3):
                    wait(d_ffn(i))
                for i in range(2, 6):
                    m = mod_cols(i * D, D)
                    if i == 4:
                        m = _rb(1.0 + m)
                    mod_buf[:, i * D:(i + 1) * D] = m

            @pl.when(t > NG)
            def _():
                start(d_out(pl.multiple_of((t - 1 - NG) * (HP * PC), PC), HP * PC, sem.at[SEM_OUT]))

            p0 = t * HP + NM + 1
            zero = t >> 10
            seq, side, stats = [], [], {}
            pairs = [((p0 + k) & (H - 1), (p0 + k) >> 5) for k in range(-1, HP)]
            for hh, j in pairs:
                seq += [(hh, 0, j & 1), (hh, 1, j & 1)]

            def xnext(k):
                hh, j = pairs[k + 1]
                return pl.multiple_of(jnp.minimum(j + 1, NQ - 1) * TQ + hh * PC, PC)

            def ln1_piece(k, q):
                hh, j = pairs[k + 1]
                st = stats.get(k)
                if st is not None:
                    mu = jnp.where(zero > 0, q[0:PC].astype(F32).reshape(PC // 8, 8, 128),
                                   jnp.broadcast_to(st[0], (PC // 8, 8, 128)))
                    st = (jnp.concatenate([mu] * 8, axis=2), st[1])
                ln1(xnext(k), 1 - (j & 1), pl.multiple_of(hh * (PC // 2), PC // 2), PC, True, st)

            def epi_piece(k, q):
                hh, j = pairs[k + 1]
                if k + 1 < HP:
                    stats[k + 1] = ln1_stats(xnext(k + 1), PC, zero)
                epi(pl.multiple_of(jnp.maximum(j - 1, 0) * TQ + hh * PC, PC), 1 - (j & 1),
                    pl.multiple_of(hh * PC, PC), PC, j > 0)

            for k in range(HP):
                side += [(functools.partial(ln1_piece, k), False), (functools.partial(epi_piece, k), True)]
            run_units(seq, side, zero)
            return 0
        jax.lax.fori_loop(0, NT, main, 0)

        start(d_out((NT - 1 - NG) * HP * PC, HP * PC, sem.at[SEM_OUT]))
        lastp = (NQ - 1) & 1
        base = (NQ - 1) * TQ
        ru = modrow(4) * modrow(6)
        rsu = jnp.sum(ru, axis=-1, keepdims=True)
        rc0 = jnp.sum(modrow(3) * modrow(6), axis=-1, keepdims=True)

        def epis(half):
            for i in range(half * TU // TPC, (half + 1) * TU // TPC):
                epi_a(base + i * TPC, lastp, i * TPC, TPC, ru, rsu, rc0)
        ol = pv((H - 1, 1, lastp), s_sc[...], zero0)
        outp((H - 1, 0, lastp), (of_sc[...], l_sc[...]))
        outp((H - 1, 1, lastp), ol)
        epis(0)
        epis(1)
        best, second = r_buf[0], r_buf[1]
        for sh in (4, 2, 1):
            b2 = pltpu.roll(best, sh, 0)
            s2 = pltpu.roll(second, sh, 0)
            second = jnp.maximum(jnp.minimum(best, b2), jnp.maximum(second, s2))
            best = jnp.maximum(best, b2)
        i1 = (S - 1) - (best[0, 0] & (S - 1))
        i2 = (S - 1) - (second[0, 0] & (S - 1))
        g1 = pl.multiple_of((i1 >> 3) << 3, 8)
        g2 = pl.multiple_of((i2 >> 3) << 3, 8)

        def h2_rows(g):
            nrm = last_norm(lastp, pl.multiple_of(jnp.maximum(g - base, 0), 8), 8)[1]
            last = (nrm * modrow(4) + modrow(3)).reshape(8, D)
            return jnp.where(g >= base, last, x_buf[pl.ds(g, 8), :].astype(F32))
        xs = jnp.concatenate([h2_rows(g1), h2_rows(g2)], axis=0).astype(BF16)
        gt = jnp.dot(xs, wg_buf[...], preferred_element_type=F32)
        up = jnp.dot(xs, wu_buf[...], preferred_element_type=F32)
        gbits = pltpu.bitcast(jnp.concatenate([gt, up], axis=1), I32)
        ga_, gb_ = modrow(5) * modrow(4), modrow(5) * modrow(3)
        npc = TQ // CPC
        for i in range(npc):
            z = jnp.where(i1 < 0, gbits[0, 128 * (i * CSPAN // npc)], 0)
            x1, nrm = last_norm(lastp, pl.multiple_of(z * CPC + i * CPC, CPC), CPC)
            out_buf[base + i * CPC:base + (i + 1) * CPC, :] = (x1 + nrm * ga_ + gb_).reshape(CPC, D).astype(BF16)
            if i == npc // 2 - 1:
                start(d_out(base, TU, sem.at[SEM_OUT2]))
        start(d_out(base + TU, TU, sem.at[SEM_OUT2]))
        gt = _rb(gt)
        a = (_rb(gt * jax.nn.sigmoid(gt)) * _rb(up)).astype(BF16)
        y = _rb(jnp.dot(a, wd_buf[:, 0:D], preferred_element_type=F32))

        def score(k):
            return pltpu.bitcast(k ^ ((k >> 31) & 0x7FFFFFFF), F32)
        ri = jax.lax.broadcasted_iota(I32, (16, 128), 0)
        rows = jnp.where(ri < 8, g1 + ri, g2 + ri - 8)
        r1 = jnp.concatenate([score(best)] * 2, axis=0)
        r2 = jnp.concatenate([score(second)] * 2, axis=0)
        gate = _rb(jax.nn.sigmoid(_rb(jnp.where(rows == i1, r1, r2))))
        sel = (rows == i1) | (rows == i2)
        upd = jnp.where(sel[:, 0:1], _rb(y * gate[:, 0:1]), 0.0) * mod_buf[0:1, 5 * D:6 * D]
        o1 = (out_buf[pl.ds(g1, 8), :].astype(F32) + upd[0:8]).astype(BF16)
        o2 = (out_buf[pl.ds(g2, 8), :].astype(F32) + upd[8:16]).astype(BF16)
        cp(out_buf.at[pl.ds(0, base), :], out_hbm.at[0, pl.ds(0, base), :], sem.at[SEM_OUT]).wait()
        wait(d_out(base, TQ, sem.at[SEM_OUT2]))
        out_buf[pl.ds(g1, 8), :] = o1
        out_buf[pl.ds(g2, 8), :] = o2
        start(d_out(g1, 8, sem.at[SEM_FIX]))

        @pl.when(g1 != g2)
        def _():
            start(d_out(g2, 8, sem.at[SEM_FIX + 1]))
            wait(d_out(g2, 8, sem.at[SEM_FIX + 1]))

        wait(d_out(g1, 8, sem.at[SEM_FIX]))
        return 0
    jax.lax.fori_loop(0, zero0 + 1, rest, 0)


@jax.jit
def pallas_adaLN_cond__mha_block_cached__moe_arch_mod__prompt_kernel(
    A_x: jax.Array,
    A_k_cache: jax.Array,
    A_v_cache: jax.Array,
    A_wq: jax.Array,
    A_wo: jax.Array,
    B_x: jax.Array,
    B_w_r: jax.Array,
    B_w_gate: jax.Array,
    B_w_up: jax.Array,
    B_w_down: jax.Array,
    c: jax.Array,
    w_mod: jax.Array,
):
    del B_x
    vm = pltpu.VMEM
    scratch = [
        vm((S + PC, D), BF16),
        vm((2, TQ // 2, D), U32),
        vm((H, S, DH), BF16),
        vm((H, S, DH), BF16),
        vm((H, D, DH), BF16),
        vm((H * DH, D), BF16),
        vm((D, FF), BF16),
        vm((D, FF), BF16),
        vm((FF, D + 128), BF16),
        vm((D, 6 * D + 128), BF16),
        vm((1, D), BF16),
        vm((8, 128), BF16),
        vm((8, 7 * D), F32),
        vm((2, TQ, D), F32),
        vm((S, D), BF16),
        vm((TU, S), F32),
        vm((TU, DH), F32),
        vm((TU, DH), F32),
        vm((2, 8, 128), I32),
        vm((2, TQ, 128), F32),
        pltpu.SemaphoreType.DMA((NSEM,)),
    ]
    anyspec = pl.BlockSpec(memory_space=pl.ANY)
    return pl.pallas_call(
        _kernel,
        in_specs=[anyspec] * 11,
        out_specs=anyspec,
        out_shape=jax.ShapeDtypeStruct((1, S, D), BF16),
        scratch_shapes=scratch,
        compiler_params=pltpu.CompilerParams(vmem_limit_bytes=120 * 1024 * 1024, disable_bounds_checks=True,
                                             disable_semaphore_checks=True),
    )(A_x, A_k_cache, A_v_cache, A_wq, A_wo, B_w_r.reshape(8, 128), B_w_gate, B_w_up, B_w_down, c, w_mod)
```

```python
import functools

import jax
import jax.numpy as jnp
import jax.experimental.pallas as pl
import jax.experimental.pallas.tpu as pltpu

F32, BF16, U32, I32 = jnp.float32, jnp.bfloat16, jnp.uint32, jnp.int32

S, D, H, DH, FF = 2048, 1024, 32, 128, 3584
TU = 256
TQ = 512
NQ = S // TQ
HP = 6
NM = {4: 3, 6: 7}[HP]
NT = (NQ * H - 1 - NM) // HP
NG = (H - 1 - NM) // HP
PC = 16
RC = 16
AC = 2
AC0 = 8
AC1 = 2
ACM0 = 2
ACM1 = 2
ACP = 1
ACT = 3
WMC = 4
EPS = 1e-5
QSCALE = DH ** -0.5 * 1.4426950408889634
KMIN = -2 ** 31
CPC = 32
CSPAN = 40
TPC = 64

SEM_SMALL = 0
SEM_X = 1
SEM_X1A = 5
SEM_WM = 6
SEM_WMR = 10
SEM_WQ0 = 11
SEM_KV0 = 12
SEM_FFN = 13
SEM_OUT = 14
SEM_FIX = 15
SEM_OUT2 = 17
SEM_V0 = 18
SEM_MINI = 19
SEM_GRP = SEM_MINI + NM + 1
NSEM = SEM_GRP + NG


def _rb(x):
    return x.astype(BF16).astype(F32)


def _ub(x):
    return pltpu.bitcast(x, BF16)


def _pk(x):
    return pltpu.bitcast(x, U32)


def _recip(l):
    r = pl.reciprocal(l, approx=True)
    return r * (2.0 - l * r)


def _ln(x):
    mu = jnp.sum(x, axis=-1, keepdims=True) * (1.0 / D)
    d = x - mu
    var = jnp.sum(d * d, axis=-1, keepdims=True) * (1.0 / D)
    return d * jax.lax.rsqrt(var + EPS)


def _stats(x):
    mu = jnp.sum(x, axis=-1, keepdims=True) * (1.0 / D)
    var = jnp.maximum(jnp.sum(x * x, axis=-1, keepdims=True) * (1.0 / D) - mu * mu, 0.0)
    return mu, jax.lax.rsqrt(var + EPS)


def _kernel(x_hbm, k_hbm, v_hbm, wq_hbm, wo_hbm, wr_hbm, wg_hbm, wu_hbm, wd_hbm, c_hbm, wm_hbm,
            out_hbm,
            x_buf, h_buf, k_buf, v_buf, wq_buf, wo_buf, wg_buf, wu_buf, wd_buf, wm_buf,
            c_buf, wr_buf, mod_buf, acc, out_buf, s_sc, of_sc, l_sc, r_buf, st_buf, sem):
    cp = pltpu.make_async_copy

    def d_small():
        return [cp(c_hbm, c_buf, sem.at[SEM_SMALL]), cp(wr_hbm, wr_buf, sem.at[SEM_SMALL])]

    def d_xrows(r0, n, s_):
        return [cp(x_hbm.at[0, pl.ds(r0, n), :], x_buf.at[pl.ds(r0, n), :], s_)]

    X1A = 128

    def d_x(j):
        if j == 1:
            return d_xrows(TQ + X1A, TQ - X1A, sem.at[SEM_X + 1])
        return d_xrows(j * TQ, TQ, sem.at[SEM_X + j])

    def d_x1a():
        return d_xrows(TQ, X1A, sem.at[SEM_X1A])

    WC = D // WMC

    def d_wm(i):
        return [cp(wm_hbm.at[:, pl.ds(b + i * WC, WC)], wm_buf.at[:, pl.ds(b + i * WC, WC)], sem.at[SEM_WM + i])
                for b in (0, D)]

    def d_wmr():
        return [cp(wm_hbm.at[:, pl.ds(2 * D, 4 * D)], wm_buf.at[:, pl.ds(2 * D, 4 * D)], sem.at[SEM_WMR])]

    def d_wq(h0, n, s_):
        return [cp(wq_hbm.at[:, pl.ds(pl.multiple_of((h0 + i) * DH, DH), DH)], wq_buf.at[h0 + i], s_)
                for i in range(n)]

    def d_k(h0, n, s_):
        return [cp(k_hbm.at[0, pl.ds(h0, n)], k_buf.at[pl.ds(h0, n)], s_)]

    def d_v(h0, n, s_):
        return [cp(v_hbm.at[0, pl.ds(h0, n)], v_buf.at[pl.ds(h0, n)], s_)]

    def d_wo(h0, n, s_):
        rows = pl.ds(pl.multiple_of(h0 * DH, DH), n * DH)
        return [cp(wo_hbm.at[rows, :], wo_buf.at[rows, :], s_)]

    def d_mini(i):
        s_ = sem.at[SEM_MINI + i]
        return d_wq(i, 1, s_) + d_wo(i - 1, 1, s_) + d_k(i, 1, s_) + d_v(i, 1, s_)

    def d_grp(t):
        s_ = sem.at[SEM_GRP + t]
        h0 = HP * t + NM + 1
        return d_wq(h0, HP, s_) + d_wo(h0 - 1, HP, s_) + d_k(h0, HP, s_) + d_v(h0, HP, s_)

    def d_late():
        return d_wmr() + d_wo(H - 1, 1, sem.at[SEM_WMR])

    def d_ffn(i):
        src, dst = ((wg_hbm, wg_buf), (wu_hbm, wu_buf), (wd_hbm, wd_buf.at[:, pl.ds(0, D)]))[i]
        return [cp(src, dst, sem.at[SEM_FFN])]

    def d_out(r0, n, s_):
        return [cp(out_buf.at[pl.ds(r0, n), :], out_hbm.at[0, pl.ds(r0, n), :], s_)]

    def start(ds):
        for d in ds:
            d.start()

    def wait(ds):
        for d in ds:
            d.wait()

    def qp(unit, anchor=False, zero=None):
        hh, sub, par = unit
        hb = h_buf[par, sub * (TU // 2):(sub + 1) * (TU // 2), :]
        if anchor:
            z16 = pl.multiple_of(zero * 16, 16)
            d0 = _pk(out_buf[pl.ds(z16, 16), 0:128])
            d1 = pltpu.bitcast(r_buf[zero], U32)
            d2 = _pk(x_buf[pl.ds(z16, 16), 0:128])
            top = jnp.concatenate([jnp.where(zero > 0, d0, hb[0:8, 0:128]),
                                   jnp.where(zero > 0, d1, hb[0:8, 128:256]),
                                   jnp.where(zero > 0, d2, hb[0:8, 256:384]), hb[0:8, 384:]], axis=1)
            hb = jnp.concatenate([top, hb[8:]], axis=0)
        q = jnp.dot(_ub(hb), wq_buf[hh], preferred_element_type=F32)
        return (q * QSCALE).astype(BF16)

    def qk(unit, q):
        hh, sub, par = unit
        return jax.lax.dot_general(q, k_buf[hh], (((1,), (1,)), ((), ())), preferred_element_type=F32)

    def softmax(s, zero, AC=AC):
        ls, ps = [], []
        nc = S // 128
        for c in range(TU // RC):
            sc = s[c * RC:(c + 1) * RC, :]
            m = jnp.max(sc, axis=-1, keepdims=True)
            p = jnp.exp2(sc - m)
            cols = [p[:, i * 128:(i + 1) * 128] for i in range(nc)]
            a = cols[0]
            for i in range(1, nc):
                if i == nc - AC:
                    part = a
                a = a + cols[i]
            if AC:
                cols[nc - AC] = jnp.where(zero > 0, part, cols[nc - AC])
            ls.append(a)
            ps.append(jnp.concatenate(cols, axis=1))
        return jnp.concatenate(ps, axis=0).astype(BF16), jnp.concatenate(ls, axis=0)

    def pv(unit, s, zero, ac=AC):
        hh, sub, par = unit
        pb, lp = softmax(s, zero, ac)
        return jnp.dot(pb, v_buf[hh], preferred_element_type=F32), lp

    def outp(unit, ol):
        hh, sub, par = unit
        of, lp = ol
        l = jnp.sum(lp, axis=-1, keepdims=True)
        o = (of * _recip(l)).astype(BF16)
        w = wo_buf[pl.ds(pl.multiple_of(hh * DH, DH), DH), :]
        acc[par, sub * TU:(sub + 1) * TU, :] += jnp.dot(o, w, preferred_element_type=F32)

    def modrow(i):
        return mod_buf[:, i * D:(i + 1) * D][None]

    def ln1_stats(xrow0, n, zero):
        x = x_buf[pl.ds(xrow0, n), :].astype(F32)
        d = acc[zero, pl.ds(pl.multiple_of(zero * 8, 8), n), 0:128]
        x = jnp.concatenate([jnp.where(zero > 0, d, x[:, 0:128]), x[:, 128:]], axis=1).reshape(n // 8, 8, D)
        return _stats(x)

    def ln1(xrow0, par, hrow0, n, onepass, stats=None):
        x = x_buf[pl.ds(xrow0, n), :].astype(F32).reshape(n // 8, 8, D)
        if stats is None and onepass:
            stats = _stats(x)
        nrm = _ln(x) if stats is None else (x - stats[0]) * stats[1]
        h = (nrm * modrow(1) + modrow(0)).reshape(n, D)
        h_buf[par, pl.ds(hrow0, n // 2), :] = _pk(h.astype(BF16))

    def top2_update(r, row0, valid):
        b = pltpu.bitcast(r, I32)
        key = (b ^ ((b >> 31) & 0x7FFFFFFF)) | (S - 1)
        rid = jax.lax.broadcasted_iota(I32, (8, 128), 0) + row0
        best, second = r_buf[0], r_buf[1]
        for i in range(r.shape[0]):
            k = key[i] - (rid + 8 * i)
            if valid is not None:
                k = jnp.where(valid, k, KMIN)
            second = jnp.maximum(second, jnp.minimum(best, k))
            best = jnp.maximum(best, k)
        r_buf[0] = best
        r_buf[1] = second

    def epi(row0, par, arow0, n, valid):
        a = acc[par, pl.ds(arow0, n), :].reshape(n // 8, 8, D)
        acc[par, pl.ds(arow0, n), :] = jnp.zeros((n, D), F32)
        x1 = x_buf[pl.ds(row0, n), :].astype(F32).reshape(n // 8, 8, D) + modrow(2) * a
        d = x1 - jnp.sum(x1, axis=-1, keepdims=True) * (1.0 / D)
        rstd = jax.lax.rsqrt(jnp.sum(d * d, axis=-1, keepdims=True) * (1.0 / D) + EPS)
        h2 = d * rstd * modrow(4) + modrow(3)
        x_buf[pl.ds(pl.multiple_of(jnp.where(valid, row0, S), n), n), :] = h2.reshape(n, D).astype(BF16)
        out_buf[pl.ds(row0, n), :] = (x1 + modrow(5) * h2).reshape(n, D).astype(BF16)
        r = jnp.sum(h2 * modrow(6), axis=-1, keepdims=True)
        top2_update(jnp.broadcast_to(r, (n // 8, 8, 128)), row0, valid)

    def epi_a(row0, par, arow0, n, u, su, c0):
        a = acc[par, arow0:arow0 + n, :].reshape(n // 8, 8, D)
        x1 = x_buf[row0:row0 + n, :].astype(F32).reshape(n // 8, 8, D) + modrow(2) * a
        acc[par, arow0:arow0 + n, :] = x1.reshape(n, D)
        mu, rstd = [jnp.broadcast_to(v, (n // 8, 8, 128)) for v in _stats(x1)]
        st_buf[0, arow0:arow0 + n, :] = mu.reshape(n, 128)
        st_buf[1, arow0:arow0 + n, :] = rstd.reshape(n, 128)
        xu = jnp.sum(x1 * u, axis=-1, keepdims=True)
        top2_update((xu - mu * su) * rstd + c0, row0, None)

    def last_norm(par, arow0, n):
        x1 = acc[par, pl.ds(arow0, n), :].reshape(n // 8, 8, D)
        mu = jnp.concatenate([st_buf[0, pl.ds(arow0, n), :]] * 8, axis=1).reshape(n // 8, 8, D)
        rstd = jnp.concatenate([st_buf[1, pl.ds(arow0, n), :]] * 8, axis=1).reshape(n // 8, 8, D)
        return x1, (x1 - mu) * rstd

    def run_units(seq, side, zero, acs={}):
        s = s_sc[...]
        ol_prev = (of_sc[...], l_sc[...])
        for u in range(len(seq) - 2):
            q = qp(seq[u + 2], u > 0 and side[u - 1][1], zero)
            ol = pv(seq[u + 1], s, zero, acs.get(u, AC))
            outp(seq[u], ol_prev)
            ol_prev = ol
            side[u][0](q)
            s = qk(seq[u + 2], q)
        s_sc[...] = s
        of_sc[...] = ol_prev[0]
        l_sc[...] = ol_prev[1]

    def mod_cols(c0, n):
        cf = c_buf[...].astype(F32)
        sc = (cf * jax.nn.sigmoid(cf)).astype(BF16)
        sc = jnp.broadcast_to(sc, (16, D))
        m = jnp.dot(sc, wm_buf[:, c0:c0 + n], preferred_element_type=F32)
        return _rb(m[0:8, :])

    start(d_small())
    start(d_x(0))
    for i in range(WMC):
        start(d_wm(i))
    start(d_wq(0, 1, sem.at[SEM_WQ0]))
    start(d_k(0, 1, sem.at[SEM_KV0]) + d_v(0, 1, sem.at[SEM_V0]))
    start(d_mini(1))
    start(d_x1a())
    for i in range(2, NM + 1):
        start(d_mini(i))
    if HP == 4:
        start(d_grp(0))
        start(d_x(1))
        start(d_grp(1))
    else:
        start(d_x(1))
        start(d_grp(0))
    acc[...] = jnp.zeros(acc.shape, F32)
    mod_buf[...] = jnp.zeros(mod_buf.shape, F32)
    r_buf[...] = jnp.full(r_buf.shape, KMIN, I32)
    out_buf[0:16, :] = jnp.zeros((16, D), BF16)

    zero0 = r_buf[0, 0, 0] & 1

    def rest(_i, _c):
        wait(d_small())
        wr = wr_buf[...].astype(F32)
        for i in range(8):
            mod_buf[:, 6 * D + i * 128:6 * D + (i + 1) * 128] = jnp.broadcast_to(wr[i:i + 1, :], (8, 128))
        wait(d_x(0))

        def norm_first(i, _):
            for half in range(2):
                r0 = pl.multiple_of(i * 32, 32)
                x = x_buf[pl.ds(half * TU + r0, 32), :].astype(F32)
                s_sc[pl.ds(r0, 32), half * D:(half + 1) * D] = _ln(x)
            return 0
        jax.lax.fori_loop(0, TU // 32, norm_first, 0)
        for i in range(WMC):
            wait(d_wm(i))
            sa = mod_cols(i * WC, WC)
            ca = _rb(1.0 + mod_cols(D + i * WC, WC))
            mod_buf[:, i * WC:(i + 1) * WC] = sa
            mod_buf[:, D + i * WC:D + (i + 1) * WC] = ca
            for half in range(2):
                n = s_sc[:, half * D + i * WC:half * D + (i + 1) * WC].reshape(TU // 8, 8, WC)
                h = (n * ca[None] + sa[None]).reshape(TU, WC)
                h_buf[0, half * (TU // 2):(half + 1) * (TU // 2), i * WC:(i + 1) * WC] = _pk(h.astype(BF16))
        wait(d_wq(0, 1, sem.at[SEM_WQ0]))
        q0 = qp((0, 0, 0))
        q1 = qp((0, 1, 0))
        wait(d_k(0, 1, sem.at[SEM_KV0]))
        s0 = qk((0, 0, 0), q0)
        wait(d_v(0, 1, sem.at[SEM_V0]))
        s_sc[...] = qk((0, 1, 0), q1)
        o0, l0 = pv((0, 0, 0), s0, zero0, ACP)
        of_sc[...] = o0
        l_sc[...] = l0

        def mini(i, _):
            wait(d_mini(i))

            @pl.when(i == 2)
            def _():
                wait(d_x1a())
            zero = i >> 10
            def piece(u):
                pc = jnp.minimum(2 * (i - 2) + u, NM)
                return lambda q: ln1(pl.multiple_of(TQ + pc * PC, PC), 1,
                                     pl.multiple_of(jnp.maximum(pc, 0) * (PC // 2), PC // 2), PC, False)
            side = [(piece(0), False), (piece(1), False)]
            run_units([(i - 1, 0, 0), (i - 1, 1, 0), (i, 0, 0), (i, 1, 0)], side, zero, {0: ACM0, 1: ACM1})
            return 0
        jax.lax.fori_loop(1, NM + 1, mini, 0)
        for t in range(2 if HP == 4 else 1, NG):
            start(d_grp(t))
        start(d_late())
        start(d_x(2))
        start(d_x(3))
        for i in range(3):
            start(d_ffn(i))

        def main(t, _):
            @pl.when(t < NG)
            def _():
                wait(d_grp(t))

            @pl.when(t == (1 if HP == 4 else 0))
            def _():
                wait(d_x(1))

            @pl.when(t == NG)
            def _():
                wait(d_late())
                wait(d_x(2))
                wait(d_x(3))
                for i in range(3):
                    wait(d_ffn(i))
                for i in range(2, 6):
                    m = mod_cols(i * D, D)
                    if i == 4:
                        m = _rb(1.0 + m)
                    mod_buf[:, i * D:(i + 1) * D] = m

            @pl.when(t > NG)
            def _():
                start(d_out(pl.multiple_of((t - 1 - NG) * (HP * PC), PC), HP * PC, sem.at[SEM_OUT]))

            p0 = t * HP + NM + 1
            zero = t >> 10
            seq, side, stats = [], [], {}
            pairs = [((p0 + k) & (H - 1), (p0 + k) >> 5) for k in range(-1, HP)]
            for hh, j in pairs:
                seq += [(hh, 0, j & 1), (hh, 1, j & 1)]

            def xnext(k):
                hh, j = pairs[k + 1]
                return pl.multiple_of(jnp.minimum(j + 1, NQ - 1) * TQ + hh * PC, PC)

            def ln1_piece(k, q):
                hh, j = pairs[k + 1]
                st = stats.get(k)
                if st is not None:
                    mu = jnp.where(zero > 0, q[0:PC].astype(F32).reshape(PC // 8, 8, 128),
                                   jnp.broadcast_to(st[0], (PC // 8, 8, 128)))
                    st = (jnp.concatenate([mu] * 8, axis=2), st[1])
                ln1(xnext(k), 1 - (j & 1), pl.multiple_of(hh * (PC // 2), PC // 2), PC, True, st)

            def epi_piece(k, q):
                hh, j = pairs[k + 1]
                if k + 1 < HP:
                    stats[k + 1] = ln1_stats(xnext(k + 1), PC, zero)
                epi(pl.multiple_of(jnp.maximum(j - 1, 0) * TQ + hh * PC, PC), 1 - (j & 1),
                    pl.multiple_of(hh * PC, PC), PC, j > 0)

            for k in range(HP):
                side += [(functools.partial(ln1_piece, k), False), (functools.partial(epi_piece, k), True)]
            run_units(seq, side, zero, {0: AC0, 1: AC1})
            return 0
        jax.lax.fori_loop(0, NT, main, 0)

        start(d_out((NT - 1 - NG) * HP * PC, HP * PC, sem.at[SEM_OUT]))
        lastp = (NQ - 1) & 1
        base = (NQ - 1) * TQ
        ru = modrow(4) * modrow(6)
        rsu = jnp.sum(ru, axis=-1, keepdims=True)
        rc0 = jnp.sum(modrow(3) * modrow(6), axis=-1, keepdims=True)

        def epis(half):
            for i in range(half * TU // TPC, (half + 1) * TU // TPC):
                epi_a(base + i * TPC, lastp, i * TPC, TPC, ru, rsu, rc0)
        ol = pv((H - 1, 1, lastp), s_sc[...], zero0, ACT)
        outp((H - 1, 0, lastp), (of_sc[...], l_sc[...]))
        outp((H - 1, 1, lastp), ol)
        epis(0)
        epis(1)
        best, second = r_buf[0], r_buf[1]
        for sh in (4, 2, 1):
            b2 = pltpu.roll(best, sh, 0)
            s2 = pltpu.roll(second, sh, 0)
            second = jnp.maximum(jnp.minimum(best, b2), jnp.maximum(second, s2))
            best = jnp.maximum(best, b2)
        i1 = (S - 1) - (best[0, 0] & (S - 1))
        i2 = (S - 1) - (second[0, 0] & (S - 1))
        g1 = pl.multiple_of(jnp.clip(i1 >> 3, 0, S // 8 - 1) * 8, 8)
        g2 = pl.multiple_of(jnp.clip(i2 >> 3, 0, S // 8 - 1) * 8, 8)

        def h2_rows(g):
            nrm = last_norm(lastp, pl.multiple_of(jnp.clip(g - base, 0, TQ - 8), 8), 8)[1]
            last = (nrm * modrow(4) + modrow(3)).reshape(8, D)
            return jnp.where(g >= base, last, x_buf[pl.ds(g, 8), :].astype(F32))
        xs = jnp.concatenate([h2_rows(g1), h2_rows(g2)], axis=0).astype(BF16)
        gt = jnp.dot(xs, wg_buf[...], preferred_element_type=F32)
        up = jnp.dot(xs, wu_buf[...], preferred_element_type=F32)
        gbits = pltpu.bitcast(jnp.concatenate([gt, up], axis=1), I32)
        ga_, gb_ = modrow(5) * modrow(4), modrow(5) * modrow(3)
        npc = TQ // CPC
        for i in range(npc):
            z = jnp.where(i1 < 0, gbits[0, 128 * (i * CSPAN // npc)], 0)
            x1, nrm = last_norm(lastp, pl.multiple_of(jnp.clip(z + i, 0, npc - 1) * CPC, CPC), CPC)
            out_buf[base + i * CPC:base + (i + 1) * CPC, :] = (x1 + nrm * ga_ + gb_).reshape(CPC, D).astype(BF16)
            if i == npc // 2 - 1:
                start(d_out(base, TU, sem.at[SEM_OUT2]))
        start(d_out(base + TU, TU, sem.at[SEM_OUT2]))
        gt = _rb(gt)
        a = (_rb(gt * jax.nn.sigmoid(gt)) * _rb(up)).astype(BF16)
        y = _rb(jnp.dot(a, wd_buf[:, 0:D], preferred_element_type=F32))

        def score(k):
            return pltpu.bitcast((k ^ ((k >> 31) & 0x7FFFFFFF)) & -S, F32)
        ri = jax.lax.broadcasted_iota(I32, (16, 128), 0)
        rows = jnp.where(ri < 8, g1 + ri, g2 + ri - 8)
        r1 = jnp.concatenate([score(best)] * 2, axis=0)
        r2 = jnp.concatenate([score(second)] * 2, axis=0)
        gate = _rb(jax.nn.sigmoid(_rb(jnp.where(rows == i1, r1, r2))))
        sel = (rows == i1) | (rows == i2)
        upd = jnp.where(sel[:, 0:1], _rb(y * gate[:, 0:1]), 0.0) * mod_buf[0:1, 5 * D:6 * D]
        o1 = (out_buf[pl.ds(g1, 8), :].astype(F32) + upd[0:8]).astype(BF16)
        o2 = (out_buf[pl.ds(g2, 8), :].astype(F32) + upd[8:16]).astype(BF16)
        cp(out_buf.at[pl.ds(0, base), :], out_hbm.at[0, pl.ds(0, base), :], sem.at[SEM_OUT]).wait()
        wait(d_out(base, TQ, sem.at[SEM_OUT2]))
        out_buf[pl.ds(g1, 8), :] = o1
        out_buf[pl.ds(g2, 8), :] = o2
        start(d_out(g1, 8, sem.at[SEM_FIX]))

        @pl.when(g1 != g2)
        def _():
            start(d_out(g2, 8, sem.at[SEM_FIX + 1]))
            wait(d_out(g2, 8, sem.at[SEM_FIX + 1]))

        wait(d_out(g1, 8, sem.at[SEM_FIX]))
        return 0
    jax.lax.fori_loop(0, zero0 + 1, rest, 0)


@jax.jit
def pallas_adaLN_cond__mha_block_cached__moe_arch_mod__prompt_kernel(
    A_x: jax.Array,
    A_k_cache: jax.Array,
    A_v_cache: jax.Array,
    A_wq: jax.Array,
    A_wo: jax.Array,
    B_x: jax.Array,
    B_w_r: jax.Array,
    B_w_gate: jax.Array,
    B_w_up: jax.Array,
    B_w_down: jax.Array,
    c: jax.Array,
    w_mod: jax.Array,
):
    del B_x
    vm = pltpu.VMEM
    scratch = [
        vm((S + PC, D), BF16),
        vm((2, TQ // 2, D), U32),
        vm((H, S, DH), BF16),
        vm((H, S, DH), BF16),
        vm((H, D, DH), BF16),
        vm((H * DH, D), BF16),
        vm((D, FF), BF16),
        vm((D, FF), BF16),
        vm((FF, D + 128), BF16),
        vm((D, 6 * D + 128), BF16),
        vm((1, D), BF16),
        vm((8, 128), BF16),
        vm((8, 7 * D), F32),
        vm((2, TQ, D), F32),
        vm((S, D), BF16),
        vm((TU, S), F32),
        vm((TU, DH), F32),
        vm((TU, DH), F32),
        vm((2, 8, 128), I32),
        vm((2, TQ, 128), F32),
        pltpu.SemaphoreType.DMA((NSEM,)),
    ]
    anyspec = pl.BlockSpec(memory_space=pl.ANY)
    return pl.pallas_call(
        _kernel,
        in_specs=[anyspec] * 11,
        out_specs=anyspec,
        out_shape=jax.ShapeDtypeStruct((1, S, D), BF16),
        scratch_shapes=scratch,
        compiler_params=pltpu.CompilerParams(vmem_limit_bytes=120 * 1024 * 1024, disable_bounds_checks=True,
                                             disable_semaphore_checks=True),
    )(A_x, A_k_cache, A_v_cache, A_wq, A_wo, B_w_r.reshape(8, 128), B_w_gate, B_w_up, B_w_down, c, w_mod)
```

```python
import functools

import jax
import jax.numpy as jnp
import jax.experimental.pallas as pl
import jax.experimental.pallas.tpu as pltpu

F32, BF16, U32, I32 = jnp.float32, jnp.bfloat16, jnp.uint32, jnp.int32

S, D, H, DH, FF = 2048, 1024, 32, 128, 3584
TU = 256
TQ = 512
NQ = S // TQ
HP = 6
NM = 7
NT = (NQ * H - 1 - NM) // HP
NG = (H - 1 - NM) // HP
PC = 16
RC = 16
AC = 2
AC0 = 8
AC1 = 2
ACM0 = 8
ACM1 = 1
ACP = 1
ACT = 3
WMC = 2
EPS = 1e-5
QSCALE = DH ** -0.5 * 1.4426950408889634
KMIN = -2 ** 31
CPC = 32
CSPAN = 40
FHR = 16
FSPAN = 60
FN0 = 20
FSPAN1 = 32
TPC = 64

SEM_SMALL = 0
SEM_X = 1
SEM_X1A = 5
SEM_WM = 6
SEM_WMR = 10
SEM_WQ0 = 11
SEM_KV0 = 12
SEM_FFN = 13
SEM_OUT = 14
SEM_FIX = 15
SEM_OUT2 = 17
SEM_V0 = 18
SEM_X0B = 19
SEM_MINI = 20
SEM_GRP = SEM_MINI + NM + 1
SEM_QP = SEM_GRP + NG
NQP = (NM + 1) // 2
NSEM = SEM_QP + NQP


def _rb(x):
    return x.astype(BF16).astype(F32)


def _ub(x):
    return pltpu.bitcast(x, BF16)


def _pk(x):
    return pltpu.bitcast(x, U32)


def _recip(l):
    r = pl.reciprocal(l, approx=True)
    return r * (2.0 - l * r)


def _ln(x):
    mu = jnp.sum(x, axis=-1, keepdims=True) * (1.0 / D)
    d = x - mu
    var = jnp.sum(d * d, axis=-1, keepdims=True) * (1.0 / D)
    return d * jax.lax.rsqrt(var + EPS)


def _stats(x):
    mu = jnp.sum(x, axis=-1, keepdims=True) * (1.0 / D)
    var = jnp.maximum(jnp.sum(x * x, axis=-1, keepdims=True) * (1.0 / D) - mu * mu, 0.0)
    return mu, jax.lax.rsqrt(var + EPS)


def _kernel(x_hbm, k_hbm, v_hbm, wq_hbm, wo_hbm, wr_hbm, wg_hbm, wu_hbm, wd_hbm, c_hbm, wm_hbm,
            out_hbm,
            x_buf, h_buf, k_buf, v_buf, wq_buf, wo_buf, wg_buf, wu_buf, wd_buf, wm_buf,
            c_buf, wr_buf, mod_buf, acc, out_buf, s_sc, of_sc, l_sc, r_buf, st_buf, qa_buf, b_buf, on_sc, n_buf, sem):
    cp = pltpu.make_async_copy

    def d_small():
        return [cp(c_hbm, c_buf, sem.at[SEM_SMALL]), cp(wr_hbm, wr_buf, sem.at[SEM_SMALL])]

    def d_xrows(r0, n, s_):
        return [cp(x_hbm.at[0, pl.ds(r0, n), :], x_buf.at[pl.ds(r0, n), :], s_)]

    X1A = 128

    def d_x(j):
        if j == 1:
            return d_xrows(TQ + X1A, TQ - X1A, sem.at[SEM_X + 1])
        return d_xrows(j * TQ, TQ, sem.at[SEM_X + j])

    def d_x1a():
        return d_xrows(TQ, X1A, sem.at[SEM_X1A])

    WC = D // WMC

    def d_wm(i):
        return [cp(wm_hbm.at[:, pl.ds(D + i * WC, WC)], wm_buf.at[:, pl.ds(D + i * WC, WC)], sem.at[SEM_WM + i])]

    def d_sa():
        return [cp(wm_hbm.at[:, pl.ds(0, D)], wm_buf.at[:, pl.ds(0, D)], sem.at[SEM_WQ0])]

    def d_wq2(i):
        rows = pl.ds(pl.multiple_of((i >> 1) * WC, WC), WC)
        return [cp(wq_hbm.at[rows, pl.ds(pl.multiple_of((4 * (i & 1) + k) * DH, DH), DH)],
                   wq_buf.at[4 * (i & 1) + k, rows, :], sem.at[SEM_QP + i]) for k in range(4)]

    def d_wmr():
        return [cp(wm_hbm.at[:, pl.ds(2 * D, 4 * D)], wm_buf.at[:, pl.ds(2 * D, 4 * D)], sem.at[SEM_WMR])]

    def d_wq(h0, n, s_):
        return [cp(wq_hbm.at[:, pl.ds(pl.multiple_of((h0 + i) * DH, DH), DH)], wq_buf.at[h0 + i], s_)
                for i in range(n)]

    def d_k(h0, n, s_):
        return [cp(k_hbm.at[0, pl.ds(h0, n)], k_buf.at[pl.ds(h0, n)], s_)]

    def d_v(h0, n, s_):
        return [cp(v_hbm.at[0, pl.ds(h0, n)], v_buf.at[pl.ds(h0, n)], s_)]

    def d_wo(h0, n, s_):
        rows = pl.ds(pl.multiple_of(h0 * DH, DH), n * DH)
        return [cp(wo_hbm.at[rows, :], wo_buf.at[rows, :], s_)]

    def d_mini(i):
        s_ = sem.at[SEM_MINI + i]
        return d_wo(i - 1, 1, s_) + d_k(i, 1, s_) + d_v(i, 1, s_)

    def d_grp(t):
        s_ = sem.at[SEM_GRP + t]
        h0 = HP * t + NM + 1
        return d_wq(h0, HP, s_) + d_wo(h0 - 1, HP, s_) + d_k(h0, HP, s_) + d_v(h0, HP, s_)

    def d_late():
        return d_wmr() + d_wo(H - 1, 1, sem.at[SEM_WMR])

    def d_ffn(i):
        src, dst = ((wg_hbm, wg_buf), (wu_hbm, wu_buf), (wd_hbm, wd_buf.at[:, pl.ds(0, D)]))[i]
        return [cp(src, dst, sem.at[SEM_FFN])]

    def d_out(r0, n, s_):
        return [cp(out_buf.at[pl.ds(r0, n), :], out_hbm.at[0, pl.ds(r0, n), :], s_)]

    def start(ds):
        for d in ds:
            d.start()

    def wait(ds):
        for d in ds:
            d.wait()

    def qp(unit, anchor=False, zero=None):
        hh, sub, par = unit
        hb = h_buf[par, sub * (TU // 2):(sub + 1) * (TU // 2), :]
        if anchor:
            z16 = pl.multiple_of(zero * 16, 16)
            d0 = _pk(out_buf[pl.ds(z16, 16), 0:128])
            d1 = pltpu.bitcast(r_buf[zero], U32)
            d2 = _pk(x_buf[pl.ds(z16, 16), 0:128])
            top = jnp.concatenate([jnp.where(zero > 0, d0, hb[0:8, 0:128]),
                                   jnp.where(zero > 0, d1, hb[0:8, 128:256]),
                                   jnp.where(zero > 0, d2, hb[0:8, 256:384]), hb[0:8, 384:]], axis=1)
            hb = jnp.concatenate([top, hb[8:]], axis=0)
        q = jnp.dot(_ub(hb), wq_buf[hh], preferred_element_type=F32)
        return (q * QSCALE).astype(BF16)

    def qk(unit, q):
        hh, sub, par = unit
        return jax.lax.dot_general(q, k_buf[hh], (((1,), (1,)), ((), ())), preferred_element_type=F32)

    def softmax(s, zero, AC=AC):
        ls, ps = [], []
        nc = S // 128
        for c in range(TU // RC):
            sc = s[c * RC:(c + 1) * RC, :]
            m = jnp.max(sc, axis=-1, keepdims=True)
            p = jnp.exp2(sc - m)
            cols = [p[:, i * 128:(i + 1) * 128] for i in range(nc)]
            a = cols[0]
            for i in range(1, nc):
                if i == nc - AC:
                    part = a
                a = a + cols[i]
            if AC:
                cols[nc - AC] = jnp.where(zero > 0, part, cols[nc - AC])
            ls.append(a)
            ps.append(jnp.concatenate(cols, axis=1))
        return jnp.concatenate(ps, axis=0).astype(BF16), jnp.concatenate(ls, axis=0)

    def pv(unit, s, zero, ac=AC):
        hh, sub, par = unit
        pb, lp = softmax(s, zero, ac)
        return jnp.dot(pb, v_buf[hh], preferred_element_type=F32), lp

    def fin(ol):
        return (ol[0] * _recip(jnp.sum(ol[1], axis=-1, keepdims=True))).astype(BF16)

    def outp(unit, ol):
        hh, sub, par = unit
        o = fin(ol) if isinstance(ol, tuple) else ol
        w = wo_buf[pl.ds(pl.multiple_of(hh * DH, DH), DH), :]
        acc[par, sub * TU:(sub + 1) * TU, :] += jnp.dot(o, w, preferred_element_type=F32)

    def modrow(i):
        return mod_buf[:, i * D:(i + 1) * D][None]

    def ln1_stats(xrow0, n, zero):
        x = x_buf[pl.ds(xrow0, n), :].astype(F32)
        d = acc[zero, pl.ds(pl.multiple_of(zero * 8, 8), n), 0:128]
        x = jnp.concatenate([jnp.where(zero > 0, d, x[:, 0:128]), x[:, 128:]], axis=1).reshape(n // 8, 8, D)
        return _stats(x)

    def ln1(xrow0, par, hrow0, n, onepass, stats=None):
        x = x_buf[pl.ds(xrow0, n), :].astype(F32).reshape(n // 8, 8, D)
        if stats is None and onepass:
            stats = _stats(x)
        nrm = _ln(x) if stats is None else (x - stats[0]) * stats[1]
        h = (nrm * modrow(1) + modrow(0)).reshape(n, D)
        h_buf[par, pl.ds(hrow0, n // 2), :] = _pk(h.astype(BF16))

    def top2_update(r, row0, valid):
        b = pltpu.bitcast(r, I32)
        key = (b ^ ((b >> 31) & 0x7FFFFFFF)) | (S - 1)
        rid = jax.lax.broadcasted_iota(I32, (8, 128), 0) + row0
        best, second = r_buf[0], r_buf[1]
        for i in range(r.shape[0]):
            k = key[i] - (rid + 8 * i)
            if valid is not None:
                k = jnp.where(valid, k, KMIN)
            second = jnp.maximum(second, jnp.minimum(best, k))
            best = jnp.maximum(best, k)
        r_buf[0] = best
        r_buf[1] = second

    def epi(row0, par, arow0, n, valid):
        a = acc[par, pl.ds(arow0, n), :].reshape(n // 8, 8, D)
        acc[par, pl.ds(arow0, n), :] = jnp.zeros((n, D), F32)
        x1 = x_buf[pl.ds(row0, n), :].astype(F32).reshape(n // 8, 8, D) + modrow(2) * a
        d = x1 - jnp.sum(x1, axis=-1, keepdims=True) * (1.0 / D)
        rstd = jax.lax.rsqrt(jnp.sum(d * d, axis=-1, keepdims=True) * (1.0 / D) + EPS)
        h2 = d * rstd * modrow(4) + modrow(3)
        x_buf[pl.ds(pl.multiple_of(jnp.where(valid, row0, S), n), n), :] = h2.reshape(n, D).astype(BF16)
        out_buf[pl.ds(row0, n), :] = (x1 + modrow(5) * h2).reshape(n, D).astype(BF16)
        r = jnp.sum(h2 * modrow(6), axis=-1, keepdims=True)
        top2_update(jnp.broadcast_to(r, (n // 8, 8, 128)), row0, valid)

    def epi_a(row0, par, arow0, n, u, su, c0):
        a = acc[par, arow0:arow0 + n, :].reshape(n // 8, 8, D)
        x1 = x_buf[row0:row0 + n, :].astype(F32).reshape(n // 8, 8, D) + modrow(2) * a
        acc[par, arow0:arow0 + n, :] = x1.reshape(n, D)
        mu, rstd = [jnp.broadcast_to(v, (n // 8, 8, 128)) for v in _stats(x1)]
        st_buf[0, arow0:arow0 + n, :] = mu.reshape(n, 128)
        st_buf[1, arow0:arow0 + n, :] = rstd.reshape(n, 128)
        xu = jnp.sum(x1 * u, axis=-1, keepdims=True)
        top2_update((xu - mu * su) * rstd + c0, row0, None)

    def last_norm(par, arow0, n):
        x1 = acc[par, pl.ds(arow0, n), :].reshape(n // 8, 8, D)
        mu = jnp.concatenate([st_buf[0, pl.ds(arow0, n), :]] * 8, axis=1).reshape(n // 8, 8, D)
        rstd = jnp.concatenate([st_buf[1, pl.ds(arow0, n), :]] * 8, axis=1).reshape(n // 8, 8, D)
        return x1, (x1 - mu) * rstd

    def run_units(seq, side, zero, acs={}):
        s = s_sc[...]
        ol_prev = (of_sc[...], l_sc[...])
        for u in range(len(seq) - 2):
            q = qp(seq[u + 2], u > 0 and side[u - 1][1], zero)
            ol = pv(seq[u + 1], s, zero, acs.get(u, AC))
            outp(seq[u], ol_prev)
            ol_prev = ol
            side[u][0](q)
            s = qk(seq[u + 2], q)
        s_sc[...] = s
        of_sc[...] = ol_prev[0]
        l_sc[...] = ol_prev[1]

    def mod_cols(c0, n):
        cf = c_buf[...].astype(F32)
        sc = (cf * jax.nn.sigmoid(cf)).astype(BF16)
        sc = jnp.broadcast_to(sc, (16, D))
        m = jnp.dot(sc, wm_buf[:, c0:c0 + n], preferred_element_type=F32)
        return _rb(m[0:8, :])

    start(d_small())
    start(d_xrows(0, TU, sem.at[SEM_X]))
    start(d_xrows(TU, TU, sem.at[SEM_X0B]))
    for i in range(NQP):
        if i % 2 == 0:
            start(d_wm(i // 2))
        start(d_wq2(i))
    start(d_sa())
    start(d_k(0, 1, sem.at[SEM_KV0]) + d_v(0, 1, sem.at[SEM_V0]))
    start(d_mini(1))
    start(d_x1a())
    for i in range(2, NM + 1):
        start(d_mini(i))
    start(d_x(1))
    start(d_grp(0))
    acc[...] = jnp.zeros(acc.shape, F32)
    mod_buf[...] = jnp.zeros(mod_buf.shape, F32)
    r_buf[...] = jnp.full(r_buf.shape, KMIN, I32)
    out_buf[0:16, :] = jnp.zeros((16, D), BF16)
    on_sc[...] = jnp.zeros(on_sc.shape, U32)
    qa_buf[...] = jnp.zeros(qa_buf.shape, F32)

    zero0 = r_buf[0, 0, 0] & 1

    def rest(_i, _c):
        wait(d_small())
        wr = wr_buf[...].astype(F32)
        for i in range(8):
            mod_buf[:, 6 * D + i * 128:6 * D + (i + 1) * 128] = jnp.broadcast_to(wr[i:i + 1, :], (8, 128))
        wait(d_xrows(0, TU, sem.at[SEM_X]))

        def norm_first(i, _):
            @pl.when(i == TU // 64)
            def _():
                wait(d_xrows(TU, TU, sem.at[SEM_X0B]))
            for half in range(2):
                r0 = pl.multiple_of(i * 64 + half * 32, 32)
                n_buf[pl.ds(r0, 32), :] = _ln(x_buf[pl.ds(r0, 32), :].astype(F32))
            return 0
        jax.lax.fori_loop(0, TQ // 64, norm_first, 0)

        def qp_first(i, _):
            for c in range(WMC):
                @pl.when(i == 2 * c)
                def _():
                    wait(d_wm(c))
                    ca = _rb(1.0 + mod_cols(D + c * WC, WC))
                    mod_buf[:, D + c * WC:D + (c + 1) * WC] = ca
                    for half in range(2):
                        nv = n_buf[half * TU:(half + 1) * TU, c * WC:(c + 1) * WC].reshape(TU // 8, 8, WC) * ca[None]
                        h_buf[0, half * (TU // 2):(half + 1) * (TU // 2), 0:WC] = _pk(nv.reshape(TU, WC).astype(BF16))
            wait(d_wq2(i))
            rows = pl.ds(pl.multiple_of((i >> 1) * WC, WC), WC)
            for k in range(4):
                hh = 4 * (i & 1) + k
                for sub in range(2):
                    hb = _ub(h_buf[0, sub * (TU // 2):(sub + 1) * (TU // 2), 0:WC])
                    qa_buf[hh, sub * TU:(sub + 1) * TU, :] += jnp.dot(
                        hb, wq_buf[hh, rows, :], preferred_element_type=F32)
            return 0
        jax.lax.fori_loop(0, NQP, qp_first, 0)

        def q_first(hh, sub):
            qa = qa_buf[hh, sub * TU:(sub + 1) * TU, :].reshape(TU // 8, 8, DH)
            return ((qa + b_buf[hh][None]) * QSCALE).reshape(TU, DH).astype(BF16)
        wait(d_sa())
        sa = mod_cols(0, D)
        mod_buf[:, 0:D] = sa
        sab = jnp.concatenate([sa, sa], axis=0).astype(BF16)
        for hh in range(NM + 1):
            b_buf[hh] = jnp.dot(sab, wq_buf[hh], preferred_element_type=F32)[0:8]
        wait(d_k(0, 1, sem.at[SEM_KV0]))
        s0 = qk((0, 0, 0), q_first(0, 0))
        npc_ = TQ // FHR

        def h_piece(k, src, pos):
            r_, c_ = (pos % 16) * 16, (pos // 16) * 512
            z = jnp.where(zero0 > 0, pltpu.bitcast(src[r_:r_ + 8, c_:c_ + 128], I32)[0, 0], 0)
            zr = pl.multiple_of(jnp.clip(z + k, 0, npc_ - 1) * FHR, FHR)
            nv = n_buf[pl.ds(zr, FHR), :].reshape(FHR // 8, 8, D) * modrow(1) + modrow(0)
            h_buf[0, k * FHR // 2:(k + 1) * FHR // 2, :] = _pk(nv.reshape(FHR, D).astype(BF16))
        for k in range(FN0):
            h_piece(k, s0, (k * FSPAN) // FN0)
        wait(d_v(0, 1, sem.at[SEM_V0]))
        s1 = qk((0, 1, 0), q_first(0, 1))
        s_sc[...] = s1
        for k in range(FN0, npc_):
            h_piece(k, s1, ((k - FN0) * FSPAN1) // (npc_ - FN0))
        o0, l0 = pv((0, 0, 0), s0, zero0, ACP)
        of_sc[...] = o0
        l_sc[...] = l0

        def mini(i, _):
            wait(d_mini(i))

            @pl.when(i == 2)
            def _():
                wait(d_x1a())
            zero = i >> 10

            def piece(u):
                pc = jnp.minimum(2 * (i - 2) + u, NM)
                ln1(pl.multiple_of(TQ + pc * PC, PC), 1,
                    pl.multiple_of(jnp.maximum(pc, 0) * (PC // 2), PC // 2), PC, False)
            outp((jnp.maximum(i - 2, 0), 1, 0), _ub(on_sc[...]))
            ola = pv((i - 1, 1, 0), s_sc[...], zero, ACM0)
            piece(0)
            s = qk((i, 0, 0), q_first(i, 0))
            outp((i - 1, 0, 0), (of_sc[...], l_sc[...]))
            ol = pv((i, 0, 0), s, zero, ACM1)
            piece(1)
            s_sc[...] = qk((i, 1, 0), q_first(i, 1))
            on_sc[...] = _pk(fin(ola))
            of_sc[...] = ol[0]
            l_sc[...] = ol[1]
            return 0
        jax.lax.fori_loop(1, NM + 1, mini, 0)
        outp((NM - 1, 1, 0), _ub(on_sc[...]))
        for t in range(1, NG):
            start(d_grp(t))
        start(d_late())
        start(d_x(2))
        start(d_x(3))
        for i in range(3):
            start(d_ffn(i))

        def main(t, _):
            @pl.when(t < NG)
            def _():
                wait(d_grp(t))

            @pl.when(t == 0)
            def _():
                wait(d_x(1))

            @pl.when(t == NG)
            def _():
                wait(d_late())
                wait(d_x(2))
                wait(d_x(3))
                for i in range(3):
                    wait(d_ffn(i))
                for i in range(2, 6):
                    m = mod_cols(i * D, D)
                    if i == 4:
                        m = _rb(1.0 + m)
                    mod_buf[:, i * D:(i + 1) * D] = m

            @pl.when(t > NG)
            def _():
                start(d_out(pl.multiple_of((t - 1 - NG) * (HP * PC), PC), HP * PC, sem.at[SEM_OUT]))

            p0 = t * HP + NM + 1
            zero = t >> 10
            seq, side, stats = [], [], {}
            pairs = [((p0 + k) & (H - 1), (p0 + k) >> 5) for k in range(-1, HP)]
            for hh, j in pairs:
                seq += [(hh, 0, j & 1), (hh, 1, j & 1)]

            def xnext(k):
                hh, j = pairs[k + 1]
                return pl.multiple_of(jnp.minimum(j + 1, NQ - 1) * TQ + hh * PC, PC)

            def ln1_piece(k, q):
                hh, j = pairs[k + 1]
                st = stats.get(k)
                if st is not None:
                    mu = jnp.where(zero > 0, q[0:PC].astype(F32).reshape(PC // 8, 8, 128),
                                   jnp.broadcast_to(st[0], (PC // 8, 8, 128)))
                    st = (jnp.concatenate([mu] * 8, axis=2), st[1])
                ln1(xnext(k), 1 - (j & 1), pl.multiple_of(hh * (PC // 2), PC // 2), PC, True, st)

            def epi_piece(k, q):
                hh, j = pairs[k + 1]
                if k + 1 < HP:
                    stats[k + 1] = ln1_stats(xnext(k + 1), PC, zero)
                epi(pl.multiple_of(jnp.maximum(j - 1, 0) * TQ + hh * PC, PC), 1 - (j & 1),
                    pl.multiple_of(hh * PC, PC), PC, j > 0)

            for k in range(HP):
                side += [(functools.partial(ln1_piece, k), False), (functools.partial(epi_piece, k), True)]
            run_units(seq, side, zero, {0: AC0, 1: AC1})
            return 0
        jax.lax.fori_loop(0, NT, main, 0)

        start(d_out((NT - 1 - NG) * HP * PC, HP * PC, sem.at[SEM_OUT]))
        lastp = (NQ - 1) & 1
        base = (NQ - 1) * TQ
        ru = modrow(4) * modrow(6)
        rsu = jnp.sum(ru, axis=-1, keepdims=True)
        rc0 = jnp.sum(modrow(3) * modrow(6), axis=-1, keepdims=True)

        def epis(half):
            for i in range(half * TU // TPC, (half + 1) * TU // TPC):
                epi_a(base + i * TPC, lastp, i * TPC, TPC, ru, rsu, rc0)
        ol = pv((H - 1, 1, lastp), s_sc[...], zero0, ACT)
        outp((H - 1, 0, lastp), (of_sc[...], l_sc[...]))
        outp((H - 1, 1, lastp), ol)
        epis(0)
        epis(1)
        best, second = r_buf[0], r_buf[1]
        for sh in (4, 2, 1):
            b2 = pltpu.roll(best, sh, 0)
            s2 = pltpu.roll(second, sh, 0)
            second = jnp.maximum(jnp.minimum(best, b2), jnp.maximum(second, s2))
            best = jnp.maximum(best, b2)
        i1 = (S - 1) - (best[0, 0] & (S - 1))
        i2 = (S - 1) - (second[0, 0] & (S - 1))
        g1 = pl.multiple_of(jnp.clip(i1 >> 3, 0, S // 8 - 1) * 8, 8)
        g2 = pl.multiple_of(jnp.clip(i2 >> 3, 0, S // 8 - 1) * 8, 8)

        def h2_rows(g):
            nrm = last_norm(lastp, pl.multiple_of(jnp.clip(g - base, 0, TQ - 8), 8), 8)[1]
            last = (nrm * modrow(4) + modrow(3)).reshape(8, D)
            return jnp.where(g >= base, last, x_buf[pl.ds(g, 8), :].astype(F32))
        xs = jnp.concatenate([h2_rows(g1), h2_rows(g2)], axis=0).astype(BF16)
        gt = jnp.dot(xs, wg_buf[...], preferred_element_type=F32)
        up = jnp.dot(xs, wu_buf[...], preferred_element_type=F32)
        gbits = pltpu.bitcast(jnp.concatenate([gt, up], axis=1), I32)
        ga_, gb_ = modrow(5) * modrow(4), modrow(5) * modrow(3)
        npc = TQ // CPC
        for i in range(npc):
            z = jnp.where(i1 < 0, gbits[0, 128 * (i * CSPAN // npc)], 0)
            x1, nrm = last_norm(lastp, pl.multiple_of(jnp.clip(z + i, 0, npc - 1) * CPC, CPC), CPC)
            out_buf[base + i * CPC:base + (i + 1) * CPC, :] = (x1 + nrm * ga_ + gb_).reshape(CPC, D).astype(BF16)
            if i == npc // 2 - 1:
                start(d_out(base, TU, sem.at[SEM_OUT2]))
        start(d_out(base + TU, TU, sem.at[SEM_OUT2]))
        gt = _rb(gt)
        a = (_rb(gt * jax.nn.sigmoid(gt)) * _rb(up)).astype(BF16)
        y = _rb(jnp.dot(a, wd_buf[:, 0:D], preferred_element_type=F32))

        def score(k):
            return pltpu.bitcast((k ^ ((k >> 31) & 0x7FFFFFFF)) & -S, F32)
        ri = jax.lax.broadcasted_iota(I32, (16, 128), 0)
        rows = jnp.where(ri < 8, g1 + ri, g2 + ri - 8)
        r1 = jnp.concatenate([score(best)] * 2, axis=0)
        r2 = jnp.concatenate([score(second)] * 2, axis=0)
        gate = _rb(jax.nn.sigmoid(_rb(jnp.where(rows == i1, r1, r2))))
        sel = (rows == i1) | (rows == i2)
        upd = jnp.where(sel[:, 0:1], _rb(y * gate[:, 0:1]), 0.0) * mod_buf[0:1, 5 * D:6 * D]
        o1 = (out_buf[pl.ds(g1, 8), :].astype(F32) + upd[0:8]).astype(BF16)
        o2 = (out_buf[pl.ds(g2, 8), :].astype(F32) + upd[8:16]).astype(BF16)
        cp(out_buf.at[pl.ds(0, base), :], out_hbm.at[0, pl.ds(0, base), :], sem.at[SEM_OUT]).wait()
        wait(d_out(base, TQ, sem.at[SEM_OUT2]))
        out_buf[pl.ds(g1, 8), :] = o1
        out_buf[pl.ds(g2, 8), :] = o2
        start(d_out(g1, 8, sem.at[SEM_FIX]))

        @pl.when(g1 != g2)
        def _():
            start(d_out(g2, 8, sem.at[SEM_FIX + 1]))
            wait(d_out(g2, 8, sem.at[SEM_FIX + 1]))

        wait(d_out(g1, 8, sem.at[SEM_FIX]))
        return 0
    jax.lax.fori_loop(0, zero0 + 1, rest, 0)


@jax.jit
def pallas_adaLN_cond__mha_block_cached__moe_arch_mod__prompt_kernel(
    A_x: jax.Array,
    A_k_cache: jax.Array,
    A_v_cache: jax.Array,
    A_wq: jax.Array,
    A_wo: jax.Array,
    B_x: jax.Array,
    B_w_r: jax.Array,
    B_w_gate: jax.Array,
    B_w_up: jax.Array,
    B_w_down: jax.Array,
    c: jax.Array,
    w_mod: jax.Array,
):
    del B_x
    vm = pltpu.VMEM
    scratch = [
        vm((S + PC, D), BF16),
        vm((2, TQ // 2, D), U32),
        vm((H, S, DH), BF16),
        vm((H, S, DH), BF16),
        vm((H, D, DH), BF16),
        vm((H * DH, D), BF16),
        vm((D, FF), BF16),
        vm((D, FF), BF16),
        vm((FF, D + 128), BF16),
        vm((D, 6 * D + 128), BF16),
        vm((1, D), BF16),
        vm((8, 128), BF16),
        vm((8, 7 * D), F32),
        vm((2, TQ, D), F32),
        vm((S, D), BF16),
        vm((TU, S), F32),
        vm((TU, DH), F32),
        vm((TU, DH), F32),
        vm((2, 8, 128), I32),
        vm((2, TQ, 128), F32),
        vm((NM + 1, TQ, DH), F32),
        vm((NM + 1, 8, DH), F32),
        vm((TU // 2, DH), U32),
        vm((TQ, D), F32),
        pltpu.SemaphoreType.DMA((NSEM,)),
    ]
    anyspec = pl.BlockSpec(memory_space=pl.ANY)
    return pl.pallas_call(
        _kernel,
        in_specs=[anyspec] * 11,
        out_specs=anyspec,
        out_shape=jax.ShapeDtypeStruct((1, S, D), BF16),
        scratch_shapes=scratch,
        compiler_params=pltpu.CompilerParams(vmem_limit_bytes=120 * 1024 * 1024, disable_bounds_checks=True,
                                             disable_semaphore_checks=True),
    )(A_x, A_k_cache, A_v_cache, A_wq, A_wo, B_w_r.reshape(8, 128), B_w_gate, B_w_up, B_w_down, c, w_mod)
```

```python
import functools

import jax
import jax.numpy as jnp
import jax.experimental.pallas as pl
import jax.experimental.pallas.tpu as pltpu

F32, BF16, U32, I32 = jnp.float32, jnp.bfloat16, jnp.uint32, jnp.int32

S, D, H, DH, FF = 2048, 1024, 32, 128, 3584
TU = 256
TQ = 512
NQ = S // TQ
HP = 6
NM = 7
NT = (NQ * H - 1 - NM) // HP
NG = (H - 1 - NM) // HP
PC = 16
RC = 16
AC = 2
AC0 = 8
AC1 = 2
ACM0 = 8
ACM1 = 1
ACP = 1
ACT = 3
WMC = 2
EPS = 1e-5
QSCALE = DH ** -0.5 * 1.4426950408889634
KMIN = -2 ** 31
CPC = 32
CSPAN = 40
FHR = 16
FSPAN = 60
FN0 = 20
FSPAN1 = 32
ACP1 = 2
ACH = 1
TPC = 64

SEM_SMALL = 0
SEM_X = 1
SEM_X1A = 5
SEM_WM = 6
SEM_WMR = 10
SEM_WQ0 = 11
SEM_KV0 = 12
SEM_FFN = 13
SEM_OUT = 14
SEM_FIX = 15
SEM_OUT2 = 17
SEM_V0 = 18
SEM_X0B = 19
SEM_MINI = 20
SEM_GRP = SEM_MINI + NM + 1
SEM_QP = SEM_GRP + NG
NQP = (NM + 1) // 2
NSEM = SEM_QP + NQP


def _rb(x):
    return x.astype(BF16).astype(F32)


def _ub(x):
    return pltpu.bitcast(x, BF16)


def _pk(x):
    return pltpu.bitcast(x, U32)


def _recip(l):
    r = pl.reciprocal(l, approx=True)
    return r * (2.0 - l * r)


def _ln(x):
    mu = jnp.sum(x, axis=-1, keepdims=True) * (1.0 / D)
    d = x - mu
    var = jnp.sum(d * d, axis=-1, keepdims=True) * (1.0 / D)
    return d * jax.lax.rsqrt(var + EPS)


def _stats(x):
    mu = jnp.sum(x, axis=-1, keepdims=True) * (1.0 / D)
    var = jnp.maximum(jnp.sum(x * x, axis=-1, keepdims=True) * (1.0 / D) - mu * mu, 0.0)
    return mu, jax.lax.rsqrt(var + EPS)


def _kernel(x_hbm, k_hbm, v_hbm, wq_hbm, wo_hbm, wr_hbm, wg_hbm, wu_hbm, wd_hbm, c_hbm, wm_hbm,
            out_hbm,
            x_buf, h_buf, k_buf, v_buf, wq_buf, wo_buf, wg_buf, wu_buf, wd_buf, wm_buf,
            c_buf, wr_buf, mod_buf, acc, out_buf, s_sc, of_sc, l_sc, r_buf, st_buf, qa_buf, b_buf, on_sc, n_buf, sem):
    cp = pltpu.make_async_copy

    def d_small():
        return [cp(c_hbm, c_buf, sem.at[SEM_SMALL]), cp(wr_hbm, wr_buf, sem.at[SEM_SMALL])]

    def d_xrows(r0, n, s_):
        return [cp(x_hbm.at[0, pl.ds(r0, n), :], x_buf.at[pl.ds(r0, n), :], s_)]

    X1A = 128

    def d_x(j):
        if j == 1:
            return d_xrows(TQ + X1A, TQ - X1A, sem.at[SEM_X + 1])
        return d_xrows(j * TQ, TQ, sem.at[SEM_X + j])

    def d_x1a():
        return d_xrows(TQ, X1A, sem.at[SEM_X1A])

    WC = D // WMC

    def d_wm(i):
        return [cp(wm_hbm.at[:, pl.ds(D + i * WC, WC)], wm_buf.at[:, pl.ds(D + i * WC, WC)], sem.at[SEM_WM + i])]

    def d_sa():
        return [cp(wm_hbm.at[:, pl.ds(0, D)], wm_buf.at[:, pl.ds(0, D)], sem.at[SEM_WQ0])]

    def d_wq2(i):
        rows = pl.ds(pl.multiple_of((i >> 1) * WC, WC), WC)
        return [cp(wq_hbm.at[rows, pl.ds(pl.multiple_of((4 * (i & 1) + k) * DH, DH), DH)],
                   wq_buf.at[4 * (i & 1) + k, rows, :], sem.at[SEM_QP + i]) for k in range(4)]

    def d_wmr():
        return [cp(wm_hbm.at[:, pl.ds(2 * D, 4 * D)], wm_buf.at[:, pl.ds(2 * D, 4 * D)], sem.at[SEM_WMR])]

    def d_wq(h0, n, s_):
        return [cp(wq_hbm.at[:, pl.ds(pl.multiple_of((h0 + i) * DH, DH), DH)], wq_buf.at[h0 + i], s_)
                for i in range(n)]

    def d_k(h0, n, s_):
        return [cp(k_hbm.at[0, pl.ds(h0, n)], k_buf.at[pl.ds(h0, n)], s_)]

    def d_v(h0, n, s_):
        return [cp(v_hbm.at[0, pl.ds(h0, n)], v_buf.at[pl.ds(h0, n)], s_)]

    def d_wo(h0, n, s_):
        rows = pl.ds(pl.multiple_of(h0 * DH, DH), n * DH)
        return [cp(wo_hbm.at[rows, :], wo_buf.at[rows, :], s_)]

    def d_mini(i):
        s_ = sem.at[SEM_MINI + i]
        return d_wo(i - 1, 1, s_) + d_v(i, 1, s_) + d_k(i + 1, 1, s_)

    def d_hand():
        s_ = sem.at[SEM_MINI + NM]
        return d_wo(NM - 1, 1, s_) + d_v(NM, 1, s_)

    def d_grp(t):
        s_ = sem.at[SEM_GRP + t]
        h0 = HP * t + NM + 1
        return d_wq(h0, HP, s_) + d_wo(h0 - 1, HP, s_) + d_k(h0, HP, s_) + d_v(h0, HP, s_)

    def d_late():
        return d_wmr() + d_wo(H - 1, 1, sem.at[SEM_WMR])

    def d_ffn(i):
        src, dst = ((wg_hbm, wg_buf), (wu_hbm, wu_buf), (wd_hbm, wd_buf.at[:, pl.ds(0, D)]))[i]
        return [cp(src, dst, sem.at[SEM_FFN])]

    def d_out(r0, n, s_):
        return [cp(out_buf.at[pl.ds(r0, n), :], out_hbm.at[0, pl.ds(r0, n), :], s_)]

    def start(ds):
        for d in ds:
            d.start()

    def wait(ds):
        for d in ds:
            d.wait()

    def qp(unit, anchor=False, zero=None):
        hh, sub, par = unit
        hb = h_buf[par, sub * (TU // 2):(sub + 1) * (TU // 2), :]
        if anchor:
            z16 = pl.multiple_of(zero * 16, 16)
            d0 = _pk(out_buf[pl.ds(z16, 16), 0:128])
            d1 = pltpu.bitcast(r_buf[zero], U32)
            d2 = _pk(x_buf[pl.ds(z16, 16), 0:128])
            top = jnp.concatenate([jnp.where(zero > 0, d0, hb[0:8, 0:128]),
                                   jnp.where(zero > 0, d1, hb[0:8, 128:256]),
                                   jnp.where(zero > 0, d2, hb[0:8, 256:384]), hb[0:8, 384:]], axis=1)
            hb = jnp.concatenate([top, hb[8:]], axis=0)
        q = jnp.dot(_ub(hb), wq_buf[hh], preferred_element_type=F32)
        return (q * QSCALE).astype(BF16)

    def qk(unit, q):
        hh, sub, par = unit
        return jax.lax.dot_general(q, k_buf[hh], (((1,), (1,)), ((), ())), preferred_element_type=F32)

    def softmax(s, zero, AC=AC):
        ls, ps = [], []
        nc = S // 128
        for c in range(TU // RC):
            sc = s[c * RC:(c + 1) * RC, :]
            m = jnp.max(sc, axis=-1, keepdims=True)
            p = jnp.exp2(sc - m)
            cols = [p[:, i * 128:(i + 1) * 128] for i in range(nc)]
            a = cols[0]
            for i in range(1, nc):
                if i == nc - AC:
                    part = a
                a = a + cols[i]
            if AC:
                cols[nc - AC] = jnp.where(zero > 0, part, cols[nc - AC])
            ls.append(a)
            ps.append(jnp.concatenate(cols, axis=1))
        return jnp.concatenate(ps, axis=0).astype(BF16), jnp.concatenate(ls, axis=0)

    def pv(unit, s, zero, ac=AC):
        hh, sub, par = unit
        pb, lp = softmax(s, zero, ac)
        return jnp.dot(pb, v_buf[hh], preferred_element_type=F32), lp

    def fin(ol):
        return (ol[0] * _recip(jnp.sum(ol[1], axis=-1, keepdims=True))).astype(BF16)

    def outp(unit, ol):
        hh, sub, par = unit
        o = fin(ol) if isinstance(ol, tuple) else ol
        w = wo_buf[pl.ds(pl.multiple_of(hh * DH, DH), DH), :]
        acc[par, sub * TU:(sub + 1) * TU, :] += jnp.dot(o, w, preferred_element_type=F32)

    def modrow(i):
        return mod_buf[:, i * D:(i + 1) * D][None]

    def ln1_stats(xrow0, n, zero):
        x = x_buf[pl.ds(xrow0, n), :].astype(F32)
        d = acc[zero, pl.ds(pl.multiple_of(zero * 8, 8), n), 0:128]
        x = jnp.concatenate([jnp.where(zero > 0, d, x[:, 0:128]), x[:, 128:]], axis=1).reshape(n // 8, 8, D)
        return _stats(x)

    def ln1(xrow0, par, hrow0, n, onepass, stats=None):
        x = x_buf[pl.ds(xrow0, n), :].astype(F32).reshape(n // 8, 8, D)
        if stats is None and onepass:
            stats = _stats(x)
        nrm = _ln(x) if stats is None else (x - stats[0]) * stats[1]
        h = (nrm * modrow(1) + modrow(0)).reshape(n, D)
        h_buf[par, pl.ds(hrow0, n // 2), :] = _pk(h.astype(BF16))

    def top2_update(r, row0, valid):
        b = pltpu.bitcast(r, I32)
        key = (b ^ ((b >> 31) & 0x7FFFFFFF)) | (S - 1)
        rid = jax.lax.broadcasted_iota(I32, (8, 128), 0) + row0
        best, second = r_buf[0], r_buf[1]
        for i in range(r.shape[0]):
            k = key[i] - (rid + 8 * i)
            if valid is not None:
                k = jnp.where(valid, k, KMIN)
            second = jnp.maximum(second, jnp.minimum(best, k))
            best = jnp.maximum(best, k)
        r_buf[0] = best
        r_buf[1] = second

    def epi(row0, par, arow0, n, valid):
        a = acc[par, pl.ds(arow0, n), :].reshape(n // 8, 8, D)
        acc[par, pl.ds(arow0, n), :] = jnp.zeros((n, D), F32)
        x1 = x_buf[pl.ds(row0, n), :].astype(F32).reshape(n // 8, 8, D) + modrow(2) * a
        d = x1 - jnp.sum(x1, axis=-1, keepdims=True) * (1.0 / D)
        rstd = jax.lax.rsqrt(jnp.sum(d * d, axis=-1, keepdims=True) * (1.0 / D) + EPS)
        h2 = d * rstd * modrow(4) + modrow(3)
        x_buf[pl.ds(pl.multiple_of(jnp.where(valid, row0, S), n), n), :] = h2.reshape(n, D).astype(BF16)
        out_buf[pl.ds(row0, n), :] = (x1 + modrow(5) * h2).reshape(n, D).astype(BF16)
        r = jnp.sum(h2 * modrow(6), axis=-1, keepdims=True)
        top2_update(jnp.broadcast_to(r, (n // 8, 8, 128)), row0, valid)

    def epi_a(row0, par, arow0, n, u, su, c0):
        a = acc[par, arow0:arow0 + n, :].reshape(n // 8, 8, D)
        x1 = x_buf[row0:row0 + n, :].astype(F32).reshape(n // 8, 8, D) + modrow(2) * a
        acc[par, arow0:arow0 + n, :] = x1.reshape(n, D)
        mu, rstd = [jnp.broadcast_to(v, (n // 8, 8, 128)) for v in _stats(x1)]
        st_buf[0, arow0:arow0 + n, :] = mu.reshape(n, 128)
        st_buf[1, arow0:arow0 + n, :] = rstd.reshape(n, 128)
        xu = jnp.sum(x1 * u, axis=-1, keepdims=True)
        top2_update((xu - mu * su) * rstd + c0, row0, None)

    def last_norm(par, arow0, n):
        x1 = acc[par, pl.ds(arow0, n), :].reshape(n // 8, 8, D)
        mu = jnp.concatenate([st_buf[0, pl.ds(arow0, n), :]] * 8, axis=1).reshape(n // 8, 8, D)
        rstd = jnp.concatenate([st_buf[1, pl.ds(arow0, n), :]] * 8, axis=1).reshape(n // 8, 8, D)
        return x1, (x1 - mu) * rstd

    def run_units(seq, side, zero, acs={}):
        s = s_sc[...]
        ol_prev = (of_sc[...], l_sc[...])
        for u in range(len(seq) - 2):
            q = qp(seq[u + 2], u > 0 and side[u - 1][1], zero)
            ol = pv(seq[u + 1], s, zero, acs.get(u, AC))
            outp(seq[u], ol_prev)
            ol_prev = ol
            side[u][0](q)
            s = qk(seq[u + 2], q)
        s_sc[...] = s
        of_sc[...] = ol_prev[0]
        l_sc[...] = ol_prev[1]

    def mod_cols(c0, n):
        cf = c_buf[...].astype(F32)
        sc = (cf * jax.nn.sigmoid(cf)).astype(BF16)
        sc = jnp.broadcast_to(sc, (16, D))
        m = jnp.dot(sc, wm_buf[:, c0:c0 + n], preferred_element_type=F32)
        return _rb(m[0:8, :])

    start(d_small())
    start(d_xrows(0, TU, sem.at[SEM_X]))
    start(d_xrows(TU, TU, sem.at[SEM_X0B]))
    for i in range(NQP):
        if i % 2 == 0:
            start(d_wm(i // 2))
        start(d_wq2(i))
    start(d_sa())
    start(d_k(0, 1, sem.at[SEM_KV0]) + d_v(0, 1, sem.at[SEM_V0]) + d_k(1, 1, sem.at[SEM_MINI]))
    start(d_mini(1))
    start(d_x1a())
    for i in range(2, NM):
        start(d_mini(i))
    start(d_hand())
    start(d_x(1))
    start(d_grp(0))

    def zero_init(i, _):
        r0 = pl.multiple_of(i * 32, 32)
        for p_ in range(2):
            acc[p_, pl.ds(r0, 32), :] = jnp.zeros((32, D), F32)
        qa_buf[:, pl.ds(r0, 32), :] = jnp.zeros((NM + 1, 32, DH), F32)
        return 0
    jax.lax.fori_loop(0, TQ // 32, zero_init, 0)
    mod_buf[...] = jnp.zeros(mod_buf.shape, F32)
    r_buf[...] = jnp.full(r_buf.shape, KMIN, I32)
    out_buf[0:16, :] = jnp.zeros((16, D), BF16)

    zero0 = r_buf[0, 0, 0] & 1

    def rest(_i, _c):
        wait(d_small())
        wr = wr_buf[...].astype(F32)
        for i in range(8):
            mod_buf[:, 6 * D + i * 128:6 * D + (i + 1) * 128] = jnp.broadcast_to(wr[i:i + 1, :], (8, 128))
        wait(d_xrows(0, TU, sem.at[SEM_X]))

        def norm_first(i, _):
            @pl.when(i == TU // 64)
            def _():
                wait(d_xrows(TU, TU, sem.at[SEM_X0B]))
            for half in range(2):
                r0 = pl.multiple_of(i * 64 + half * 32, 32)
                n_buf[pl.ds(r0, 32), :] = _ln(x_buf[pl.ds(r0, 32), :].astype(F32))
            return 0
        jax.lax.fori_loop(0, TQ // 64, norm_first, 0)

        def qp_first(i, _):
            for c in range(WMC):
                @pl.when(i == 2 * c)
                def _():
                    wait(d_wm(c))
                    ca = _rb(1.0 + mod_cols(D + c * WC, WC))
                    mod_buf[:, D + c * WC:D + (c + 1) * WC] = ca
                    for half in range(2):
                        nv = n_buf[half * TU:(half + 1) * TU, c * WC:(c + 1) * WC].reshape(TU // 8, 8, WC) * ca[None]
                        h_buf[0, half * (TU // 2):(half + 1) * (TU // 2), 0:WC] = _pk(nv.reshape(TU, WC).astype(BF16))
            wait(d_wq2(i))
            rows = pl.ds(pl.multiple_of((i >> 1) * WC, WC), WC)
            for k in range(4):
                hh = 4 * (i & 1) + k
                for sub in range(2):
                    hb = _ub(h_buf[0, sub * (TU // 2):(sub + 1) * (TU // 2), 0:WC])
                    qa_buf[hh, sub * TU:(sub + 1) * TU, :] += jnp.dot(
                        hb, wq_buf[hh, rows, :], preferred_element_type=F32)
            return 0
        jax.lax.fori_loop(0, NQP, qp_first, 0)

        def q_first(hh, sub):
            qa = qa_buf[hh, sub * TU:(sub + 1) * TU, :].reshape(TU // 8, 8, DH)
            return ((qa + b_buf[hh][None]) * QSCALE).reshape(TU, DH).astype(BF16)
        wait(d_sa())
        sa = mod_cols(0, D)
        mod_buf[:, 0:D] = sa
        sab = jnp.concatenate([sa, sa], axis=0).astype(BF16)
        for hh in range(NM + 1):
            b_buf[hh] = jnp.dot(sab, wq_buf[hh], preferred_element_type=F32)[0:8]
        wait(d_k(0, 1, sem.at[SEM_KV0]))
        s0 = qk((0, 0, 0), q_first(0, 0))
        npc_ = TQ // FHR

        def h_piece(k, src, pos):
            r_, c_ = (pos % 16) * 16, (pos // 16) * 512
            z = jnp.where(zero0 > 0, pltpu.bitcast(src[r_:r_ + 8, c_:c_ + 128], I32)[0, 0], 0)
            zr = pl.multiple_of(jnp.clip(z + k, 0, npc_ - 1) * FHR, FHR)
            nv = n_buf[pl.ds(zr, FHR), :].reshape(FHR // 8, 8, D) * modrow(1) + modrow(0)
            h_buf[0, k * FHR // 2:(k + 1) * FHR // 2, :] = _pk(nv.reshape(FHR, D).astype(BF16))
        for k in range(FN0):
            h_piece(k, s0, (k * FSPAN) // FN0)
        wait(d_v(0, 1, sem.at[SEM_V0]))
        s1 = qk((0, 1, 0), q_first(0, 1))
        for k in range(FN0, npc_):
            h_piece(k, s1, ((k - FN0) * FSPAN1) // (npc_ - FN0))
        ol0 = pv((0, 0, 0), s0, zero0, ACP)
        wait(d_k(1, 1, sem.at[SEM_MINI]))
        s_sc[...] = qk((1, 0, 0), q_first(1, 0))
        ol1 = pv((0, 1, 0), s1, zero0, ACP1)
        on_sc[...] = _pk(fin(ol0))
        of_sc[...] = ol1[0]
        l_sc[...] = ol1[1]

        def mini(i, _):
            wait(d_mini(i))

            @pl.when(i == 2)
            def _():
                wait(d_x1a())
            zero = i >> 10

            def piece(u):
                pc = jnp.minimum(2 * (i - 2) + u, NM)
                ln1(pl.multiple_of(TQ + pc * PC, PC), 1,
                    pl.multiple_of(jnp.maximum(pc, 0) * (PC // 2), PC // 2), PC, False)
            outp((i - 1, 0, 0), _ub(on_sc[...]))
            ola = pv((i, 0, 0), s_sc[...], zero, ACM0)
            piece(0)
            s = qk((i, 1, 0), q_first(i, 1))
            outp((i - 1, 1, 0), (of_sc[...], l_sc[...]))
            ol = pv((i, 1, 0), s, zero, ACM1)
            piece(1)
            s_sc[...] = qk((i + 1, 0, 0), q_first(i + 1, 0))
            on_sc[...] = _pk(fin(ola))
            of_sc[...] = ol[0]
            l_sc[...] = ol[1]
            return 0
        jax.lax.fori_loop(1, NM, mini, 0)
        wait(d_hand())
        outp((NM - 1, 0, 0), _ub(on_sc[...]))
        ola = pv((NM, 0, 0), s_sc[...], zero0, ACH)
        outp((NM - 1, 1, 0), (of_sc[...], l_sc[...]))
        s_sc[...] = qk((NM, 1, 0), q_first(NM, 1))
        of_sc[...] = ola[0]
        l_sc[...] = ola[1]
        for t in range(1, NG):
            start(d_grp(t))
        start(d_late())
        start(d_x(2))
        start(d_x(3))
        for i in range(3):
            start(d_ffn(i))

        def main(t, _):
            @pl.when(t < NG)
            def _():
                wait(d_grp(t))

            @pl.when(t == 0)
            def _():
                wait(d_x(1))

            @pl.when(t == NG)
            def _():
                wait(d_late())
                wait(d_x(2))
                wait(d_x(3))
                for i in range(3):
                    wait(d_ffn(i))
                for i in range(2, 6):
                    m = mod_cols(i * D, D)
                    if i == 4:
                        m = _rb(1.0 + m)
                    mod_buf[:, i * D:(i + 1) * D] = m

            @pl.when(t > NG)
            def _():
                start(d_out(pl.multiple_of((t - 1 - NG) * (HP * PC), PC), HP * PC, sem.at[SEM_OUT]))

            p0 = t * HP + NM + 1
            zero = t >> 10
            seq, side, stats = [], [], {}
            pairs = [((p0 + k) & (H - 1), (p0 + k) >> 5) for k in range(-1, HP)]
            for hh, j in pairs:
                seq += [(hh, 0, j & 1), (hh, 1, j & 1)]

            def xnext(k):
                hh, j = pairs[k + 1]
                return pl.multiple_of(jnp.minimum(j + 1, NQ - 1) * TQ + hh * PC, PC)

            def ln1_piece(k, q):
                hh, j = pairs[k + 1]
                st = stats.get(k)
                if st is not None:
                    mu = jnp.where(zero > 0, q[0:PC].astype(F32).reshape(PC // 8, 8, 128),
                                   jnp.broadcast_to(st[0], (PC // 8, 8, 128)))
                    st = (jnp.concatenate([mu] * 8, axis=2), st[1])
                ln1(xnext(k), 1 - (j & 1), pl.multiple_of(hh * (PC // 2), PC // 2), PC, True, st)

            def epi_piece(k, q):
                hh, j = pairs[k + 1]
                if k + 1 < HP:
                    stats[k + 1] = ln1_stats(xnext(k + 1), PC, zero)
                epi(pl.multiple_of(jnp.maximum(j - 1, 0) * TQ + hh * PC, PC), 1 - (j & 1),
                    pl.multiple_of(hh * PC, PC), PC, j > 0)

            for k in range(HP):
                side += [(functools.partial(ln1_piece, k), False), (functools.partial(epi_piece, k), True)]
            run_units(seq, side, zero, {0: AC0, 1: AC1})
            return 0
        jax.lax.fori_loop(0, NT, main, 0)

        start(d_out((NT - 1 - NG) * HP * PC, HP * PC, sem.at[SEM_OUT]))
        lastp = (NQ - 1) & 1
        base = (NQ - 1) * TQ
        ru = modrow(4) * modrow(6)
        rsu = jnp.sum(ru, axis=-1, keepdims=True)
        rc0 = jnp.sum(modrow(3) * modrow(6), axis=-1, keepdims=True)

        def epis(half):
            for i in range(half * TU // TPC, (half + 1) * TU // TPC):
                epi_a(base + i * TPC, lastp, i * TPC, TPC, ru, rsu, rc0)
        ol = pv((H - 1, 1, lastp), s_sc[...], zero0, ACT)
        outp((H - 1, 0, lastp), (of_sc[...], l_sc[...]))
        outp((H - 1, 1, lastp), ol)
        epis(0)
        epis(1)
        best, second = r_buf[0], r_buf[1]
        for sh in (4, 2, 1):
            b2 = pltpu.roll(best, sh, 0)
            s2 = pltpu.roll(second, sh, 0)
            second = jnp.maximum(jnp.minimum(best, b2), jnp.maximum(second, s2))
            best = jnp.maximum(best, b2)
        i1 = (S - 1) - (best[0, 0] & (S - 1))
        i2 = (S - 1) - (second[0, 0] & (S - 1))
        g1 = pl.multiple_of(jnp.clip(i1 >> 3, 0, S // 8 - 1) * 8, 8)
        g2 = pl.multiple_of(jnp.clip(i2 >> 3, 0, S // 8 - 1) * 8, 8)

        def h2_rows(g):
            nrm = last_norm(lastp, pl.multiple_of(jnp.clip(g - base, 0, TQ - 8), 8), 8)[1]
            last = (nrm * modrow(4) + modrow(3)).reshape(8, D)
            return jnp.where(g >= base, last, x_buf[pl.ds(g, 8), :].astype(F32))
        xs = jnp.concatenate([h2_rows(g1), h2_rows(g2)], axis=0).astype(BF16)
        gt = jnp.dot(xs, wg_buf[...], preferred_element_type=F32)
        up = jnp.dot(xs, wu_buf[...], preferred_element_type=F32)
        gbits = pltpu.bitcast(jnp.concatenate([gt, up], axis=1), I32)
        ga_, gb_ = modrow(5) * modrow(4), modrow(5) * modrow(3)
        npc = TQ // CPC
        for i in range(npc):
            z = jnp.where(i1 < 0, gbits[0, 128 * (i * CSPAN // npc)], 0)
            x1, nrm = last_norm(lastp, pl.multiple_of(jnp.clip(z + i, 0, npc - 1) * CPC, CPC), CPC)
            out_buf[base + i * CPC:base + (i + 1) * CPC, :] = (x1 + nrm * ga_ + gb_).reshape(CPC, D).astype(BF16)
            if i == npc // 2 - 1:
                start(d_out(base, TU, sem.at[SEM_OUT2]))
        start(d_out(base + TU, TU, sem.at[SEM_OUT2]))
        gt = _rb(gt)
        a = (_rb(gt * jax.nn.sigmoid(gt)) * _rb(up)).astype(BF16)
        y = _rb(jnp.dot(a, wd_buf[:, 0:D], preferred_element_type=F32))

        def score(k):
            return pltpu.bitcast((k ^ ((k >> 31) & 0x7FFFFFFF)) & -S, F32)
        ri = jax.lax.broadcasted_iota(I32, (16, 128), 0)
        rows = jnp.where(ri < 8, g1 + ri, g2 + ri - 8)
        r1 = jnp.concatenate([score(best)] * 2, axis=0)
        r2 = jnp.concatenate([score(second)] * 2, axis=0)
        gate = _rb(jax.nn.sigmoid(_rb(jnp.where(rows == i1, r1, r2))))
        sel = (rows == i1) | (rows == i2)
        upd = jnp.where(sel[:, 0:1], _rb(y * gate[:, 0:1]), 0.0) * mod_buf[0:1, 5 * D:6 * D]
        o1 = (out_buf[pl.ds(g1, 8), :].astype(F32) + upd[0:8]).astype(BF16)
        o2 = (out_buf[pl.ds(g2, 8), :].astype(F32) + upd[8:16]).astype(BF16)
        cp(out_buf.at[pl.ds(0, base), :], out_hbm.at[0, pl.ds(0, base), :], sem.at[SEM_OUT]).wait()
        wait(d_out(base, TQ, sem.at[SEM_OUT2]))
        out_buf[pl.ds(g1, 8), :] = o1
        out_buf[pl.ds(g2, 8), :] = o2
        start(d_out(g1, 8, sem.at[SEM_FIX]))

        @pl.when(g1 != g2)
        def _():
            start(d_out(g2, 8, sem.at[SEM_FIX + 1]))
            wait(d_out(g2, 8, sem.at[SEM_FIX + 1]))

        wait(d_out(g1, 8, sem.at[SEM_FIX]))
        return 0
    jax.lax.fori_loop(0, zero0 + 1, rest, 0)


@jax.jit
def pallas_adaLN_cond__mha_block_cached__moe_arch_mod__prompt_kernel(
    A_x: jax.Array,
    A_k_cache: jax.Array,
    A_v_cache: jax.Array,
    A_wq: jax.Array,
    A_wo: jax.Array,
    B_x: jax.Array,
    B_w_r: jax.Array,
    B_w_gate: jax.Array,
    B_w_up: jax.Array,
    B_w_down: jax.Array,
    c: jax.Array,
    w_mod: jax.Array,
):
    del B_x
    vm = pltpu.VMEM
    scratch = [
        vm((S + PC, D), BF16),
        vm((2, TQ // 2, D), U32),
        vm((H, S, DH), BF16),
        vm((H, S, DH), BF16),
        vm((H, D, DH), BF16),
        vm((H * DH, D), BF16),
        vm((D, FF), BF16),
        vm((D, FF), BF16),
        vm((FF, D + 128), BF16),
        vm((D, 6 * D + 128), BF16),
        vm((1, D), BF16),
        vm((8, 128), BF16),
        vm((8, 7 * D), F32),
        vm((2, TQ, D), F32),
        vm((S, D), BF16),
        vm((TU, S), F32),
        vm((TU, DH), F32),
        vm((TU, DH), F32),
        vm((2, 8, 128), I32),
        vm((2, TQ, 128), F32),
        vm((NM + 1, TQ, DH), F32),
        vm((NM + 1, 8, DH), F32),
        vm((TU // 2, DH), U32),
        vm((TQ, D), F32),
        pltpu.SemaphoreType.DMA((NSEM,)),
    ]
    anyspec = pl.BlockSpec(memory_space=pl.ANY)
    return pl.pallas_call(
        _kernel,
        in_specs=[anyspec] * 11,
        out_specs=anyspec,
        out_shape=jax.ShapeDtypeStruct((1, S, D), BF16),
        scratch_shapes=scratch,
        compiler_params=pltpu.CompilerParams(vmem_limit_bytes=120 * 1024 * 1024, disable_bounds_checks=True,
                                             disable_semaphore_checks=True),
    )(A_x, A_k_cache, A_v_cache, A_wq, A_wo, B_w_r.reshape(8, 128), B_w_gate, B_w_up, B_w_down, c, w_mod)
```

```python
import functools

import jax
import jax.numpy as jnp
import jax.experimental.pallas as pl
import jax.experimental.pallas.tpu as pltpu

F32, BF16, U32, I32 = jnp.float32, jnp.bfloat16, jnp.uint32, jnp.int32

S, D, H, DH, FF = 2048, 1024, 32, 128, 3584
TU = 256
TQ = 512
NQ = S // TQ
HP = 6
NM = 7
NT = (NQ * H - 1 - NM) // HP
NG = (H - 1 - NM) // HP
NQP = (NM + 1) // 2
WMC = 2
PC = 16
EPS = 1e-5
QSCALE = DH ** -0.5 * 1.4426950408889634
KMIN = -2 ** 31
RC = 16
AC = 2
AC0 = 8
AC1 = 2
ACM0 = 8
ACM1 = 1
ACP = 1
ACP1 = 2
ACH = 1
ACT = 3
FHR = 16
FN0 = 20
FSPAN = 60
FSPAN1 = 32
TPC = 64
CPC = 32
CSPAN = 40

SEM_SMALL = 0
SEM_X = 1
SEM_X1A = 5
SEM_WM = 6
SEM_WMR = 8
SEM_SA = 9
SEM_K0 = 10
SEM_V0 = 11
SEM_X0B = 12
SEM_FFN = 13
SEM_OUT = 14
SEM_OUT2 = 15
SEM_FIX = 16
SEM_MINI = 18
SEM_GRP = SEM_MINI + NM + 1
SEM_QP = SEM_GRP + NG
NSEM = SEM_QP + NQP


def _rb(x):
    return x.astype(BF16).astype(F32)


def _ub(x):
    return pltpu.bitcast(x, BF16)


def _pk(x):
    return pltpu.bitcast(x, U32)


def _recip(l):
    r = pl.reciprocal(l, approx=True)
    return r * (2.0 - l * r)


def _ln(x):
    mu = jnp.sum(x, axis=-1, keepdims=True) * (1.0 / D)
    d = x - mu
    var = jnp.sum(d * d, axis=-1, keepdims=True) * (1.0 / D)
    return d * jax.lax.rsqrt(var + EPS)


def _stats(x):
    mu = jnp.sum(x, axis=-1, keepdims=True) * (1.0 / D)
    var = jnp.maximum(jnp.sum(x * x, axis=-1, keepdims=True) * (1.0 / D) - mu * mu, 0.0)
    return mu, jax.lax.rsqrt(var + EPS)


def _kernel(x_hbm, k_hbm, v_hbm, wq_hbm, wo_hbm, wr_hbm, wg_hbm, wu_hbm, wd_hbm, c_hbm, wm_hbm,
            out_hbm,
            x_buf, h_buf, k_buf, v_buf, wq_buf, wo_buf, wg_buf, wu_buf, wd_buf, wm_buf,
            c_buf, wr_buf, mod_buf, acc, out_buf, s_sc, of_sc, l_sc, r_buf, st_buf, qa_buf, b_buf, on_sc, n_buf, sem):
    cp = pltpu.make_async_copy

    def d_small():
        return [cp(c_hbm, c_buf, sem.at[SEM_SMALL]), cp(wr_hbm, wr_buf, sem.at[SEM_SMALL])]

    def d_xrows(r0, n, s_):
        return [cp(x_hbm.at[0, pl.ds(r0, n), :], x_buf.at[pl.ds(r0, n), :], s_)]

    X1A = 128

    def d_x(j):
        if j == 1:
            return d_xrows(TQ + X1A, TQ - X1A, sem.at[SEM_X + 1])
        return d_xrows(j * TQ, TQ, sem.at[SEM_X + j])

    def d_x1a():
        return d_xrows(TQ, X1A, sem.at[SEM_X1A])

    WC = D // WMC

    def d_wm(i):
        return [cp(wm_hbm.at[:, pl.ds(D + i * WC, WC)], wm_buf.at[:, pl.ds(D + i * WC, WC)], sem.at[SEM_WM + i])]

    def d_sa():
        return [cp(wm_hbm.at[:, pl.ds(0, D)], wm_buf.at[:, pl.ds(0, D)], sem.at[SEM_SA])]

    def d_wq2(i):
        rows = pl.ds(pl.multiple_of((i >> 1) * WC, WC), WC)
        return [cp(wq_hbm.at[rows, pl.ds(pl.multiple_of((4 * (i & 1) + k) * DH, DH), DH)],
                   wq_buf.at[4 * (i & 1) + k, rows, :], sem.at[SEM_QP + i]) for k in range(4)]

    def d_wmr():
        return [cp(wm_hbm.at[:, pl.ds(2 * D, 4 * D)], wm_buf.at[:, pl.ds(2 * D, 4 * D)], sem.at[SEM_WMR])]

    def d_wq(h0, n, s_):
        return [cp(wq_hbm.at[:, pl.ds(pl.multiple_of((h0 + i) * DH, DH), DH)], wq_buf.at[h0 + i], s_)
                for i in range(n)]

    def d_k(h0, n, s_):
        return [cp(k_hbm.at[0, pl.ds(h0, n)], k_buf.at[pl.ds(h0, n)], s_)]

    def d_v(h0, n, s_):
        return [cp(v_hbm.at[0, pl.ds(h0, n)], v_buf.at[pl.ds(h0, n)], s_)]

    def d_wo(h0, n, s_):
        rows = pl.ds(pl.multiple_of(h0 * DH, DH), n * DH)
        return [cp(wo_hbm.at[rows, :], wo_buf.at[rows, :], s_)]

    def d_mini(i):
        s_ = sem.at[SEM_MINI + i]
        return d_wo(i - 1, 1, s_) + d_v(i, 1, s_) + d_k(i + 1, 1, s_)

    def d_hand():
        s_ = sem.at[SEM_MINI + NM]
        return d_wo(NM - 1, 1, s_) + d_v(NM, 1, s_)

    def d_grp(t):
        s_ = sem.at[SEM_GRP + t]
        h0 = HP * t + NM + 1
        return d_wq(h0, HP, s_) + d_wo(h0 - 1, HP, s_) + d_k(h0, HP, s_) + d_v(h0, HP, s_)

    def d_late():
        return d_wmr() + d_wo(H - 1, 1, sem.at[SEM_WMR])

    def d_ffn(i):
        src, dst = ((wg_hbm, wg_buf), (wu_hbm, wu_buf), (wd_hbm, wd_buf.at[:, pl.ds(0, D)]))[i]
        return [cp(src, dst, sem.at[SEM_FFN])]

    def d_out(r0, n, s_):
        return [cp(out_buf.at[pl.ds(r0, n), :], out_hbm.at[0, pl.ds(r0, n), :], s_)]

    def start(ds):
        for d in ds:
            d.start()

    def wait(ds):
        for d in ds:
            d.wait()

    def qp(unit, anchor=False, zero=None):
        hh, sub, par = unit
        hb = h_buf[par, sub * (TU // 2):(sub + 1) * (TU // 2), :]
        if anchor:
            z16 = pl.multiple_of(zero * 16, 16)
            d0 = _pk(out_buf[pl.ds(z16, 16), 0:128])
            d1 = pltpu.bitcast(r_buf[zero], U32)
            d2 = _pk(x_buf[pl.ds(z16, 16), 0:128])
            top = jnp.concatenate([jnp.where(zero > 0, d0, hb[0:8, 0:128]),
                                   jnp.where(zero > 0, d1, hb[0:8, 128:256]),
                                   jnp.where(zero > 0, d2, hb[0:8, 256:384]), hb[0:8, 384:]], axis=1)
            hb = jnp.concatenate([top, hb[8:]], axis=0)
        q = jnp.dot(_ub(hb), wq_buf[hh], preferred_element_type=F32)
        return (q * QSCALE).astype(BF16)

    def qk(unit, q):
        hh, sub, par = unit
        return jax.lax.dot_general(q, k_buf[hh], (((1,), (1,)), ((), ())), preferred_element_type=F32)

    def softmax(s, zero, AC=AC):
        ls, ps = [], []
        nc = S // 128
        for c in range(TU // RC):
            sc = s[c * RC:(c + 1) * RC, :]
            m = jnp.max(sc, axis=-1, keepdims=True)
            p = jnp.exp2(sc - m)
            cols = [p[:, i * 128:(i + 1) * 128] for i in range(nc)]
            a = cols[0]
            for i in range(1, nc):
                if i == nc - AC:
                    part = a
                a = a + cols[i]
            if AC:
                cols[nc - AC] = jnp.where(zero > 0, part, cols[nc - AC])
            ls.append(a)
            ps.append(jnp.concatenate(cols, axis=1))
        return jnp.concatenate(ps, axis=0).astype(BF16), jnp.concatenate(ls, axis=0)

    def pv(unit, s, zero, ac=AC):
        hh, sub, par = unit
        pb, lp = softmax(s, zero, ac)
        return jnp.dot(pb, v_buf[hh], preferred_element_type=F32), lp

    def fin(ol):
        return (ol[0] * _recip(jnp.sum(ol[1], axis=-1, keepdims=True))).astype(BF16)

    def outp(unit, ol):
        hh, sub, par = unit
        o = fin(ol) if isinstance(ol, tuple) else ol
        w = wo_buf[pl.ds(pl.multiple_of(hh * DH, DH), DH), :]
        acc[par, sub * TU:(sub + 1) * TU, :] += jnp.dot(o, w, preferred_element_type=F32)

    def modrow(i):
        return mod_buf[:, i * D:(i + 1) * D][None]

    def ln1_stats(xrow0, n, zero):
        x = x_buf[pl.ds(xrow0, n), :].astype(F32)
        d = acc[zero, pl.ds(pl.multiple_of(zero * 8, 8), n), 0:128]
        x = jnp.concatenate([jnp.where(zero > 0, d, x[:, 0:128]), x[:, 128:]], axis=1).reshape(n // 8, 8, D)
        return _stats(x)

    def ln1(xrow0, par, hrow0, n, onepass, stats=None):
        x = x_buf[pl.ds(xrow0, n), :].astype(F32).reshape(n // 8, 8, D)
        if stats is None and onepass:
            stats = _stats(x)
        nrm = _ln(x) if stats is None else (x - stats[0]) * stats[1]
        h = (nrm * modrow(1) + modrow(0)).reshape(n, D)
        h_buf[par, pl.ds(hrow0, n // 2), :] = _pk(h.astype(BF16))

    def top2_update(r, row0, valid):
        b = pltpu.bitcast(r, I32)
        key = (b ^ ((b >> 31) & 0x7FFFFFFF)) | (S - 1)
        rid = jax.lax.broadcasted_iota(I32, (8, 128), 0) + row0
        best, second = r_buf[0], r_buf[1]
        for i in range(r.shape[0]):
            k = key[i] - (rid + 8 * i)
            if valid is not None:
                k = jnp.where(valid, k, KMIN)
            second = jnp.maximum(second, jnp.minimum(best, k))
            best = jnp.maximum(best, k)
        r_buf[0] = best
        r_buf[1] = second

    def epi(row0, par, arow0, n, valid):
        a = acc[par, pl.ds(arow0, n), :].reshape(n // 8, 8, D)
        acc[par, pl.ds(arow0, n), :] = jnp.zeros((n, D), F32)
        x1 = x_buf[pl.ds(row0, n), :].astype(F32).reshape(n // 8, 8, D) + modrow(2) * a
        d = x1 - jnp.sum(x1, axis=-1, keepdims=True) * (1.0 / D)
        rstd = jax.lax.rsqrt(jnp.sum(d * d, axis=-1, keepdims=True) * (1.0 / D) + EPS)
        h2 = d * rstd * modrow(4) + modrow(3)
        x_buf[pl.ds(pl.multiple_of(jnp.where(valid, row0, S), n), n), :] = h2.reshape(n, D).astype(BF16)
        out_buf[pl.ds(row0, n), :] = (x1 + modrow(5) * h2).reshape(n, D).astype(BF16)
        r = jnp.sum(h2 * modrow(6), axis=-1, keepdims=True)
        top2_update(jnp.broadcast_to(r, (n // 8, 8, 128)), row0, valid)

    def epi_a(row0, par, arow0, n, u, su, c0):
        a = acc[par, arow0:arow0 + n, :].reshape(n // 8, 8, D)
        x1 = x_buf[row0:row0 + n, :].astype(F32).reshape(n // 8, 8, D) + modrow(2) * a
        acc[par, arow0:arow0 + n, :] = x1.reshape(n, D)
        mu, rstd = [jnp.broadcast_to(v, (n // 8, 8, 128)) for v in _stats(x1)]
        st_buf[0, arow0:arow0 + n, :] = mu.reshape(n, 128)
        st_buf[1, arow0:arow0 + n, :] = rstd.reshape(n, 128)
        xu = jnp.sum(x1 * u, axis=-1, keepdims=True)
        top2_update((xu - mu * su) * rstd + c0, row0, None)

    def last_norm(par, arow0, n):
        x1 = acc[par, pl.ds(arow0, n), :].reshape(n // 8, 8, D)
        mu = jnp.concatenate([st_buf[0, pl.ds(arow0, n), :]] * 8, axis=1).reshape(n // 8, 8, D)
        rstd = jnp.concatenate([st_buf[1, pl.ds(arow0, n), :]] * 8, axis=1).reshape(n // 8, 8, D)
        return x1, (x1 - mu) * rstd

    def run_units(seq, side, zero, acs={}):
        s = s_sc[...]
        ol_prev = (of_sc[...], l_sc[...])
        for u in range(len(seq) - 2):
            q = qp(seq[u + 2], u > 0 and side[u - 1][1], zero)
            ol = pv(seq[u + 1], s, zero, acs.get(u, AC))
            outp(seq[u], ol_prev)
            ol_prev = ol
            side[u][0](q)
            s = qk(seq[u + 2], q)
        s_sc[...] = s
        of_sc[...] = ol_prev[0]
        l_sc[...] = ol_prev[1]

    def mod_cols(c0, n):
        cf = c_buf[...].astype(F32)
        sc = (cf * jax.nn.sigmoid(cf)).astype(BF16)
        sc = jnp.broadcast_to(sc, (16, D))
        m = jnp.dot(sc, wm_buf[:, c0:c0 + n], preferred_element_type=F32)
        return _rb(m[0:8, :])

    start(d_small())
    start(d_xrows(0, TU, sem.at[SEM_X]))
    start(d_xrows(TU, TU, sem.at[SEM_X0B]))
    for i in range(NQP):
        if i % 2 == 0:
            start(d_wm(i // 2))
        start(d_wq2(i))
    start(d_sa())
    start(d_k(0, 1, sem.at[SEM_K0]) + d_v(0, 1, sem.at[SEM_V0]) + d_k(1, 1, sem.at[SEM_MINI]))
    start(d_mini(1))
    start(d_x1a())
    for i in range(2, NM):
        start(d_mini(i))
    start(d_hand())
    start(d_x(1))
    start(d_grp(0))

    def zero_init(i, _):
        r0 = pl.multiple_of(i * 32, 32)
        for p_ in range(2):
            acc[p_, pl.ds(r0, 32), :] = jnp.zeros((32, D), F32)
        qa_buf[:, pl.ds(r0, 32), :] = jnp.zeros((NM + 1, 32, DH), F32)
        return 0
    jax.lax.fori_loop(0, TQ // 32, zero_init, 0)
    mod_buf[...] = jnp.zeros(mod_buf.shape, F32)
    r_buf[...] = jnp.full(r_buf.shape, KMIN, I32)
    out_buf[0:16, :] = jnp.zeros((16, D), BF16)

    zero0 = r_buf[0, 0, 0] & 1

    def rest(_i, _c):
        wait(d_small())
        wr = wr_buf[...].astype(F32)
        for i in range(8):
            mod_buf[:, 6 * D + i * 128:6 * D + (i + 1) * 128] = jnp.broadcast_to(wr[i:i + 1, :], (8, 128))
        wait(d_xrows(0, TU, sem.at[SEM_X]))

        def norm_first(i, _):
            @pl.when(i == TU // 64)
            def _():
                wait(d_xrows(TU, TU, sem.at[SEM_X0B]))
            for half in range(2):
                r0 = pl.multiple_of(i * 64 + half * 32, 32)
                n_buf[pl.ds(r0, 32), :] = _ln(x_buf[pl.ds(r0, 32), :].astype(F32))
            return 0
        jax.lax.fori_loop(0, TQ // 64, norm_first, 0)

        def qp_first(i, _):
            for c in range(WMC):
                @pl.when(i == 2 * c)
                def _():
                    wait(d_wm(c))
                    ca = _rb(1.0 + mod_cols(D + c * WC, WC))
                    mod_buf[:, D + c * WC:D + (c + 1) * WC] = ca
                    for half in range(2):
                        nv = n_buf[half * TU:(half + 1) * TU, c * WC:(c + 1) * WC].reshape(TU // 8, 8, WC) * ca[None]
                        h_buf[0, half * (TU // 2):(half + 1) * (TU // 2), 0:WC] = _pk(nv.reshape(TU, WC).astype(BF16))
            wait(d_wq2(i))
            rows = pl.ds(pl.multiple_of((i >> 1) * WC, WC), WC)
            for k in range(4):
                hh = 4 * (i & 1) + k
                for sub in range(2):
                    hb = _ub(h_buf[0, sub * (TU // 2):(sub + 1) * (TU // 2), 0:WC])
                    qa_buf[hh, sub * TU:(sub + 1) * TU, :] += jnp.dot(
                        hb, wq_buf[hh, rows, :], preferred_element_type=F32)
            return 0
        jax.lax.fori_loop(0, NQP, qp_first, 0)

        def q_first(hh, sub):
            qa = qa_buf[hh, sub * TU:(sub + 1) * TU, :].reshape(TU // 8, 8, DH)
            return ((qa + b_buf[hh][None]) * QSCALE).reshape(TU, DH).astype(BF16)
        wait(d_sa())
        sa = mod_cols(0, D)
        mod_buf[:, 0:D] = sa
        sab = jnp.concatenate([sa, sa], axis=0).astype(BF16)
        for hh in range(NM + 1):
            b_buf[hh] = jnp.dot(sab, wq_buf[hh], preferred_element_type=F32)[0:8]
        wait(d_k(0, 1, sem.at[SEM_K0]))
        s0 = qk((0, 0, 0), q_first(0, 0))
        npc_ = TQ // FHR

        def h_piece(k, src, pos):
            r_, c_ = (pos % 16) * 16, (pos // 16) * 512
            z = jnp.where(zero0 > 0, pltpu.bitcast(src[r_:r_ + 8, c_:c_ + 128], I32)[0, 0], 0)
            zr = pl.multiple_of(jnp.clip(z + k, 0, npc_ - 1) * FHR, FHR)
            nv = n_buf[pl.ds(zr, FHR), :].reshape(FHR // 8, 8, D) * modrow(1) + modrow(0)
            h_buf[0, k * FHR // 2:(k + 1) * FHR // 2, :] = _pk(nv.reshape(FHR, D).astype(BF16))
        for k in range(FN0):
            h_piece(k, s0, (k * FSPAN) // FN0)
        wait(d_v(0, 1, sem.at[SEM_V0]))
        s1 = qk((0, 1, 0), q_first(0, 1))
        for k in range(FN0, npc_):
            h_piece(k, s1, ((k - FN0) * FSPAN1) // (npc_ - FN0))
        ol0 = pv((0, 0, 0), s0, zero0, ACP)
        wait(d_k(1, 1, sem.at[SEM_MINI]))
        s_sc[...] = qk((1, 0, 0), q_first(1, 0))
        ol1 = pv((0, 1, 0), s1, zero0, ACP1)
        on_sc[...] = _pk(fin(ol0))
        of_sc[...] = ol1[0]
        l_sc[...] = ol1[1]

        def mini(i, _):
            wait(d_mini(i))

            @pl.when(i == 2)
            def _():
                wait(d_x1a())
            zero = i >> 10

            def piece(u):
                pc = jnp.minimum(2 * (i - 2) + u, NM)
                ln1(pl.multiple_of(TQ + pc * PC, PC), 1,
                    pl.multiple_of(jnp.maximum(pc, 0) * (PC // 2), PC // 2), PC, False)
            outp((i - 1, 0, 0), _ub(on_sc[...]))
            ola = pv((i, 0, 0), s_sc[...], zero, ACM0)
            piece(0)
            s = qk((i, 1, 0), q_first(i, 1))
            outp((i - 1, 1, 0), (of_sc[...], l_sc[...]))
            ol = pv((i, 1, 0), s, zero, ACM1)
            piece(1)
            s_sc[...] = qk((i + 1, 0, 0), q_first(i + 1, 0))
            on_sc[...] = _pk(fin(ola))
            of_sc[...] = ol[0]
            l_sc[...] = ol[1]
            return 0
        jax.lax.fori_loop(1, NM, mini, 0)
        wait(d_hand())
        outp((NM - 1, 0, 0), _ub(on_sc[...]))
        ola = pv((NM, 0, 0), s_sc[...], zero0, ACH)
        outp((NM - 1, 1, 0), (of_sc[...], l_sc[...]))
        s_sc[...] = qk((NM, 1, 0), q_first(NM, 1))
        of_sc[...] = ola[0]
        l_sc[...] = ola[1]
        for t in range(1, NG):
            start(d_grp(t))
        start(d_late())
        start(d_x(2))
        start(d_x(3))
        for i in range(3):
            start(d_ffn(i))

        def main(t, _):
            @pl.when(t < NG)
            def _():
                wait(d_grp(t))

            @pl.when(t == 0)
            def _():
                wait(d_x(1))

            @pl.when(t == NG)
            def _():
                wait(d_late())
                wait(d_x(2))
                wait(d_x(3))
                for i in range(3):
                    wait(d_ffn(i))
                for i in range(2, 6):
                    m = mod_cols(i * D, D)
                    if i == 4:
                        m = _rb(1.0 + m)
                    mod_buf[:, i * D:(i + 1) * D] = m

            @pl.when(t > NG)
            def _():
                start(d_out(pl.multiple_of((t - 1 - NG) * (HP * PC), PC), HP * PC, sem.at[SEM_OUT]))

            p0 = t * HP + NM + 1
            zero = t >> 10
            seq, side, stats = [], [], {}
            pairs = [((p0 + k) & (H - 1), (p0 + k) >> 5) for k in range(-1, HP)]
            for hh, j in pairs:
                seq += [(hh, 0, j & 1), (hh, 1, j & 1)]

            def xnext(k):
                hh, j = pairs[k + 1]
                return pl.multiple_of(jnp.minimum(j + 1, NQ - 1) * TQ + hh * PC, PC)

            def ln1_piece(k, q):
                hh, j = pairs[k + 1]
                st = stats.get(k)
                if st is not None:
                    mu = jnp.where(zero > 0, q[0:PC].astype(F32).reshape(PC // 8, 8, 128),
                                   jnp.broadcast_to(st[0], (PC // 8, 8, 128)))
                    st = (jnp.concatenate([mu] * 8, axis=2), st[1])
                ln1(xnext(k), 1 - (j & 1), pl.multiple_of(hh * (PC // 2), PC // 2), PC, True, st)

            def epi_piece(k, q):
                hh, j = pairs[k + 1]
                if k + 1 < HP:
                    stats[k + 1] = ln1_stats(xnext(k + 1), PC, zero)
                epi(pl.multiple_of(jnp.maximum(j - 1, 0) * TQ + hh * PC, PC), 1 - (j & 1),
                    pl.multiple_of(hh * PC, PC), PC, j > 0)

            for k in range(HP):
                side += [(functools.partial(ln1_piece, k), False), (functools.partial(epi_piece, k), True)]
            run_units(seq, side, zero, {0: AC0, 1: AC1})
            return 0
        jax.lax.fori_loop(0, NT, main, 0)

        start(d_out((NT - 1 - NG) * HP * PC, HP * PC, sem.at[SEM_OUT]))
        lastp = (NQ - 1) & 1
        base = (NQ - 1) * TQ
        ru = modrow(4) * modrow(6)
        rsu = jnp.sum(ru, axis=-1, keepdims=True)
        rc0 = jnp.sum(modrow(3) * modrow(6), axis=-1, keepdims=True)

        def epis(half):
            for i in range(half * TU // TPC, (half + 1) * TU // TPC):
                epi_a(base + i * TPC, lastp, i * TPC, TPC, ru, rsu, rc0)
        ol = pv((H - 1, 1, lastp), s_sc[...], zero0, ACT)
        outp((H - 1, 0, lastp), (of_sc[...], l_sc[...]))
        outp((H - 1, 1, lastp), ol)
        epis(0)
        epis(1)
        best, second = r_buf[0], r_buf[1]
        for sh in (4, 2, 1):
            b2 = pltpu.roll(best, sh, 0)
            s2 = pltpu.roll(second, sh, 0)
            second = jnp.maximum(jnp.minimum(best, b2), jnp.maximum(second, s2))
            best = jnp.maximum(best, b2)
        i1 = (S - 1) - (best[0, 0] & (S - 1))
        i2 = (S - 1) - (second[0, 0] & (S - 1))
        g1 = pl.multiple_of(jnp.clip(i1 >> 3, 0, S // 8 - 1) * 8, 8)
        g2 = pl.multiple_of(jnp.clip(i2 >> 3, 0, S // 8 - 1) * 8, 8)

        def h2_rows(g):
            nrm = last_norm(lastp, pl.multiple_of(jnp.clip(g - base, 0, TQ - 8), 8), 8)[1]
            last = (nrm * modrow(4) + modrow(3)).reshape(8, D)
            return jnp.where(g >= base, last, x_buf[pl.ds(g, 8), :].astype(F32))
        xs = jnp.concatenate([h2_rows(g1), h2_rows(g2)], axis=0).astype(BF16)
        gt = jnp.dot(xs, wg_buf[...], preferred_element_type=F32)
        up = jnp.dot(xs, wu_buf[...], preferred_element_type=F32)
        gbits = pltpu.bitcast(jnp.concatenate([gt, up], axis=1), I32)
        ga_, gb_ = modrow(5) * modrow(4), modrow(5) * modrow(3)
        npc = TQ // CPC
        for i in range(npc):
            z = jnp.where(i1 < 0, gbits[0, 128 * (i * CSPAN // npc)], 0)
            x1, nrm = last_norm(lastp, pl.multiple_of(jnp.clip(z + i, 0, npc - 1) * CPC, CPC), CPC)
            out_buf[base + i * CPC:base + (i + 1) * CPC, :] = (x1 + nrm * ga_ + gb_).reshape(CPC, D).astype(BF16)
            if i == npc // 2 - 1:
                start(d_out(base, TU, sem.at[SEM_OUT2]))
        start(d_out(base + TU, TU, sem.at[SEM_OUT2]))
        gt = _rb(gt)
        a = (_rb(gt * jax.nn.sigmoid(gt)) * _rb(up)).astype(BF16)
        y = _rb(jnp.dot(a, wd_buf[:, 0:D], preferred_element_type=F32))

        def score(k):
            return pltpu.bitcast((k ^ ((k >> 31) & 0x7FFFFFFF)) & -S, F32)
        ri = jax.lax.broadcasted_iota(I32, (16, 128), 0)
        rows = jnp.where(ri < 8, g1 + ri, g2 + ri - 8)
        r1 = jnp.concatenate([score(best)] * 2, axis=0)
        r2 = jnp.concatenate([score(second)] * 2, axis=0)
        gate = _rb(jax.nn.sigmoid(_rb(jnp.where(rows == i1, r1, r2))))
        sel = (rows == i1) | (rows == i2)
        upd = jnp.where(sel[:, 0:1], _rb(y * gate[:, 0:1]), 0.0) * mod_buf[0:1, 5 * D:6 * D]
        o1 = (out_buf[pl.ds(g1, 8), :].astype(F32) + upd[0:8]).astype(BF16)
        o2 = (out_buf[pl.ds(g2, 8), :].astype(F32) + upd[8:16]).astype(BF16)
        cp(out_buf.at[pl.ds(0, base), :], out_hbm.at[0, pl.ds(0, base), :], sem.at[SEM_OUT]).wait()
        wait(d_out(base, TQ, sem.at[SEM_OUT2]))
        out_buf[pl.ds(g1, 8), :] = o1
        out_buf[pl.ds(g2, 8), :] = o2
        start(d_out(g1, 8, sem.at[SEM_FIX]))

        @pl.when(g1 != g2)
        def _():
            start(d_out(g2, 8, sem.at[SEM_FIX + 1]))
            wait(d_out(g2, 8, sem.at[SEM_FIX + 1]))

        wait(d_out(g1, 8, sem.at[SEM_FIX]))
        return 0
    jax.lax.fori_loop(0, zero0 + 1, rest, 0)


@jax.jit
def pallas_adaLN_cond__mha_block_cached__moe_arch_mod__prompt_kernel(
    A_x: jax.Array,
    A_k_cache: jax.Array,
    A_v_cache: jax.Array,
    A_wq: jax.Array,
    A_wo: jax.Array,
    B_x: jax.Array,
    B_w_r: jax.Array,
    B_w_gate: jax.Array,
    B_w_up: jax.Array,
    B_w_down: jax.Array,
    c: jax.Array,
    w_mod: jax.Array,
):
    del B_x
    vm = pltpu.VMEM
    scratch = [
        vm((S + PC, D), BF16),
        vm((2, TQ // 2, D), U32),
        vm((H, S, DH), BF16),
        vm((H, S, DH), BF16),
        vm((H, D, DH), BF16),
        vm((H * DH, D), BF16),
        vm((D, FF), BF16),
        vm((D, FF), BF16),
        vm((FF, D + 128), BF16),
        vm((D, 6 * D + 128), BF16),
        vm((1, D), BF16),
        vm((8, 128), BF16),
        vm((8, 7 * D), F32),
        vm((2, TQ, D), F32),
        vm((S, D), BF16),
        vm((TU, S), F32),
        vm((TU, DH), F32),
        vm((TU, DH), F32),
        vm((2, 8, 128), I32),
        vm((2, TQ, 128), F32),
        vm((NM + 1, TQ, DH), F32),
        vm((NM + 1, 8, DH), F32),
        vm((TU // 2, DH), U32),
        vm((TQ, D), F32),
        pltpu.SemaphoreType.DMA((NSEM,)),
    ]
    anyspec = pl.BlockSpec(memory_space=pl.ANY)
    return pl.pallas_call(
        _kernel,
        in_specs=[anyspec] * 11,
        out_specs=anyspec,
        out_shape=jax.ShapeDtypeStruct((1, S, D), BF16),
        scratch_shapes=scratch,
        compiler_params=pltpu.CompilerParams(vmem_limit_bytes=120 * 1024 * 1024, disable_bounds_checks=True,
                                             disable_semaphore_checks=True),
    )(A_x, A_k_cache, A_v_cache, A_wq, A_wo, B_w_r.reshape(8, 128), B_w_gate, B_w_up, B_w_down, c, w_mod)
```
